```python
import jax
import jax.numpy as jnp

def _softmax(x, axis=-1):
    return jax.nn.softmax(x, axis=axis)

def _gelu(x):
    return jax.nn.gelu(x, approximate=True)

def _silu(x):
    return jax.nn.silu(x)

def _sigmoid(x):
    return jax.nn.sigmoid(x)

def _layernorm(x, axis=-1, eps=1e-05):
    m = jnp.mean(x, axis=axis, keepdims=True)
    v = jnp.var(x, axis=axis, keepdims=True)
    return (x - m) / jnp.sqrt(v + eps)

def _scatter_add(tgt, idx, src, axis=0):
    return tgt.at[idx].add(src)

def _segment_sum(src, seg, n):
    return jax.ops.segment_sum(src, seg, n)

class _Rng:

    def __init__(self, key):
        self._k = key

    def _next(self):
        self._k, sub = jax.random.split(self._k)
        return sub

    def normal(self, shape):
        return jax.random.normal(self._next(), shape, dtype=jnp.bfloat16)

    def randint(self, lo, hi, shape):
        return jax.random.randint(self._next(), shape, lo, hi, dtype=jnp.int32)

    def uniform(self, shape, lo=0.0, hi=1.0):
        return jax.random.uniform(self._next(), shape, jnp.bfloat16, lo, hi)

    def permutation(self, n):
        return jax.random.permutation(self._next(), n)
kernel_name = 'adaLN_cond__compressed_kv_cla__moe_arch_mod__prompt'

def setup_inputs():
    _rng = _Rng(jax.random.key(int.from_bytes(__import__("os").urandom(4), "little")))
    _w = lambda a: (lambda t: t.astype(jnp.bfloat16) if jnp.issubdtype(t.dtype, jnp.floating) else t)(jnp.asarray(a))

    def _A_setup():
        B, H, Sq, Sk, D, M = (1, 32, 2048, 2048, 128, 640)
        Dc = 4 * D
        return {'x': _w((lambda *s: _rng.normal(s) * 0.05)(B, Sq, M)), 'c_kv': _w((lambda *s: _rng.normal(s) * 0.05)(B, Sk, Dc)), 'w_q': _w((lambda *s: _rng.normal(s) * 0.05)(M, H, D) * M ** (-0.5)), 'w_uk': _w((lambda *s: _rng.normal(s) * 0.05)(Dc, H, D) * Dc ** (-0.5)), 'w_uv': _w((lambda *s: _rng.normal(s) * 0.05)(Dc, H, D) * Dc ** (-0.5)), 'w_o': _w((lambda *s: _rng.normal(s) * 0.05)(H, D, M) * (H * D) ** (-0.5))}
    _A_in = _A_setup()

    def _B_setup():
        B, S, D, F, C = (1, 2048, 640, 1728, 8)
        return {'x': _w((lambda *s: _rng.normal(s) * 0.05)(B, S, D)), 'w_r': _w((lambda *s: _rng.normal(s) * 0.05)(D)), 'w_gate': _w((lambda *s: _rng.normal(s) * 0.05)(D, F)), 'w_up': _w((lambda *s: _rng.normal(s) * 0.05)(D, F)), 'w_down': _w((lambda *s: _rng.normal(s) * 0.05)(F, D))}
    _B_in = _B_setup()
    return {'A_x': _A_in['x'], 'A_c_kv': _A_in['c_kv'], 'A_w_q': _A_in['w_q'], 'A_w_uk': _A_in['w_uk'], 'A_w_uv': _A_in['w_uv'], 'A_w_o': _A_in['w_o'], 'B_x': _B_in['x'], 'B_w_r': _B_in['w_r'], 'B_w_gate': _B_in['w_gate'], 'B_w_up': _B_in['w_up'], 'B_w_down': _B_in['w_down'], 'c': _w((lambda *s: _rng.normal(s) * 0.05)(1, 640)), 'w_mod': _w((lambda *s: _rng.normal(s) * 0.05)(640, 6 * 640) * 640 ** (-0.5))}

def reference(A_x, A_c_kv, A_w_q, A_w_uk, A_w_uv, A_w_o, B_x, B_w_r, B_w_gate, B_w_up, B_w_down, c, w_mod):

    def _A_ref(x, c_kv, w_q, w_uk, w_uv, w_o):
        B, Sq, M = (x.shape[0], x.shape[1], x.shape[2])
        Sk = c_kv.shape[1]
        H, D = (w_q.shape[1], w_q.shape[2])
        q = jnp.einsum('bqm,mhd->bhqd', x, w_q)
        k = jnp.einsum('bkc,chd->bhkd', c_kv, w_uk)
        v = jnp.einsum('bkc,chd->bhkd', c_kv, w_uv)
        scores = jnp.einsum('bhqd,bhkd->bhqk', q, k) * D ** (-0.5)
        off = Sk - Sq
        qi = jnp.arange(Sq)[:, None]
        kj = jnp.arange(Sk)[None, :]
        cmask = kj <= qi + off
        scores = jnp.where(cmask[None, None], scores, -1000000000.0)
        p = _softmax(scores, axis=-1)
        ctx = jnp.einsum('bhqk,bhkd->bhqd', p, v)
        return jnp.einsum('bhqd,hdm->bqm', ctx, w_o)

    def _B_ref(x, w_r, w_gate, w_up, w_down):
        B, S, D = x.shape
        C = 8
        r = x @ w_r
        idx = jnp.argsort(-r, axis=-1)[:, :C]
        idx_e = jnp.repeat(idx.reshape(B, C, 1), D, axis=2)
        x_sel = jnp.take_along_axis(x, idx_e, axis=1)
        g = _silu(x_sel @ w_gate)
        u = x_sel @ w_up
        y = g * u @ w_down
        r_sel = _sigmoid(jnp.take_along_axis(r, idx, axis=1))
        y = y * r_sel.reshape(B, C, 1)
        b_off = (jnp.arange(B) * S).reshape(B, 1)
        flat_idx = (idx + b_off).reshape(B * C)
        zero = (x * 0.0).reshape(B * S, D)
        upd = _scatter_add(zero, flat_idx, y.reshape(B * C, D), axis=0)
        return x + upd.reshape(B, S, D)
    x = A_x
    mod = (_silu(c) @ w_mod).reshape(c.shape[0], 6, 1, -1)
    sa, ca, ga, sb, cb, gb = (mod[:, 0].copy(), mod[:, 1].copy(), mod[:, 2].copy(), mod[:, 3].copy(), mod[:, 4].copy(), mod[:, 5].copy())
    h = _layernorm(x, axis=-1) * (1 + ca) + sa
    x = x + ga * _A_ref(h, A_c_kv, A_w_q, A_w_uk, A_w_uv, A_w_o)
    h = _layernorm(x, axis=-1) * (1 + cb) + sb
    x = x + gb * _B_ref(h, B_w_r, B_w_gate, B_w_up, B_w_down)
    return x
```

```python
import numpy as np
import jax
import jax.numpy as jnp
from jax import lax
import jax.experimental.pallas as pl
import jax.experimental.pallas.tpu as pltpu

CFG = dict(bq=256, eb=256, split_diag=True)

F32 = jnp.float32
BF16 = jnp.bfloat16
U32 = jnp.uint32
I32 = jnp.int32
TOPC = 8
LOG2E = 1.4426950408889634
NT = (((1,), (1,)), ((), ()))


def _rb(a):
    return a.astype(BF16).astype(F32)


def _dot(a, b):
    return jnp.dot(a, b, preferred_element_type=F32)


def _sigmoid(a):
    return 1.0 / (1.0 + jnp.exp(-a))


def _make_kernel(S, M, Dc, H, D, F):
    bq = CFG["bq"]
    eb = CFG["eb"]
    eps_b = float(np.float32(np.asarray(1e-5, dtype=BF16)))
    qscale = float(np.float32(np.asarray(D ** -0.5, dtype=BF16))) * LOG2E
    neg = -1e9 * LOG2E

    def kernel(x_hbm, ckv_hbm, wq_hbm, wuk_hbm, wuv_hbm, wo_hbm, wr_ref, wg_hbm, wu_hbm,
               wd_hbm, c_ref, wmod_hbm, out_hbm,
               x_s, ckv_s, h_s, wq_b, wk_b, wv_b, wo_s, wg_s, wu_s, wd_s, wmod_s,
               q_s, k_s, v_s, ctx_s, out_s, sems, wsems):
        def wcopies(pair, slot):
            return (
                pltpu.make_async_copy(wq_hbm.bitcast(U32).at[:, pair, :], wq_b.at[slot], wsems.at[3 * slot]),
                pltpu.make_async_copy(wuk_hbm.bitcast(U32).at[:, pair, :], wk_b.at[slot], wsems.at[3 * slot + 1]),
                pltpu.make_async_copy(wuv_hbm.bitcast(U32).at[:, pair, :], wv_b.at[slot], wsems.at[3 * slot + 2]),
            )

        cp_mod = pltpu.make_async_copy(wmod_hbm, wmod_s, sems.at[0])
        cp_x = pltpu.make_async_copy(x_hbm.at[0], x_s, sems.at[1])
        cp_ckv = pltpu.make_async_copy(ckv_hbm.at[0], ckv_s, sems.at[2])
        cp_wo = pltpu.make_async_copy(wo_hbm, wo_s, sems.at[3])
        cp_wg = pltpu.make_async_copy(wg_hbm, wg_s, sems.at[4])
        cp_wu = pltpu.make_async_copy(wu_hbm, wu_s, sems.at[5])
        cp_wd = pltpu.make_async_copy(wd_hbm, wd_s, sems.at[6])
        cp_mod.start()
        cp_x.start()
        cp_ckv.start()
        for cp in wcopies(0, 0):
            cp.start()

        cp_mod.wait()
        cv = c_ref[...].astype(F32)
        sc = _rb(cv * _rb(_sigmoid(cv)))
        sc8 = jnp.broadcast_to(sc, (8, M)).astype(BF16)
        mod = _rb(_dot(sc8, wmod_s[...]))[0:1]
        sa, ca, ga, sb, cb, gb = (mod[:, i * M:(i + 1) * M] for i in range(6))
        ca1 = _rb(1.0 + ca)
        cb1 = _rb(1.0 + cb)

        cp_x.wait()
        for r0 in range(0, S, eb):
            xv = x_s[r0:r0 + eb, :].astype(F32)
            mu = jnp.sum(xv, axis=-1, keepdims=True) * (1.0 / M)
            xc = xv - mu
            var = jnp.sum(xc * xc, axis=-1, keepdims=True) * (1.0 / M)
            h_s[r0:r0 + eb, :] = (xc * lax.rsqrt(var + 1e-5) * ca1 + sa).astype(BF16)
        cp_ckv.wait()
        cp_wo.start()
        cp_wg.start()
        cp_wu.start()
        cp_wd.start()

        def unpack(ref, slot, shift):
            u = ref[slot]
            return pltpu.bitcast((u << shift) & np.uint32(0xFFFF0000), F32).astype(BF16)

        def head(h, carry):
            pair = h // 2
            slot = pair % 2
            odd = h % 2

            @pl.when(odd == 0)
            def _():
                for cp in wcopies(pair, slot):
                    cp.wait()

                @pl.when(pair + 1 < H // 2)
                def _():
                    for cp in wcopies(pair + 1, 1 - slot):
                        cp.start()

            shift = (16 - 16 * odd).astype(U32)
            q_s[...] = (_dot(h_s[...], unpack(wq_b, slot, shift)) * qscale).astype(BF16)
            wkv = jnp.concatenate([unpack(wk_b, slot, shift), unpack(wv_b, slot, shift)], axis=1)
            kv = _dot(ckv_s[...], wkv).astype(BF16)
            k_s[...] = kv[:, :D]
            v_s[...] = kv[:, D:]

            tri = lax.broadcasted_iota(I32, (128, 128), 1) <= lax.broadcasted_iota(I32, (128, 128), 0)
            trib = lax.broadcasted_iota(I32, (bq, bq), 1) <= lax.broadcasted_iota(I32, (bq, bq), 0)
            for i in range(S // bq):
                r0 = i * bq
                n = r0 + bq
                q = q_s[r0:n, :]
                if not CFG["split_diag"]:
                    s = lax.dot_general(q, k_s[0:n, :], NT, preferred_element_type=F32)
                    sd = jnp.where(trib, s[:, r0:], neg)
                    s = jnp.concatenate([s[:, :r0], sd], axis=1) if r0 else sd
                    m = jnp.max(s, axis=-1, keepdims=True)
                    p = jnp.exp2(s - m)
                    l = jnp.sum(p, axis=-1, keepdims=True)
                    o = _dot(p.astype(BF16), v_s[0:n, :])
                    ctx_s[h, r0:n, :] = (o * (1.0 / l)).astype(BF16)
                else:
                    nsub = bq // 128
                    cols = []
                    if r0:
                        s0 = lax.dot_general(q, k_s[0:r0, :], NT, preferred_element_type=F32)
                    sd = []
                    for t in range(nsub):
                        st = lax.dot_general(q[128 * t:], k_s[r0 + 128 * t:r0 + 128 * (t + 1), :], NT,
                                             preferred_element_type=F32)
                        sd.append(st)
                    p_rows = []
                    l_rows = []
                    for u in range(nsub):
                        parts = [s0[128 * u:128 * (u + 1)]] if r0 else []
                        for t in range(u + 1):
                            blk = sd[t][128 * (u - t):128 * (u - t + 1)]
                            parts.append(jnp.where(tri, blk, neg) if t == u else blk)
                        srow = jnp.concatenate(parts, axis=1) if len(parts) > 1 else parts[0]
                        m = jnp.max(srow, axis=-1, keepdims=True)
                        p = jnp.exp2(srow - m)
                        l_rows.append(jnp.sum(p, axis=-1, keepdims=True))
                        p_rows.append(p.astype(BF16))
                    o = None
                    if r0:
                        o = _dot(jnp.concatenate([p[:, :r0] for p in p_rows], axis=0), v_s[0:r0, :])
                    o_rows = [o[128 * u:128 * (u + 1)] if r0 else None for u in range(nsub)]
                    for t in range(nsub):
                        pt = jnp.concatenate(
                            [p_rows[u][:, r0 + 128 * t:r0 + 128 * (t + 1)] for u in range(t, nsub)], axis=0)
                        ot = _dot(pt, v_s[r0 + 128 * t:r0 + 128 * (t + 1), :])
                        for u in range(t, nsub):
                            part = ot[128 * (u - t):128 * (u - t + 1)]
                            o_rows[u] = part if o_rows[u] is None else o_rows[u] + part
                    for u in range(nsub):
                        ctx_s[h, r0 + 128 * u:r0 + 128 * (u + 1), :] = (
                            o_rows[u] * (1.0 / l_rows[u])).astype(BF16)
            return carry

        lax.fori_loop(0, H, head, 0)

        cp_wo.wait()
        wr = wr_ref[...].astype(F32).reshape(1, M)
        lane = lax.broadcasted_iota(I32, (8, 128), 1)
        sub = lax.broadcasted_iota(I32, (8, 128), 0)
        nk = S // 1024
        rk = [jnp.zeros((8, 128), F32) for _ in range(nk)]
        for r0 in range(0, S, eb):
            ctx = jnp.concatenate([ctx_s[hh, r0:r0 + eb, :] for hh in range(H)], axis=1)
            a = _rb(_dot(ctx, wo_s[...].reshape(H * D, M)))
            x1 = _rb(x_s[r0:r0 + eb, :].astype(F32) + _rb(ga * a))
            x_s[r0:r0 + eb, :] = x1.astype(BF16)
            mu = jnp.sum(x1, axis=-1, keepdims=True) / M
            xc = x1 - mu
            var = _rb(jnp.sum(xc * xc, axis=-1, keepdims=True) / M)
            inv = 1.0 / _rb(jnp.sqrt(_rb(var + eps_b)))
            h2 = _rb(_rb(_rb(_rb(x1 - _rb(mu)) * inv) * cb1) + sb)
            h_s[r0:r0 + eb, :] = h2.astype(BF16)
            out_s[r0:r0 + eb, :] = (x1 + _rb(gb * h2)).astype(BF16)
            r = jnp.sum(h2 * wr, axis=-1, keepdims=True)
            for j in range(eb // 8):
                g = r0 // 8 + j
                rk[g // 128] = jnp.where(lane == g % 128, r[8 * j:8 * j + 8], rk[g // 128])

        keys = []
        for t in range(nk):
            rv = _rb(rk[t]) + 0.0
            b = lax.shift_right_logical(pltpu.bitcast(rv, I32), 16)
            o16 = jnp.where(b >= 0x8000, 0xFFFF - b, b + 0x8000)
            o16 = jnp.where(rv != rv, 0, o16)
            tok = t * 1024 + lane * 8 + sub
            keys.append(pltpu.bitcast((o16 << 11) + (S - 1 - tok) + (1 << 29), F32))
        sel = []
        for _ in range(TOPC):
            mk = keys[0]
            for t in range(1, nk):
                mk = jnp.maximum(mk, keys[t])
            top = jnp.max(jnp.max(mk, axis=1, keepdims=True), axis=0, keepdims=True)
            keys = [jnp.where(kk == top, 0.0, kk) for kk in keys]
            sel.append(top)
        row8 = lax.broadcasted_iota(I32, (8, 1), 0)
        kcol = jnp.zeros((8, 1), F32)
        for ci in range(TOPC):
            kcol = jnp.where(row8 == ci, sel[ci], kcol)
        ki = pltpu.bitcast(kcol, I32) - (1 << 29)
        o16 = ki >> 11
        rsel = pltpu.bitcast(jnp.where(o16 >= 0x8000, o16 - 0x8000, 0xFFFF - o16) << 16, F32)
        toks = []
        for ci in range(TOPC):
            kv = pltpu.bitcast(sel[ci], I32)
            toks.append(S - 1 - (kv[0, 0] & (S - 1)))

        row16 = lax.broadcasted_iota(I32, (16, M), 0)
        rowc = lax.broadcasted_iota(I32, (8, M), 0)
        xs = jnp.zeros((8, M), F32)
        x1s = jnp.zeros((8, M), F32)
        for ci in range(TOPC):
            g0 = pl.multiple_of((toks[ci] // 16) * 16, 16)
            msk = row16 == toks[ci] - g0
            hv = jnp.sum(jnp.where(msk, h_s[pl.ds(g0, 16), :].astype(F32), 0.0), axis=0, keepdims=True)
            xv = jnp.sum(jnp.where(msk, x_s[pl.ds(g0, 16), :].astype(F32), 0.0), axis=0, keepdims=True)
            xs = jnp.where(rowc == ci, hv, xs)
            x1s = jnp.where(rowc == ci, xv, x1s)

        cp_wg.wait()
        cp_wu.wait()
        cp_wd.wait()
        xsb = xs.astype(BF16)
        gp = _rb(lax.dot_general(xsb, wg_s[...], NT, preferred_element_type=F32))
        g = _rb(gp * _rb(_sigmoid(gp)))
        u = _rb(lax.dot_general(xsb, wu_s[...], NT, preferred_element_type=F32))
        y = _rb(_dot((g * u).astype(BF16), wd_s[...]))
        y = _rb(y * _rb(_sigmoid(rsel)))
        onew = x1s + _rb(gb * _rb(xs + y))
        for ci in range(TOPC):
            g0 = pl.multiple_of((toks[ci] // 16) * 16, 16)
            msk = row16 == toks[ci] - g0
            old = out_s[pl.ds(g0, 16), :].astype(F32)
            out_s[pl.ds(g0, 16), :] = jnp.where(msk, onew[ci:ci + 1], old).astype(BF16)

        cp_out = pltpu.make_async_copy(out_s, out_hbm.at[0], sems.at[7])
        cp_out.start()
        cp_out.wait()

    return kernel


@jax.jit
def pallas_adaLN_cond__compressed_kv_cla__moe_arch_mod__prompt_kernel(
    A_x, A_c_kv, A_w_q, A_w_uk, A_w_uv, A_w_o, B_x, B_w_r, B_w_gate, B_w_up, B_w_down, c, w_mod,
):
    del B_x
    _, S, M = A_x.shape
    Dc = A_c_kv.shape[2]
    H, D = A_w_q.shape[1:]
    F = B_w_gate.shape[1]
    any_spec = pl.BlockSpec(memory_space=pl.ANY)
    vmem_spec = pl.BlockSpec(memory_space=pltpu.VMEM)
    return pl.pallas_call(
        _make_kernel(S, M, Dc, H, D, F),
        out_shape=jax.ShapeDtypeStruct(A_x.shape, A_x.dtype),
        in_specs=[any_spec] * 6 + [vmem_spec] + [any_spec] * 3 + [vmem_spec, any_spec],
        out_specs=any_spec,
        scratch_shapes=[
            pltpu.VMEM((S, M), BF16),
            pltpu.VMEM((S, Dc), BF16),
            pltpu.VMEM((S, M), BF16),
            pltpu.VMEM((2, M, D), U32),
            pltpu.VMEM((2, Dc, D), U32),
            pltpu.VMEM((2, Dc, D), U32),
            pltpu.VMEM((H, D, M), BF16),
            pltpu.VMEM((F, M), BF16),
            pltpu.VMEM((F, M), BF16),
            pltpu.VMEM((F, M), BF16),
            pltpu.VMEM((M, 6 * M), BF16),
            pltpu.VMEM((S, D), BF16),
            pltpu.VMEM((S, D), BF16),
            pltpu.VMEM((S, D), BF16),
            pltpu.VMEM((H, S, D), BF16),
            pltpu.VMEM((S, M), BF16),
            pltpu.SemaphoreType.DMA((8,)),
            pltpu.SemaphoreType.DMA((6,)),
        ],
        compiler_params=pltpu.CompilerParams(vmem_limit_bytes=100 * 1024 * 1024),
        name="adaln_mla_mod",
    )(A_x, A_c_kv, A_w_q, A_w_uk, A_w_uv, A_w_o, B_w_r, B_w_gate.T, B_w_up.T, B_w_down, c, w_mod)
```

```python
import numpy as np
import jax
import jax.numpy as jnp
from jax import lax
import jax.experimental.pallas as pl
import jax.experimental.pallas.tpu as pltpu

CFG = dict(bq=256, eb=256, flags=None, dep=0, skip_epi=False, uw=512, sscr=0, lead=1, mode='fine', fill=None, qmid=0, ur=256, dl=0, qk_takes='f', pv_takes='of', order='Q K a0 V a1 b0 a2 b1 a3 b2 b3', tm=None, tl=1, tf=None, to=None, osched={2:2,4:4,6:6})


def _default_order(n):
    o = ["Q", "K", "a0", "a1", "s0", "V", "b0"]
    for i in range(1, n):
        if i + 1 < n:
            o.append(f"a{i + 1}")
        o += [f"s{i}", f"b{i}"]
    return " ".join(o)


F32 = jnp.float32
BF16 = jnp.bfloat16
U32 = jnp.uint32
I32 = jnp.int32
TOPC = 8
LOG2E = 1.4426950408889634
NT = (((1,), (1,)), ((), ()))


def _rb(a):
    return a.astype(BF16).astype(F32)


def _dot(a, b):
    return jnp.dot(a, b, preferred_element_type=F32)


def _sigmoid(a):
    return 1.0 / (1.0 + jnp.exp(-a))


def _make_kernel(S, M, Dc, H, D, F):
    bq = CFG["bq"]
    eb = CFG["eb"]
    eps_b = float(np.float32(np.asarray(1e-5, dtype=BF16)))
    qscale = float(np.float32(np.asarray(D ** -0.5, dtype=BF16))) * LOG2E
    neg = -1e9 * LOG2E

    def kernel(x_hbm, ckv_hbm, wq_hbm, wuk_hbm, wuv_hbm, wo_hbm, wr_ref, wg_hbm, wu_hbm,
               wd_hbm, c_ref, wmod_hbm, out_hbm,
               x_s, ckv_s, h_s, wq_b, wk_b, wv_b, wo_s, wg_s, wu_s, wd_s, wmod_s,
               q_s, k_s, v_s, ctx_s, out_s, s_s, acc_s, sems, wsems):
        def wcopies(pair, slot):
            return (
                pltpu.make_async_copy(wq_hbm.bitcast(U32).at[:, pair, :], wq_b.at[slot], wsems.at[3 * slot]),
                pltpu.make_async_copy(wuk_hbm.bitcast(U32).at[:, pair, :], wk_b.at[slot], wsems.at[3 * slot + 1]),
                pltpu.make_async_copy(wuv_hbm.bitcast(U32).at[:, pair, :], wv_b.at[slot], wsems.at[3 * slot + 2]),
            )

        cp_mod = pltpu.make_async_copy(wmod_hbm, wmod_s, sems.at[0])
        cp_x = pltpu.make_async_copy(x_hbm.at[0], x_s, sems.at[1])
        cp_ckv = pltpu.make_async_copy(ckv_hbm.at[0], ckv_s, sems.at[2])
        cp_wo = pltpu.make_async_copy(wo_hbm, wo_s, sems.at[3])
        cp_wg = pltpu.make_async_copy(wg_hbm, wg_s, sems.at[4])
        cp_wu = pltpu.make_async_copy(wu_hbm, wu_s, sems.at[5])
        cp_wd = pltpu.make_async_copy(wd_hbm, wd_s, sems.at[6])
        cp_mod.start()
        cp_x.start()
        cp_ckv.start()
        for cp in wcopies(0, 0):
            cp.start()

        cp_mod.wait()
        cv = c_ref[...].astype(F32)
        sc = _rb(cv * _rb(_sigmoid(cv)))
        sc8 = jnp.broadcast_to(sc, (8, M)).astype(BF16)
        mod = _rb(_dot(sc8, wmod_s[...]))[0:1]
        sa, ca, ga, sb, cb, gb = (mod[:, i * M:(i + 1) * M] for i in range(6))
        ca1 = _rb(1.0 + ca)
        cb1 = _rb(1.0 + cb)

        cp_x.wait()
        for r0 in range(0, S, eb):
            xv = x_s[r0:r0 + eb, :].astype(F32)
            mu = jnp.sum(xv, axis=-1, keepdims=True) * (1.0 / M)
            xc = xv - mu
            var = jnp.sum(xc * xc, axis=-1, keepdims=True) * (1.0 / M)
            h_s[r0:r0 + eb, :] = (xc * lax.rsqrt(var + 1e-5) * ca1 + sa).astype(BF16)
        cp_ckv.wait()
        cp_wo.start()
        cp_wg.start()
        cp_wu.start()
        cp_wd.start()

        def unpack(ref, slot, shift):
            u = ref[slot]
            return pltpu.bitcast((u << shift) & np.uint32(0xFFFF0000), F32).astype(BF16)

        def head(h, carry):
            pair = h // 2
            slot = pair % 2
            odd = h % 2

            @pl.when(odd == 0)
            def _():
                for cp in wcopies(pair, slot):
                    cp.wait()

                @pl.when(pair + 1 < H // 2)
                def _():
                    for cp in wcopies(pair + 1, 1 - slot):
                        cp.start()

            shift = (16 - 16 * odd).astype(U32)
            tri = lax.broadcasted_iota(I32, (128, 128), 1) <= lax.broadcasted_iota(I32, (128, 128), 0)
            G = 64
            SB = 512
            ur = CFG["ur"]
            st = {}
            clock = [0]
            pend = []
            always = lax.broadcasted_iota(I32, (8, 128), 0) < h + 8
            rr = lax.broadcasted_iota(I32, (G, 128), 0)
            cc = lax.broadcasted_iota(I32, (G, 128), 1)

            def proj(w_b, src, dst, r0, r1, scale=None):
                w = unpack(w_b, slot, shift)
                if w.shape[0] > 512:
                    n4 = (r1 - r0) // 4
                    o = jnp.concatenate([_dot(src[r0 + n4 * u:r0 + n4 * (u + 1), 512:], w[512:]) for u in range(4)], axis=0)
                    o = o + _dot(src[r0:r1, :512], w[:512])
                else:
                    o = _dot(src[r0:r1, :], w)
                dst[r0:r1, :] = (o * scale if scale else o).astype(BF16)

            def units(a):
                r0 = a * SB
                us = [[(r0 + ro, ur, c0, SB)] for c0 in range(0, r0, SB) for ro in range(0, SB, ur)]
                us.append([(r0, 256, r0, 128), (r0 + 256, 256, r0, 384)])
                us.append([(r0 + 128, 64, r0 + 128, 128), (r0 + 192, 64, r0 + 128, 128),
                           (r0 + 384, 64, r0 + 384, 128), (r0 + 448, 64, r0 + 384, 128)])
                return us

            def acc(key, r0, val, op):
                for u in range(val.shape[0] // G):
                    k = (key, r0 // G + u)
                    part = val[G * u:G * (u + 1)]
                    st[k] = op(st[k], part) if k in st else part

            def get(key, r0, nr):
                v = [st[(key, u)] for u in range(r0 // G, (r0 + nr) // G)]
                return jnp.concatenate(v, axis=0) if len(v) > 1 else v[0]

            def tie(val, deps):
                t = deps[0]
                for d in deps[1:]:
                    t = jnp.maximum(t, d)
                if val.dtype == F32:
                    return jnp.where(jnp.tile(always, (val.shape[0] // 8, 1)), val, t)
                t = pltpu.bitcast(t.astype(BF16), I32)
                return pltpu.bitcast(jnp.where(jnp.tile(always, (t.shape[0] // 8, 1)),
                                               pltpu.bitcast(val, I32), t), BF16)

            def take(nr, kinds):
                ready = [p for p in pend if p[0] <= clock[0] and p[1].shape[0] == nr and p[2] in kinds]
                pend[:] = [p for p in pend if not any(p is z for z in ready)]
                return [p[1] for p in ready]

            def qk(a, j):
                us = units(a)
                for (r0, nr, c0, nc) in us[j]:
                    q = q_s[r0:r0 + nr, :]
                    deps = take(nr, CFG["qk_takes"])
                    if deps:
                        q = tie(q, deps)
                    s = lax.dot_general(q, k_s[c0:c0 + nc, :], NT, preferred_element_type=F32)
                    tiles = []
                    for t in range(nc // 128):
                        x = s[:, 128 * t:128 * (t + 1)]
                        if c0 + 128 * (t + 1) > r0:
                            x = [x[g:g + G] if c0 + 128 * (t + 1) <= r0 + g else
                                 jnp.where(cc + (c0 + 128 * t) <= rr + (r0 + g), x[g:g + G], neg)
                                 for g in range(0, nr, G)]
                            x = jnp.concatenate(x, axis=0) if len(x) > 1 else x[0]
                        tiles.append(x)
                    mm = tiles[0]
                    for t in tiles[1:]:
                        mm = jnp.maximum(mm, t)
                    acc("m", r0, mm, jnp.maximum)
                    st[("s", r0, c0)] = tiles
                clock[0] += us[j][0][1]
                if j == len(us) - 1:
                    for u in range(a * SB // G, (a + 1) * SB // G):
                        st[("m", u)] = jnp.broadcast_to(jnp.max(st[("m", u)], axis=-1, keepdims=True), (G, 128))
                    for r0 in range(a * SB, (a + 1) * SB, ur):
                        pend.append((clock[0] + CFG["dl"], get("m", r0, ur), "M"))
                elif len(us[j]) == 1:
                    pend.append((clock[0] + CFG["dl"], get("m", r0, nr), "m"))

            def pv(a, j):
                us = units(a)
                for (r0, nr, c0, nc) in us[j]:
                    m = get("m", r0, nr)
                    deps = take(nr, CFG["pv_takes"])
                    if deps:
                        m = tie(m, deps)
                    ps = [jnp.exp2(x - m) for x in st.pop(("s", r0, c0))]
                    ll = ps[0]
                    for t in ps[1:]:
                        ll = ll + t
                    acc("l", r0, ll, jnp.add)
                    if CFG["tl"]:
                        ps[-1] = tie(ps[-1], [get("l", r0, nr)])
                    p = jnp.concatenate(ps, axis=1) if len(ps) > 1 else ps[0]
                    acc("o", r0, _dot(p.astype(BF16), v_s[c0:c0 + nc, :]), jnp.add)
                clock[0] += us[j][0][1]
                if j == len(us) - 1:
                    for r0 in range(a * SB, (a + 1) * SB, ur):
                        l = jnp.sum(get("l", r0, ur), axis=-1, keepdims=True)
                        r = pl.reciprocal(l, approx=True)
                        ctx = get("o", r0, ur) * (r * (2.0 - l * r))
                        ctx_s[0 if CFG['fill'] == 'o' else h, r0:r0 + ur, :] = ctx.astype(BF16)
                        pend.append((clock[0] + CFG["dl"], ctx, "f"))
                elif len(us[j]) == 1:
                    pend.append((clock[0] + CFG["dl"], get("o", r0, nr), "o"))

            def oproj(r0, r1):
                acc_s[r0:r1, :512] += _dot(ctx_s[0, r0:r1, :], wo_s[h, :, :512])
                n4 = (r1 - r0) // 4
                for u in range(4):
                    acc_s[r0 + n4 * u:r0 + n4 * (u + 1), 512:] += _dot(
                        ctx_s[0, r0 + n4 * u:r0 + n4 * (u + 1), :], wo_s[h, :, 512:])

            nb = S // SB
            for tok in CFG["order"].split():
                if tok == "Q": proj(wq_b, h_s, q_s, 0, S, qscale)
                elif tok == "K": proj(wk_b, ckv_s, k_s, 0, S)
                elif tok == "V": proj(wv_b, ckv_s, v_s, 0, S)
                elif tok[0] == "O": oproj(int(tok[1]) * SB, int(tok[2]) * SB)
                elif tok[0] == "a":
                    for j in range(len(units(int(tok[1])))): qk(int(tok[1]), j)
                elif tok[0] == "b":
                    for j in range(len(units(int(tok[1])))): pv(int(tok[1]), j)
                elif tok[0] == "x":
                    qa, pa = int(tok[1]), int(tok[2])
                    nq, npv = len(units(qa)), len(units(pa))
                    seq = [("q", j) for j in range(nq - npv)]
                    for j in range(npv):
                        seq += [("q", nq - npv + j), ("p", j)]
                    for kind, j in seq:
                        (qk(qa, j) if kind == "q" else pv(pa, j))
            return carry

        lax.fori_loop(0, H, head, 0)

        cp_wo.wait()
        wr = wr_ref[...].astype(F32).reshape(1, M)
        lane = lax.broadcasted_iota(I32, (8, 128), 1)
        sub = lax.broadcasted_iota(I32, (8, 128), 0)
        nk = S // 1024
        rk = [jnp.zeros((8, 128), F32) for _ in range(nk)]
        for r0 in range(0, eb if CFG['skip_epi'] else S, eb):
            ctx = jnp.concatenate([ctx_s[hh, r0:r0 + eb, :] for hh in range(H)], axis=1)
            a = _rb(_dot(ctx, wo_s[...].reshape(H * D, M)))
            x1 = _rb(x_s[r0:r0 + eb, :].astype(F32) + _rb(ga * a))
            x_s[r0:r0 + eb, :] = x1.astype(BF16)
            mu = jnp.sum(x1, axis=-1, keepdims=True) / M
            xc = x1 - mu
            var = _rb(jnp.sum(xc * xc, axis=-1, keepdims=True) / M)
            inv = 1.0 / _rb(jnp.sqrt(_rb(var + eps_b)))
            h2 = _rb(_rb(_rb(_rb(x1 - _rb(mu)) * inv) * cb1) + sb)
            h_s[r0:r0 + eb, :] = h2.astype(BF16)
            out_s[r0:r0 + eb, :] = (x1 + _rb(gb * h2)).astype(BF16)
            r = jnp.sum(h2 * wr, axis=-1, keepdims=True)
            for j in range(eb // 8):
                g = r0 // 8 + j
                rk[g // 128] = jnp.where(lane == g % 128, r[8 * j:8 * j + 8], rk[g // 128])

        keys = []
        for t in range(nk):
            rv = _rb(rk[t]) + 0.0
            b = lax.shift_right_logical(pltpu.bitcast(rv, I32), 16)
            o16 = jnp.where(b >= 0x8000, 0xFFFF - b, b + 0x8000)
            o16 = jnp.where(rv != rv, 0, o16)
            tok = t * 1024 + lane * 8 + sub
            keys.append(pltpu.bitcast((o16 << 11) + (S - 1 - tok) + (1 << 29), F32))
        sel = []
        for _ in range(TOPC):
            mk = keys[0]
            for t in range(1, nk):
                mk = jnp.maximum(mk, keys[t])
            top = jnp.max(jnp.max(mk, axis=1, keepdims=True), axis=0, keepdims=True)
            keys = [jnp.where(kk == top, 0.0, kk) for kk in keys]
            sel.append(top)
        row8 = lax.broadcasted_iota(I32, (8, 1), 0)
        kcol = jnp.zeros((8, 1), F32)
        for ci in range(TOPC):
            kcol = jnp.where(row8 == ci, sel[ci], kcol)
        ki = pltpu.bitcast(kcol, I32) - (1 << 29)
        o16 = ki >> 11
        rsel = pltpu.bitcast(jnp.where(o16 >= 0x8000, o16 - 0x8000, 0xFFFF - o16) << 16, F32)
        toks = []
        for ci in range(TOPC):
            kv = pltpu.bitcast(sel[ci], I32)
            toks.append(S - 1 - (kv[0, 0] & (S - 1)))

        row16 = lax.broadcasted_iota(I32, (16, M), 0)
        rowc = lax.broadcasted_iota(I32, (8, M), 0)
        xs = jnp.zeros((8, M), F32)
        x1s = jnp.zeros((8, M), F32)
        for ci in range(TOPC):
            g0 = pl.multiple_of((toks[ci] // 16) * 16, 16)
            msk = row16 == toks[ci] - g0
            hv = jnp.sum(jnp.where(msk, h_s[pl.ds(g0, 16), :].astype(F32), 0.0), axis=0, keepdims=True)
            xv = jnp.sum(jnp.where(msk, x_s[pl.ds(g0, 16), :].astype(F32), 0.0), axis=0, keepdims=True)
            xs = jnp.where(rowc == ci, hv, xs)
            x1s = jnp.where(rowc == ci, xv, x1s)

        cp_wg.wait()
        cp_wu.wait()
        cp_wd.wait()
        xsb = xs.astype(BF16)
        gp = _rb(lax.dot_general(xsb, wg_s[...], NT, preferred_element_type=F32))
        g = _rb(gp * _rb(_sigmoid(gp)))
        u = _rb(lax.dot_general(xsb, wu_s[...], NT, preferred_element_type=F32))
        y = _rb(_dot((g * u).astype(BF16), wd_s[...]))
        y = _rb(y * _rb(_sigmoid(rsel)))
        onew = x1s + _rb(gb * _rb(xs + y))
        for ci in range(TOPC):
            g0 = pl.multiple_of((toks[ci] // 16) * 16, 16)
            msk = row16 == toks[ci] - g0
            old = out_s[pl.ds(g0, 16), :].astype(F32)
            out_s[pl.ds(g0, 16), :] = jnp.where(msk, onew[ci:ci + 1], old).astype(BF16)

        cp_out = pltpu.make_async_copy(out_s, out_hbm.at[0], sems.at[7])
        cp_out.start()
        cp_out.wait()

    return kernel


@jax.jit
def pallas_adaLN_cond__compressed_kv_cla__moe_arch_mod__prompt_kernel(
    A_x, A_c_kv, A_w_q, A_w_uk, A_w_uv, A_w_o, B_x, B_w_r, B_w_gate, B_w_up, B_w_down, c, w_mod,
):
    del B_x
    _, S, M = A_x.shape
    Dc = A_c_kv.shape[2]
    H, D = A_w_q.shape[1:]
    F = B_w_gate.shape[1]
    any_spec = pl.BlockSpec(memory_space=pl.ANY)
    vmem_spec = pl.BlockSpec(memory_space=pltpu.VMEM)
    return pl.pallas_call(
        _make_kernel(S, M, Dc, H, D, F),
        out_shape=jax.ShapeDtypeStruct(A_x.shape, A_x.dtype),
        in_specs=[any_spec] * 6 + [vmem_spec] + [any_spec] * 3 + [vmem_spec, any_spec],
        out_specs=any_spec,
        scratch_shapes=[
            pltpu.VMEM((S, M), BF16),
            pltpu.VMEM((S, Dc), BF16),
            pltpu.VMEM((S, M), BF16),
            pltpu.VMEM((2, M, D), U32),
            pltpu.VMEM((2, Dc, D), U32),
            pltpu.VMEM((2, Dc, D), U32),
            pltpu.VMEM((H, D, M), BF16),
            pltpu.VMEM((F, M), BF16),
            pltpu.VMEM((F, M), BF16),
            pltpu.VMEM((F, M), BF16),
            pltpu.VMEM((M, 6 * M), BF16),
            pltpu.VMEM((S, D), BF16),
            pltpu.VMEM((S, D), BF16),
            pltpu.VMEM((S, D), BF16),
            pltpu.VMEM((H, S, D), BF16),
            pltpu.VMEM((S, M), BF16),
            pltpu.VMEM((max(CFG['sscr'], 1), CFG['bq'], S), F32),
            pltpu.VMEM((S, M), F32),
            pltpu.SemaphoreType.DMA((8,)),
            pltpu.SemaphoreType.DMA((6,)),
        ],
        compiler_params=pltpu.CompilerParams(vmem_limit_bytes=100 * 1024 * 1024, flags=CFG['flags']),
        name="adaln_mla_mod",
    )(A_x, A_c_kv, A_w_q, A_w_uk, A_w_uv, A_w_o, B_w_r, B_w_gate.T, B_w_up.T, B_w_down, c, w_mod)
```

```python
import numpy as np
import jax
import jax.numpy as jnp
from jax import lax
import jax.experimental.pallas as pl
import jax.experimental.pallas.tpu as pltpu

CFG = dict(ur=256, dl=0, qk_takes='f', pv_takes='ofm', tl=1, flags=None, skip_epi=False, skip_kv=False,
           eblocks=(256,) * 7 + (128, 128), ln2g=32, ln1g=32,
           order='QA a0A QB a1A b0A a2A b1A a3A b2A a0B b3A a1B b0B a2B b1B a3B b2B b3B')

F32 = jnp.float32
BF16 = jnp.bfloat16
U32 = jnp.uint32
I32 = jnp.int32
TOPC = 8
LOG2E = 1.4426950408889634
NT = (((1,), (1,)), ((), ()))
G = 64
SB = 512


def _rb(a):
    return a.astype(BF16).astype(F32)


def _dot(a, b):
    return jnp.dot(a, b, preferred_element_type=F32)


def _dot_nt(a, b):
    return lax.dot_general(a, b, NT, preferred_element_type=F32)


def _sigmoid(a):
    return 1.0 / (1.0 + jnp.exp(-a))


def _cat(xs, axis):
    return jnp.concatenate(xs, axis=axis) if len(xs) > 1 else xs[0]


def _halves(u):
    return pltpu.bitcast(u << 16, F32), pltpu.bitcast(u & np.uint32(0xFFFF0000), F32)


def _after(always, val, deps):
    t = deps[0]
    for d in deps[1:]:
        t = jnp.maximum(t, d)
    if val.dtype == F32:
        return jnp.where(jnp.tile(always, (val.shape[0] // 8, 1)), val, t)
    t = pltpu.bitcast(t.astype(BF16), I32)
    return pltpu.bitcast(jnp.where(jnp.tile(always, (t.shape[0] // 8, 1)), pltpu.bitcast(val, I32), t), BF16)


def _make_kernel(S, M, Dc, H, D, F):
    NP = H // 2
    ur = CFG["ur"]
    eps_b = float(np.float32(np.asarray(1e-5, dtype=BF16)))
    qscale = float(np.float32(np.asarray(D ** -0.5, dtype=BF16))) * LOG2E
    neg = -1e9 * LOG2E

    def units(a):
        r0 = a * SB
        us = [[(r0 + ro, ur, c0, SB)] for c0 in range(0, r0, SB) for ro in range(0, SB, ur)]
        us.append([(r0, 256, r0, 128), (r0 + 256, 256, r0, 384)])
        us.append([(r0 + 128, 64, r0 + 128, 128), (r0 + 192, 64, r0 + 128, 128),
                   (r0 + 384, 64, r0 + 384, 128), (r0 + 448, 64, r0 + 384, 128)])
        return us

    def kernel(x_hbm, ckv_hbm, wq_hbm, wuk_hbm, wuv_hbm, wo_hbm, wr_ref, wg_hbm, wu_hbm,
               wd_hbm, c_ref, wmod_hbm, out_hbm,
               x_s, ckv_s, h_s, wq_b, wk_b, wv_b, wo_s, wg_s, wu_s, wd_s, wma_s, wmb_s,
               q_s, k_s, v_s, ctx_s, out_s, sems, wsems, osems, psems):
        def wcopy(which, p):
            src, dst = ((wq_hbm, wq_b), (wuk_hbm, wk_b), (wuv_hbm, wv_b))[which]
            return pltpu.make_async_copy(src.bitcast(U32).at[:, p, :], dst.at[p], wsems.at[which * NP + p])

        def kv_copies(p0, p1):
            return [wcopy(w, p) for p in range(p0, p1) for w in (1, 2)]

        cp_ckv = pltpu.make_async_copy(ckv_hbm.at[0], ckv_s, sems.at[0])
        cp_x = pltpu.make_async_copy(x_hbm.at[0], x_s, sems.at[1])
        cp_ma = pltpu.make_async_copy(wmod_hbm.at[:, 0:2 * M], wma_s, sems.at[2])
        late = [pltpu.make_async_copy(wmod_hbm.at[:, 2 * M:6 * M], wmb_s, sems.at[3]),
                pltpu.make_async_copy(wo_hbm, wo_s, sems.at[4]),
                pltpu.make_async_copy(wg_hbm, wg_s, sems.at[5]),
                pltpu.make_async_copy(wu_hbm, wu_s, sems.at[6]),
                pltpu.make_async_copy(wd_hbm, wd_s, sems.at[7])]

        def start(cps):
            for cp in cps:
                cp.start()

        def wait(cps):
            for cp in cps:
                cp.wait()

        def kv_proj(p):
            res = []
            for w_b, dst in ((wk_b, k_s), (wv_b, v_s)):
                for e, w in enumerate(_halves(w_b[p])):
                    o = _dot(ckv_s[...], w.astype(BF16))
                    dst[2 * p + e] = o.astype(BF16)
                    res.append(o)
            return res

        start([cp_ckv] + kv_copies(0, 1))
        wait([cp_ckv] + kv_copies(0, 1))
        start(kv_copies(1, 4) + [cp_ma, cp_x])
        kv_proj(0)
        wait(kv_copies(1, 4))
        start(kv_copies(4, NP))
        if not CFG["skip_kv"]:
            for p in range(1, 4):
                kv_proj(p)
        wait([cp_ma, cp_x] + kv_copies(4, NP))
        start([wcopy(0, p) for p in range(NP)] + late)

        cv = c_ref[...].astype(F32)
        sc8 = jnp.broadcast_to(_rb(cv * _rb(_sigmoid(cv))), (8, M)).astype(BF16)
        moda = _rb(_dot(sc8, wma_s[...]))[0:1]
        sa, ca1 = moda[:, :M], _rb(1.0 + moda[:, M:])

        def kv_step(i, carry):
            always = lax.broadcasted_iota(I32, (8, 128), 0) < i + 8
            res = []
            for u in range(3):
                res += kv_proj(4 + 3 * i + u)
            g = CFG["ln1g"]
            rows = S // 4
            for n, r in enumerate(range(0, rows, g)):
                r0 = pl.multiple_of(i * rows + r, g)
                xv = x_s[pl.ds(r0, g), :].astype(F32)
                pos = n * (len(res) - 1) * S // (rows // g)
                dep = res[pos // S][pos % S:pos % S + g]
                xv = _cat([_after(always, xv[:, t:t + 128], [dep]) for t in range(0, M, 128)], 1)
                mu = jnp.sum(xv, axis=-1, keepdims=True) * (1.0 / M)
                xc = xv - mu
                var = jnp.sum(xc * xc, axis=-1, keepdims=True) * (1.0 / M)
                h_s[pl.ds(r0, g), :] = (xc * lax.rsqrt(var + 1e-5) * ca1 + sa).astype(BF16)
            return carry

        lax.fori_loop(0, 4, kv_step, 0)
        wait([wcopy(0, p) for p in range(NP)])

        def pair(p, carry):
            always = lax.broadcasted_iota(I32, (8, 128), 0) < p + 8
            rr = lax.broadcasted_iota(I32, (G, 128), 0)
            cc = lax.broadcasted_iota(I32, (G, 128), 1)
            st, clock, pend = {}, [0], []

            def proj_q(e):
                w = _halves(wq_b[p])[e].astype(BF16)
                n4 = S // 4
                o = _cat([_dot(h_s[n4 * u:n4 * (u + 1), 512:], w[512:]) for u in range(4)], 0)
                o = o + _dot(h_s[:, :512], w[:512])
                q_s[e] = (o * qscale).astype(BF16)
                clock[0] += S

            def acc(key, r0, val, op):
                for u in range(val.shape[0] // G):
                    k = (key, r0 // G + u)
                    part = val[G * u:G * (u + 1)]
                    st[k] = op(st[k], part) if k in st else part

            def get(key, r0, nr):
                return _cat([st[(key, u)] for u in range(r0 // G, (r0 + nr) // G)], 0)

            def take(val, kinds):
                ready = [z for z in pend if z[0] <= clock[0] and z[1].shape[0] == val.shape[0] and z[2] in kinds]
                pend[:] = [z for z in pend if not any(z is y for y in ready)]
                return _after(always, val, [z[1] for z in ready]) if ready else val

            def qk(e, a, j):
                us = units(a)
                for (r0, nr, c0, nc) in us[j]:
                    q = take(q_s[e, r0:r0 + nr, :], CFG["qk_takes"])
                    s = _dot_nt(q, k_s[2 * p + e, c0:c0 + nc, :])
                    tiles = []
                    for t in range(nc // 128):
                        x = s[:, 128 * t:128 * (t + 1)]
                        if c0 + 128 * (t + 1) > r0:
                            x = _cat([x[g:g + G] if c0 + 128 * (t + 1) <= r0 + g else
                                      jnp.where(cc + (c0 + 128 * t) <= rr + (r0 + g), x[g:g + G], neg)
                                      for g in range(0, nr, G)], 0)
                        tiles.append(x)
                    mm = tiles[0]
                    for t in tiles[1:]:
                        mm = jnp.maximum(mm, t)
                    acc(("m", e), r0, mm, jnp.maximum)
                    st[("s", e, r0, c0)] = tiles
                clock[0] += us[j][0][1]
                if j == len(us) - 1:
                    for u in range(a * SB // G, (a + 1) * SB // G):
                        k = (("m", e), u)
                        st[k] = jnp.broadcast_to(jnp.max(st[k], axis=-1, keepdims=True), (G, 128))
                    for r0 in range(a * SB, (a + 1) * SB, ur):
                        pend.append((clock[0] + CFG["dl"], get(("m", e), r0, ur), "M"))
                else:
                    pend[:] = [z for z in pend if z[2] not in "mo"]
                    pend.append((clock[0] + CFG["dl"], get(("m", e), r0, nr), "m"))

            def pv(e, a, j):
                us = units(a)
                for (r0, nr, c0, nc) in us[j]:
                    m = take(get(("m", e), r0, nr), CFG["pv_takes"])
                    ps = [jnp.exp2(x - m) for x in st.pop(("s", e, r0, c0))]
                    ll = ps[0]
                    for t in ps[1:]:
                        ll = ll + t
                    acc(("l", e), r0, ll, jnp.add)
                    if CFG["tl"]:
                        ps[-1] = _after(always, ps[-1], [get(("l", e), r0, nr)])
                    acc(("o", e), r0, _dot(_cat(ps, 1).astype(BF16), v_s[2 * p + e, c0:c0 + nc, :]), jnp.add)
                clock[0] += us[j][0][1]
                if j == len(us) - 1:
                    for r0 in range(a * SB, (a + 1) * SB, ur):
                        l = jnp.sum(get(("l", e), r0, ur), axis=-1, keepdims=True)
                        r = pl.reciprocal(l, approx=True)
                        ctx = get(("o", e), r0, ur) * (r * (2.0 - l * r))
                        ctx_s[2 * p + e, r0:r0 + ur, :] = ctx.astype(BF16)
                        pend.append((clock[0] + CFG["dl"], ctx, "f"))
                else:
                    pend[:] = [z for z in pend if z[2] not in "mo"]
                    pend.append((clock[0] + CFG["dl"], get(("o", e), r0, nr), "o"))

            for tok in CFG["order"].split():
                if tok[0] == "Q":
                    proj_q("AB".index(tok[1]))
                elif tok[0] in "ab":
                    for j in range(len(units(int(tok[1])))):
                        (qk if tok[0] == "a" else pv)("AB".index(tok[2]), int(tok[1]), j)
                elif tok[0] == "x":
                    qa, qe, pa, pe = int(tok[1]), "AB".index(tok[2]), int(tok[3]), "AB".index(tok[4])
                    nq, npv = len(units(qa)), len(units(pa))
                    seq = sorted([((j + 0.5) / nq, 0, j) for j in range(nq)] + [((j + 1.0) / npv, 1, j) for j in range(npv)])
                    for _, kind, j in seq:
                        (pv(pe, pa, j) if kind else qk(qe, qa, j))
            return carry

        lax.fori_loop(0, NP, pair, 0)

        wait(late)
        modb = _rb(_dot(sc8, wmb_s[...]))[0:1]
        ga, sb, cb1, gb = modb[:, :M], modb[:, M:2 * M], _rb(1.0 + modb[:, 2 * M:3 * M]), modb[:, 3 * M:]
        wr = wr_ref[...].astype(F32).reshape(1, M)
        always = jnp.broadcast_to(pltpu.bitcast(wr[:, :128], I32) | 1, (8, 128)) != 0
        lane = lax.broadcasted_iota(I32, (8, 128), 1)
        sub = lax.broadcasted_iota(I32, (8, 128), 0)
        nk = S // 1024
        rk = [jnp.zeros((8, 128), F32) for _ in range(nk)]

        def o_proj(r0, nr):
            cols, marks = [], []
            for n in range(0, M, 128):
                o = None
                for h0 in range(0, H, 4):
                    ctx = _cat([ctx_s[hh, r0:r0 + nr, :] for hh in range(h0, h0 + 4)], 1)
                    w = _cat([wo_s[hh, :, n:n + 128] for hh in range(h0, h0 + 4)], 0)
                    d = _dot(ctx, w)
                    o = d if o is None else o + d
                    marks.append(o)
                cols.append(o)
            return cols, marks

        def ln2(r0, cols):
            nr = cols[0].shape[0]
            a = _rb(_cat(cols, 1))
            x1 = _rb(x_s[r0:r0 + nr, :].astype(F32) + _rb(ga * a))
            x_s[r0:r0 + nr, :] = x1.astype(BF16)
            mu = jnp.sum(x1, axis=-1, keepdims=True) / M
            xc = x1 - mu
            var = _rb(jnp.sum(xc * xc, axis=-1, keepdims=True) / M)
            inv = 1.0 / _rb(jnp.sqrt(_rb(var + eps_b)))
            h2 = _rb(_rb(_rb(_rb(x1 - _rb(mu)) * inv) * cb1) + sb)
            h_s[r0:r0 + nr, :] = h2.astype(BF16)
            out_s[r0:r0 + nr, :] = (x1 + _rb(gb * h2)).astype(BF16)
            r = jnp.sum(h2 * wr, axis=-1, keepdims=True)
            for j in range(nr // 8):
                g = r0 // 8 + j
                rk[g // 128] = jnp.where(lane == g % 128, r[8 * j:8 * j + 8], rk[g // 128])

        eblocks = CFG["eblocks"][:2] if CFG["skip_epi"] else CFG["eblocks"]
        starts = [sum(eblocks[:i]) for i in range(len(eblocks))]
        out_cps = [pltpu.make_async_copy(out_s.at[r0:r0 + nr], out_hbm.at[0, r0:r0 + nr], osems.at[i])
                   for i, (r0, nr) in enumerate(zip(starts, eblocks))]
        prev = None
        for i in range(len(eblocks) + 1):
            marks = None
            if i < len(eblocks):
                cols, marks = o_proj(starts[i], eblocks[i])
            if prev is not None:
                g = CFG["ln2g"]
                ng = eblocks[i - 1] // g
                for n in range(ng):
                    part = [cv_[n * g:(n + 1) * g] for cv_ in prev]
                    if marks:
                        dep = marks[n * (len(marks) - 8) // ng][:g]
                        part = [_after(always, pt, [dep]) for pt in part]
                    ln2(starts[i - 1] + n * g, part)
                out_cps[i - 1].start()
            prev = cols

        keys = []
        for t in range(nk):
            rv = _rb(rk[t])
            b = lax.shift_right_logical(pltpu.bitcast(jnp.where(rv == 0.0, 0.0, rv), I32), 16)
            o16 = jnp.where(b >= 0x8000, 0xFFFF - b, b + 0x8000)
            o16 = jnp.where(rv != rv, 0, o16)
            tok = t * 1024 + lane * 8 + sub
            keys.append(pltpu.bitcast((o16 << 11) + (S - 1 - tok) + (1 << 29), F32))
        sel = []
        for _ in range(TOPC):
            mk = keys[0]
            for t in range(1, nk):
                mk = jnp.maximum(mk, keys[t])
            top = jnp.max(jnp.max(mk, axis=1, keepdims=True), axis=0, keepdims=True)
            keys = [jnp.where(kk == top, 0.0, kk) for kk in keys]
            sel.append(top)
        row8 = lax.broadcasted_iota(I32, (8, 1), 0)
        kcol = jnp.zeros((8, 1), F32)
        for ci in range(TOPC):
            kcol = jnp.where(row8 == ci, sel[ci], kcol)
        o16 = (pltpu.bitcast(kcol, I32) - (1 << 29)) >> 11
        rsel = pltpu.bitcast(jnp.where(o16 >= 0x8000, o16 - 0x8000, 0xFFFF - o16) << 16, F32)
        toks = [S - 1 - (pltpu.bitcast(sel[ci], I32)[0, 0] & (S - 1)) for ci in range(TOPC)]
        grps = [pl.multiple_of(tk & (S - 16), 16) for tk in toks]

        row16 = lax.broadcasted_iota(I32, (16, M), 0)
        rowc = lax.broadcasted_iota(I32, (8, M), 0)
        xs = jnp.zeros((8, M), F32)
        x1s = jnp.zeros((8, M), F32)
        for ci in range(TOPC):
            msk = row16 == (toks[ci] & 15)
            hv = jnp.sum(jnp.where(msk, h_s[pl.ds(grps[ci], 16), :].astype(F32), 0.0), axis=0, keepdims=True)
            xv = jnp.sum(jnp.where(msk, x_s[pl.ds(grps[ci], 16), :].astype(F32), 0.0), axis=0, keepdims=True)
            xs = jnp.where(rowc == ci, hv, xs)
            x1s = jnp.where(rowc == ci, xv, x1s)

        xsb = xs.astype(BF16)
        gp = _rb(_dot_nt(xsb, wg_s[...]))
        g = _rb(gp * _rb(_sigmoid(gp)))
        u = _rb(_dot_nt(xsb, wu_s[...]))
        y = _rb(_dot((g * u).astype(BF16), wd_s[...]))
        y = _rb(y * _rb(_sigmoid(rsel)))
        onew = x1s + _rb(gb * _rb(xs + y))

        wait(out_cps)
        for ci in range(TOPC):
            msk = row16 == (toks[ci] & 15)
            old = out_s[pl.ds(grps[ci], 16), :].astype(F32)
            out_s[pl.ds(grps[ci], 16), :] = jnp.where(msk, onew[ci:ci + 1], old).astype(BF16)
        fresh = []
        for ci in range(TOPC):
            f = grps[ci] >= 0
            for cj in range(ci):
                f = jnp.logical_and(f, grps[cj] != grps[ci])
            fresh.append(f)
        patch = [pltpu.make_async_copy(out_s.at[pl.ds(grps[ci], 16)], out_hbm.at[0, pl.ds(grps[ci], 16)],
                                       psems.at[ci]) for ci in range(TOPC)]
        for ci in range(TOPC):
            pl.when(fresh[ci])(patch[ci].start)
        for ci in range(TOPC):
            pl.when(fresh[ci])(patch[ci].wait)

    return kernel


@jax.jit
def pallas_adaLN_cond__compressed_kv_cla__moe_arch_mod__prompt_kernel(
    A_x, A_c_kv, A_w_q, A_w_uk, A_w_uv, A_w_o, B_x, B_w_r, B_w_gate, B_w_up, B_w_down, c, w_mod,
):
    del B_x
    _, S, M = A_x.shape
    Dc = A_c_kv.shape[2]
    H, D = A_w_q.shape[1:]
    F = B_w_gate.shape[1]
    any_spec = pl.BlockSpec(memory_space=pl.ANY)
    vmem_spec = pl.BlockSpec(memory_space=pltpu.VMEM)
    return pl.pallas_call(
        _make_kernel(S, M, Dc, H, D, F),
        out_shape=jax.ShapeDtypeStruct(A_x.shape, A_x.dtype),
        in_specs=[any_spec] * 6 + [vmem_spec] + [any_spec] * 3 + [vmem_spec, any_spec],
        out_specs=any_spec,
        scratch_shapes=[
            pltpu.VMEM((S, M), BF16),
            pltpu.VMEM((S, Dc), BF16),
            pltpu.VMEM((S, M), BF16),
            pltpu.VMEM((H // 2, M, D), U32),
            pltpu.VMEM((H // 2, Dc, D), U32),
            pltpu.VMEM((H // 2, Dc, D), U32),
            pltpu.VMEM((H, D, M), BF16),
            pltpu.VMEM((F, M), BF16),
            pltpu.VMEM((F, M), BF16),
            pltpu.VMEM((F, M), BF16),
            pltpu.VMEM((M, 2 * M), BF16),
            pltpu.VMEM((M, 4 * M), BF16),
            pltpu.VMEM((2, S, D), BF16),
            pltpu.VMEM((H, S, D), BF16),
            pltpu.VMEM((H, S, D), BF16),
            pltpu.VMEM((H, S, D), BF16),
            pltpu.VMEM((S, M), BF16),
            pltpu.SemaphoreType.DMA((8,)),
            pltpu.SemaphoreType.DMA((3 * H // 2,)),
            pltpu.SemaphoreType.DMA((len(CFG["eblocks"]),)),
            pltpu.SemaphoreType.DMA((TOPC,)),
        ],
        compiler_params=pltpu.CompilerParams(vmem_limit_bytes=120 * 1024 * 1024, flags=CFG["flags"]),
        name="adaln_mla_mod",
    )(A_x, A_c_kv, A_w_q, A_w_uk, A_w_uv, A_w_o, B_w_r, B_w_gate.T, B_w_up.T, B_w_down, c, w_mod)
```

```python
import contextlib
import numpy as np
import jax
import jax.numpy as jnp
from jax import lax
import jax.experimental.pallas as pl
import jax.experimental.pallas.tpu as pltpu

CFG = dict(ur=256, dl=0, qk_takes='f', pv_takes='ofm', tl=1, flags=None, skip_epi=False, skip_kv=False,
           eblocks=(512, 512, 512, 256, 128, 128), ln2g=32, ln1g=32,
           order='QA W a0A QB a1A b0A a2A b1A a3A b2A a0B b3A a1B b0B a2B b1B a3B b2B b3B')

F32 = jnp.float32
BF16 = jnp.bfloat16
U32 = jnp.uint32
I32 = jnp.int32
TOPC = 8
LOG2E = 1.4426950408889634
NT = (((1,), (1,)), ((), ()))
G = 64
RG = 16
SB = 512


def _scope(name):
    return jax.named_scope(name) if CFG.get('scopes') else contextlib.nullcontext()


def _rb(a):
    return a.astype(BF16).astype(F32)


def _dot(a, b):
    return jnp.dot(a, b, preferred_element_type=F32)


def _dot_nt(a, b):
    return lax.dot_general(a, b, NT, preferred_element_type=F32)


def _sigmoid(a):
    return 1.0 / (1.0 + jnp.exp(-a))


def _cat(xs, axis):
    return jnp.concatenate(xs, axis=axis) if len(xs) > 1 else xs[0]


def _halves(u):
    return pltpu.bitcast(u << 16, F32), pltpu.bitcast(u & np.uint32(0xFFFF0000), F32)


def _after(always, val, deps):
    t = deps[0]
    for d in deps[1:]:
        t = jnp.maximum(t, d)
    if val.dtype == F32:
        return jnp.where(jnp.tile(always, (val.shape[0] // 8, 1)), val, t)
    t = pltpu.bitcast(t.astype(BF16), I32)
    return pltpu.bitcast(jnp.where(jnp.tile(always, (t.shape[0] // 8, 1)), pltpu.bitcast(val, I32), t), BF16)


def _split_rows(x):
    n = x.shape[0] // (2 * RG)
    y = x.reshape(n, 2, RG, x.shape[1])
    return y[:, 0].reshape(n * RG, x.shape[1]), y[:, 1].reshape(n * RG, x.shape[1])


def _merge_rows(top, bot):
    n = top.shape[0] // RG
    y = jnp.concatenate([top.reshape(n, 1, RG, top.shape[1]), bot.reshape(n, 1, RG, top.shape[1])], axis=1)
    return y.reshape(2 * n * RG, top.shape[1])


_LHS = (lambda a: a[0][0] + a[1][1], lambda a: a[1][0] + a[1][1], lambda a: a[0][0], lambda a: a[1][1],
        lambda a: a[0][0] + a[0][1], lambda a: a[1][0] - a[0][0], lambda a: a[0][1] - a[1][1])
_RHS = (lambda b: b[0][0] + b[1][1], lambda b: b[0][0], lambda b: b[0][1] - b[1][1],
        lambda b: b[1][0] - b[0][0], lambda b: b[1][1], lambda b: b[0][0] + b[0][1],
        lambda b: b[1][0] + b[1][1])
_ORDER = (2, 4, 3, 1, 0, 6, 5)


def _combine(m):
    return (((m[3] - m[4]) + m[0] + m[6], m[2] + m[4]),
            (m[1] + m[3], (m[2] - m[1]) + m[0] + m[5]))


def _make_kernel(S, M, Dc, H, D, F):
    NP = H // 2
    ur = CFG["ur"]
    eps_b = float(np.float32(np.asarray(1e-5, dtype=BF16)))
    qscale = float(np.float32(np.asarray(D ** -0.5, dtype=BF16))) * LOG2E
    neg = -1e9 * LOG2E

    def units(a):
        r0 = a * SB
        us = [[(r0 + ro, ur, c0, SB)] for c0 in range(0, r0, SB) for ro in range(0, SB, ur)]
        us.append([(r0, 256, r0, 128), (r0 + 256, 256, r0, 384)])
        us.append([(r0 + 128, 64, r0 + 128, 128), (r0 + 192, 64, r0 + 128, 128),
                   (r0 + 384, 64, r0 + 384, 128), (r0 + 448, 64, r0 + 384, 128)])
        return us

    def kernel(x_hbm, ckv_hbm, wq_hbm, wuk_hbm, wuv_hbm, wo_hbm, wr_ref, wg_hbm, wu_hbm,
               wd_hbm, c_ref, wmod_hbm, out_hbm,
               x_s, ckv_s, h_s, wq_b, wk_b, wv_b, wo_s, wg_s, wu_s, wd_s, wma_s, wmb_s,
               q_s, k_s, v_s, ctx_s, out_s, cl_s, hl_s, wor_s, sems, wsems, osems, psems):
        def wcopy(which, p):
            src, dst = ((wq_hbm, wq_b), (wuk_hbm, wk_b), (wuv_hbm, wv_b))[which]
            return pltpu.make_async_copy(src.bitcast(U32).at[:, p, :], dst.at[p], wsems.at[which * NP + p])

        def kv_copies(p0, p1):
            return [wcopy(w, p) for p in range(p0, p1) for w in (1, 2)]

        cp_ckv = pltpu.make_async_copy(ckv_hbm.at[0], ckv_s, sems.at[0])
        cp_x = pltpu.make_async_copy(x_hbm.at[0], x_s, sems.at[1])
        cp_ma = pltpu.make_async_copy(wmod_hbm.at[:, 0:2 * M], wma_s, sems.at[2])
        cp_wo = pltpu.make_async_copy(wo_hbm, wo_s, sems.at[4])
        late = [pltpu.make_async_copy(wmod_hbm.at[:, 2 * M:6 * M], wmb_s, sems.at[3]),
                pltpu.make_async_copy(wg_hbm, wg_s, sems.at[5]),
                pltpu.make_async_copy(wu_hbm, wu_s, sems.at[6]),
                pltpu.make_async_copy(wd_hbm, wd_s, sems.at[7])]

        def start(cps):
            for cp in cps:
                cp.start()

        nwait = [0]

        def wait(cps):
            nwait[0] += 1
            with _scope(f"wait{nwait[0]}"):
                for cp in cps:
                    cp.wait()

        def blocks_of(u):
            w = _halves(u)
            hk = u.shape[0] // 2
            return ((w[0][:hk], w[1][:hk]), (w[0][hk:], w[1][hk:]))

        def kv_proj(p):
            bk, bv = blocks_of(wk_b[p]), blocks_of(wv_b[p])
            m = [None] * 7
            for i in _ORDER:
                m[i] = _dot(cl_s[i], _cat([_RHS[i](bk), _RHS[i](bv)], 1).astype(BF16))
            cc = _combine(m)
            for e in range(2):
                o = _merge_rows(cc[0][e], cc[1][e])
                k_s[2 * p + e] = o[:, :D].astype(BF16)
                v_s[2 * p + e] = o[:, D:].astype(BF16)
            return [m[i][:, :D] for i in _ORDER]

        start([cp_ckv] + kv_copies(0, 1))
        wait([cp_ckv] + kv_copies(0, 1))
        start(kv_copies(1, 4) + [cp_ma, cp_x])
        ct, cb = _split_rows(ckv_s[...].astype(F32))
        ca = ((ct[:, :Dc // 2], ct[:, Dc // 2:]), (cb[:, :Dc // 2], cb[:, Dc // 2:]))
        for i in _ORDER:
            cl_s[i] = _LHS[i](ca).astype(BF16)
        kv_proj(0)
        wait(kv_copies(1, 4))
        start(kv_copies(4, NP))
        if not CFG["skip_kv"]:
            for p in range(1, 4):
                kv_proj(p)
        wait([cp_ma, cp_x] + kv_copies(4, NP))
        start([wcopy(0, p) for p in range(NP)] + [cp_wo] + late)

        cv = c_ref[...].astype(F32)
        sc8 = jnp.broadcast_to(_rb(cv * _rb(_sigmoid(cv))), (8, M)).astype(BF16)
        moda = _rb(_dot(sc8, wma_s[...]))[0:1]
        sa, ca1 = moda[:, :M], _rb(1.0 + moda[:, M:])

        def kv_step(i, carry):
            always = lax.broadcasted_iota(I32, (8, 128), 0) < i + 8
            res = []
            for u in range(3):
                res += kv_proj(4 + 3 * i + u)
            g = CFG["ln1g"]
            rows = S // 4
            for n, r in enumerate(range(0, rows, g)):
                r0 = pl.multiple_of(i * rows + r, g)
                xv = x_s[pl.ds(r0, g), :].astype(F32)
                dep = res[n * (len(res) - 1) // (rows // g)][:g]
                xv = _cat([_after(always, xv[:, t:t + 128], [dep]) for t in range(0, M, 128)], 1)
                mu = jnp.sum(xv, axis=-1, keepdims=True) * (1.0 / M)
                xc = xv - mu
                var = jnp.sum(xc * xc, axis=-1, keepdims=True) * (1.0 / M)
                ht, hb = _split_rows(xc * lax.rsqrt(var + 1e-5) * ca1 + sa)
                ha = ((ht[:, :256], ht[:, 256:512]), (hb[:, :256], hb[:, 256:512]))
                rh = pl.ds(pl.multiple_of(i * (rows // 2) + r // 2, g // 2), g // 2)
                for j in range(7):
                    hl_s[j, rh, :] = _LHS[j](ha).astype(BF16)
                hl_s[7, rh, :] = _cat([ht[:, 512:], hb[:, 512:]], 1).astype(BF16)
            return carry

        with _scope('kvloop'):
            lax.fori_loop(0, 4, kv_step, 0)
        wait([wcopy(0, p) for p in range(NP)] + [cp_wo])

        def o_operands(p, always=None, dep=None):
            wa, wb = wo_s[2 * p, :, :512].astype(F32), wo_s[2 * p + 1, :, :512].astype(F32)
            if dep is not None:
                wa, wb = (_cat([_after(always, w[:, t:t + 128], [dep]) for t in range(0, 512, 128)], 1) for w in (wa, wb))
            bo = ((wa[:, :256], wa[:, 256:]), (wb[:, :256], wb[:, 256:]))
            for i in range(7):
                wor_s[i, p] = _RHS[i](bo).astype(BF16)

        if "W" not in CFG["order"].split():
            for p in range(NP):
                o_operands(p)

        def pair(p, carry):
            always = lax.broadcasted_iota(I32, (8, 128), 0) < p + 8
            rr = lax.broadcasted_iota(I32, (G, 128), 0)
            cc = lax.broadcasted_iota(I32, (G, 128), 1)
            st, clock, pend = {}, [0], []

            def proj_q(e):
                bq = blocks_of(wq_b[p, :512, :])
                if e == 0:
                    wt = _cat(_halves(wq_b[p, 512:, :]), 1).astype(BF16)
                    st["qt"] = [_dot(hl_s[7, :, :128], wt), _dot(hl_s[7, :, 128:], wt)]
                    st["qm"] = [None] * 7
                    for i in _ORDER[:-1]:
                        st["qm"][i] = _dot(hl_s[i], _RHS[i](bq).astype(BF16))
                    m = st["qm"]
                    top, bot = (m[3] - m[4]) + m[0] + m[6], m[1] + m[3]
                else:
                    m = st["qm"]
                    w = _RHS[5](bq).astype(BF16)
                    m[5] = _cat([_dot(hl_s[5, :S // 4, :], w), _dot(hl_s[5, S // 4:, :], w)], 0)
                    top, bot = m[2] + m[4], (m[2] - m[1]) + m[0] + m[5]
                o = _merge_rows(top + st["qt"][0][:, D * e:D * (e + 1)], bot + st["qt"][1][:, D * e:D * (e + 1)])
                q_s[e] = (o * qscale).astype(BF16)
                clock[0] += 512

            def acc(key, r0, val, op):
                for u in range(val.shape[0] // G):
                    k = (key, r0 // G + u)
                    part = val[G * u:G * (u + 1)]
                    st[k] = op(st[k], part) if k in st else part

            def get(key, r0, nr):
                return _cat([st[(key, u)] for u in range(r0 // G, (r0 + nr) // G)], 0)

            def take(val, kinds):
                ready = [z for z in pend if z[0] <= clock[0] and z[1].shape[0] == val.shape[0] and z[2] in kinds]
                pend[:] = [z for z in pend if not any(z is y for y in ready)]
                return _after(always, val, [z[1] for z in ready]) if ready else val

            def qk(e, a, j):
                us = units(a)
                for (r0, nr, c0, nc) in us[j]:
                    q = take(q_s[e, r0:r0 + nr, :], CFG["qk_takes"])
                    s = _dot_nt(q, k_s[2 * p + e, c0:c0 + nc, :])
                    tiles = []
                    for t in range(nc // 128):
                        x = s[:, 128 * t:128 * (t + 1)]
                        if c0 + 128 * (t + 1) > r0:
                            x = _cat([x[g:g + G] if c0 + 128 * (t + 1) <= r0 + g else
                                      jnp.where(cc + (c0 + 128 * t) <= rr + (r0 + g), x[g:g + G], neg)
                                      for g in range(0, nr, G)], 0)
                        tiles.append(x)
                    mm = tiles[0]
                    for t in tiles[1:]:
                        mm = jnp.maximum(mm, t)
                    acc(("m", e), r0, mm, jnp.maximum)
                    st[("s", e, r0, c0)] = tiles
                clock[0] += us[j][0][1]
                if j == len(us) - 1:
                    for u in range(a * SB // G, (a + 1) * SB // G):
                        k = (("m", e), u)
                        st[k] = jnp.broadcast_to(jnp.max(st[k], axis=-1, keepdims=True), (G, 128))
                    for r0 in range(a * SB, (a + 1) * SB, ur):
                        pend.append((clock[0] + CFG["dl"], get(("m", e), r0, ur), "M"))
                else:
                    pend[:] = [z for z in pend if z[2] not in "mo"]
                    pend.append((clock[0] + CFG["dl"], get(("m", e), r0, nr), "m"))

            def pv(e, a, j):
                us = units(a)
                for (r0, nr, c0, nc) in us[j]:
                    m = take(get(("m", e), r0, nr), CFG["pv_takes"])
                    ps = [jnp.exp2(x - m) for x in st.pop(("s", e, r0, c0))]
                    ll = ps[0]
                    for t in ps[1:]:
                        ll = ll + t
                    acc(("l", e), r0, ll, jnp.add)
                    if CFG["tl"]:
                        ps[-1] = _after(always, ps[-1], [get(("l", e), r0, nr)])
                    acc(("o", e), r0, _dot(_cat(ps, 1).astype(BF16), v_s[2 * p + e, c0:c0 + nc, :]), jnp.add)
                clock[0] += us[j][0][1]
                if j == len(us) - 1:
                    for r0 in range(a * SB, (a + 1) * SB, ur):
                        l = jnp.sum(get(("l", e), r0, ur), axis=-1, keepdims=True)
                        r = pl.reciprocal(l, approx=True)
                        ctx = get(("o", e), r0, ur) * (r * (2.0 - l * r))
                        ctx_s[2 * p + e, r0:r0 + ur, :] = ctx.astype(BF16)
                        pend.append((clock[0] + CFG["dl"], ctx, "f"))
                else:
                    pend[:] = [z for z in pend if z[2] not in "mo"]
                    pend.append((clock[0] + CFG["dl"], get(("o", e), r0, nr), "o"))

            for tok in CFG["order"].split():
                if tok == "W":
                    o_operands(p, always, st["qm"][2][:D])
                elif tok[0] == "Q":
                    proj_q("AB".index(tok[1]))
                elif tok[0] in "ab":
                    for j in range(len(units(int(tok[1])))):
                        (qk if tok[0] == "a" else pv)("AB".index(tok[2]), int(tok[1]), j)
                elif tok[0] == "x":
                    qa, qe, pa, pe = int(tok[1]), "AB".index(tok[2]), int(tok[3]), "AB".index(tok[4])
                    nq, npv = len(units(qa)), len(units(pa))
                    seq = sorted([((j + 0.5) / nq, 0, j) for j in range(nq)] + [((j + 1.0) / npv, 1, j) for j in range(npv)])
                    for _, kind, j in seq:
                        (pv(pe, pa, j) if kind else qk(qe, qa, j))
            return carry

        with _scope('attn'):
            lax.fori_loop(0, NP, pair, 0)

        wait(late)
        modb = _rb(_dot(sc8, wmb_s[...]))[0:1]
        ga, sb, cb1, gb = modb[:, :M], modb[:, M:2 * M], _rb(1.0 + modb[:, 2 * M:3 * M]), modb[:, 3 * M:]
        wr = wr_ref[...].astype(F32).reshape(1, M)
        always = jnp.broadcast_to(pltpu.bitcast(wr[:, :128], I32) | 1, (8, 128)) != 0
        lane = lax.broadcasted_iota(I32, (8, 128), 1)
        sub = lax.broadcasted_iota(I32, (8, 128), 0)
        nk = S // 1024
        rk = [jnp.zeros((8, 128), F32) for _ in range(nk)]

        def o_proj(r0, nr):
            marks = []
            m = [None] * 7
            for p0 in range(0, NP, 2):
                for i in _ORDER:
                    lhs = []
                    for pp in (p0, p0 + 1):
                        a0, a1 = (_split_rows(ctx_s[2 * pp + e, r0:r0 + nr, :].astype(F32)) for e in range(2))
                        lhs.append(_LHS[i](((a0[0], a1[0]), (a0[1], a1[1]))))
                    d = _dot(_cat(lhs, 1).astype(BF16), _cat([wor_s[i, p0], wor_s[i, p0 + 1]], 0))
                    m[i] = d if m[i] is None else m[i] + d
                    marks.append(m[i][:, :128])
            tail = None
            for h0 in range(0, H, 4):
                d = _dot(_cat([ctx_s[hh, r0:r0 + nr, :] for hh in range(h0, h0 + 4)], 1),
                         _cat([wo_s[hh, :, 512:] for hh in range(h0, h0 + 4)], 0))
                tail = d if tail is None else tail + d
                marks.append(tail)
            cc = _combine(m)
            o = _cat([_merge_rows(cc[0][e], cc[1][e]) for e in range(2)], 1)
            return [o[:, n:n + 128] for n in range(0, 512, 128)] + [tail], marks

        def ln2(r0, cols):
            nr = cols[0].shape[0]
            a = _rb(_cat(cols, 1))
            x1 = _rb(x_s[r0:r0 + nr, :].astype(F32) + _rb(ga * a))
            x_s[r0:r0 + nr, :] = x1.astype(BF16)
            mu = jnp.sum(x1, axis=-1, keepdims=True) / M
            xc = x1 - mu
            var = _rb(jnp.sum(xc * xc, axis=-1, keepdims=True) / M)
            inv = 1.0 / _rb(jnp.sqrt(_rb(var + eps_b)))
            h2 = _rb(_rb(_rb(_rb(x1 - _rb(mu)) * inv) * cb1) + sb)
            h_s[r0:r0 + nr, :] = h2.astype(BF16)
            out_s[r0:r0 + nr, :] = (x1 + _rb(gb * h2)).astype(BF16)
            r = jnp.sum(h2 * wr, axis=-1, keepdims=True)
            for j in range(nr // 8):
                g = r0 // 8 + j
                rk[g // 128] = jnp.where(lane == g % 128, r[8 * j:8 * j + 8], rk[g // 128])

        eblocks = CFG["eblocks"][:2] if CFG["skip_epi"] else CFG["eblocks"]
        starts = [sum(eblocks[:i]) for i in range(len(eblocks))]
        out_cps = [pltpu.make_async_copy(out_s.at[r0:r0 + nr], out_hbm.at[0, r0:r0 + nr], osems.at[i])
                   for i, (r0, nr) in enumerate(zip(starts, eblocks))]
        prev = None
        for i in range(len(eblocks) + 1):
            marks = None
            if i < len(eblocks):
                cols, marks = o_proj(starts[i], eblocks[i])
            if prev is not None:
                g = CFG["ln2g"]
                ng = eblocks[i - 1] // g
                for n in range(ng):
                    part = [cv_[n * g:(n + 1) * g] for cv_ in prev]
                    if marks:
                        dep = marks[n * (len(marks) - 8) // ng][:g]
                        part = [_after(always, pt, [dep]) for pt in part]
                    ln2(starts[i - 1] + n * g, part)
                out_cps[i - 1].start()
            prev = cols

        keys = []
        for t in range(nk):
            rv = _rb(rk[t])
            b = lax.shift_right_logical(pltpu.bitcast(jnp.where(rv == 0.0, 0.0, rv), I32), 16)
            o16 = jnp.where(b >= 0x8000, 0xFFFF - b, b + 0x8000)
            o16 = jnp.where(rv != rv, 0, o16)
            tok = t * 1024 + lane * 8 + sub
            keys.append(pltpu.bitcast((o16 << 11) + (S - 1 - tok) + (1 << 29), F32))
        sel = []
        for _ in range(TOPC):
            mk = keys[0]
            for t in range(1, nk):
                mk = jnp.maximum(mk, keys[t])
            top = jnp.max(jnp.max(mk, axis=1, keepdims=True), axis=0, keepdims=True)
            keys = [jnp.where(kk == top, 0.0, kk) for kk in keys]
            sel.append(top)
        row8 = lax.broadcasted_iota(I32, (8, 1), 0)
        kcol = jnp.zeros((8, 1), F32)
        for ci in range(TOPC):
            kcol = jnp.where(row8 == ci, sel[ci], kcol)
        o16 = (pltpu.bitcast(kcol, I32) - (1 << 29)) >> 11
        rsel = pltpu.bitcast(jnp.where(o16 >= 0x8000, o16 - 0x8000, 0xFFFF - o16) << 16, F32)
        toks = [S - 1 - (pltpu.bitcast(sel[ci], I32)[0, 0] & (S - 1)) for ci in range(TOPC)]
        grps = [pl.multiple_of(tk & (S - 16), 16) for tk in toks]

        row16 = lax.broadcasted_iota(I32, (16, M), 0)
        rowc = lax.broadcasted_iota(I32, (8, M), 0)
        xs = jnp.zeros((8, M), F32)
        x1s = jnp.zeros((8, M), F32)
        for ci in range(TOPC):
            msk = row16 == (toks[ci] & 15)
            hv = jnp.sum(jnp.where(msk, h_s[pl.ds(grps[ci], 16), :].astype(F32), 0.0), axis=0, keepdims=True)
            xv = jnp.sum(jnp.where(msk, x_s[pl.ds(grps[ci], 16), :].astype(F32), 0.0), axis=0, keepdims=True)
            xs = jnp.where(rowc == ci, hv, xs)
            x1s = jnp.where(rowc == ci, xv, x1s)

        xsb = xs.astype(BF16)
        gp = _rb(_dot_nt(xsb, wg_s[...]))
        g = _rb(gp * _rb(_sigmoid(gp)))
        u = _rb(_dot_nt(xsb, wu_s[...]))
        y = _rb(_dot((g * u).astype(BF16), wd_s[...]))
        y = _rb(y * _rb(_sigmoid(rsel)))
        onew = x1s + _rb(gb * _rb(xs + y))

        wait(out_cps)
        for ci in range(TOPC):
            msk = row16 == (toks[ci] & 15)
            old = out_s[pl.ds(grps[ci], 16), :].astype(F32)
            out_s[pl.ds(grps[ci], 16), :] = jnp.where(msk, onew[ci:ci + 1], old).astype(BF16)
        fresh = []
        for ci in range(TOPC):
            f = grps[ci] >= 0
            for cj in range(ci):
                f = jnp.logical_and(f, grps[cj] != grps[ci])
            fresh.append(f)
        patch = [pltpu.make_async_copy(out_s.at[pl.ds(grps[ci], 16)], out_hbm.at[0, pl.ds(grps[ci], 16)],
                                       psems.at[ci]) for ci in range(TOPC)]
        for ci in range(TOPC):
            pl.when(fresh[ci])(patch[ci].start)
        for ci in range(TOPC):
            pl.when(fresh[ci])(patch[ci].wait)

    return kernel


@jax.jit
def pallas_adaLN_cond__compressed_kv_cla__moe_arch_mod__prompt_kernel(
    A_x, A_c_kv, A_w_q, A_w_uk, A_w_uv, A_w_o, B_x, B_w_r, B_w_gate, B_w_up, B_w_down, c, w_mod,
):
    del B_x
    _, S, M = A_x.shape
    Dc = A_c_kv.shape[2]
    H, D = A_w_q.shape[1:]
    F = B_w_gate.shape[1]
    any_spec = pl.BlockSpec(memory_space=pl.ANY)
    vmem_spec = pl.BlockSpec(memory_space=pltpu.VMEM)
    return pl.pallas_call(
        _make_kernel(S, M, Dc, H, D, F),
        out_shape=jax.ShapeDtypeStruct(A_x.shape, A_x.dtype),
        in_specs=[any_spec] * 6 + [vmem_spec] + [any_spec] * 3 + [vmem_spec, any_spec],
        out_specs=any_spec,
        scratch_shapes=[
            pltpu.VMEM((S, M), BF16),
            pltpu.VMEM((S, Dc), BF16),
            pltpu.VMEM((S, M), BF16),
            pltpu.VMEM((H // 2, M, D), U32),
            pltpu.VMEM((H // 2, Dc, D), U32),
            pltpu.VMEM((H // 2, Dc, D), U32),
            pltpu.VMEM((H, D, M), BF16),
            pltpu.VMEM((F, M), BF16),
            pltpu.VMEM((F, M), BF16),
            pltpu.VMEM((F, M), BF16),
            pltpu.VMEM((M, 2 * M), BF16),
            pltpu.VMEM((M, 4 * M), BF16),
            pltpu.VMEM((2, S, D), BF16),
            pltpu.VMEM((H, S, D), BF16),
            pltpu.VMEM((H, S, D), BF16),
            pltpu.VMEM((H, S, D), BF16),
            pltpu.VMEM((S, M), BF16),
            pltpu.VMEM((7, S // 2, Dc // 2), BF16),
            pltpu.VMEM((8, S // 2, 256), BF16),
            pltpu.VMEM((7, H // 2, D, 256), BF16),
            pltpu.SemaphoreType.DMA((8,)),
            pltpu.SemaphoreType.DMA((3 * H // 2,)),
            pltpu.SemaphoreType.DMA((len(CFG["eblocks"]),)),
            pltpu.SemaphoreType.DMA((TOPC,)),
        ],
        compiler_params=pltpu.CompilerParams(vmem_limit_bytes=124 * 1024 * 1024, flags=CFG["flags"]),
        name="adaln_mla_mod",
    )(A_x, A_c_kv, A_w_q, A_w_uk, A_w_uv, A_w_o, B_w_r, B_w_gate.T, B_w_up.T, B_w_down, c, w_mod)
```

```python
import contextlib
import numpy as np
import jax
import jax.numpy as jnp
from jax import lax
import jax.experimental.pallas as pl
import jax.experimental.pallas.tpu as pltpu

CFG = dict(ur=256, dl=0, df=256, fin_in='ab', fin_dep=1, dM=256, dposa=(-2, 0.5), dposb=(0.5, 1.5), chunks=(512, 512, 1024), stage=0, lag=2, qk_takes='fM', pv_takes='f', tl=1, flags=None, skip_epi=False, skip_kv=False,
           eblocks=(512, 512, 384, 256, 192, 128, 64), ln2g=8, ln2span=60, ln1g=32,
           order='QA W a0A QB a1A b0A a2A b1A a3A b2A a0B b3A a1B b0B a2B b1B a3B b2B b3B')

F32 = jnp.float32
BF16 = jnp.bfloat16
U32 = jnp.uint32
I32 = jnp.int32
TOPC = 8
LOG2E = 1.4426950408889634
NT = (((1,), (1,)), ((), ()))
G = 64
RG = 16
SB = 512


def _scope(name):
    return jax.named_scope(name) if CFG.get('scopes') else contextlib.nullcontext()


def _rb(a):
    return a.astype(BF16).astype(F32)


def _dot(a, b):
    return jnp.dot(a, b, preferred_element_type=F32)


def _dot_nt(a, b):
    return lax.dot_general(a, b, NT, preferred_element_type=F32)


def _sigmoid(a):
    return 1.0 / (1.0 + jnp.exp(-a))


def _cat(xs, axis):
    return jnp.concatenate(xs, axis=axis) if len(xs) > 1 else xs[0]


def _halves(u):
    return pltpu.bitcast(u << 16, F32), pltpu.bitcast(u & np.uint32(0xFFFF0000), F32)


def _after(always, val, deps):
    t = deps[0]
    for d in deps[1:]:
        t = jnp.maximum(t, d)
    if val.dtype == F32:
        return jnp.where(jnp.tile(always, (val.shape[0] // 8, 1)), val, t)
    t = pltpu.bitcast(t.astype(BF16), I32)
    return pltpu.bitcast(jnp.where(jnp.tile(always, (t.shape[0] // 8, 1)), pltpu.bitcast(val, I32), t), BF16)


class _Side:
    def __init__(self, always):
        self.always, self.jobs, self.done, self.n = always, {}, {}, 0

    def spread(self, jobs, span):
        for t, job in enumerate(jobs):
            self.jobs.setdefault(self.n + t * span // len(jobs), []).append(job)

    def lhs(self, x):
        toks = self.done.pop(self.n, None)
        if not toks:
            return x
        rows = 8 if x.dtype == F32 else 16
        head = _after(self.always, x[:rows, :128], [jnp.tile(t, (rows // 8, 1)) for t in toks])
        return _cat([_cat([head, x[rows:, :128]], 0), x[:, 128:]], 1)

    def result(self, d):
        for job in self.jobs.pop(self.n, ()):
            tok = job(d[:, :128])
            if tok is not None:
                self.done.setdefault(self.n + CFG["lag"], []).append(tok)
        self.n += 1


def _split_rows(x):
    n = x.shape[0] // (2 * RG)
    y = x.reshape(n, 2, RG, x.shape[1])
    return y[:, 0].reshape(n * RG, x.shape[1]), y[:, 1].reshape(n * RG, x.shape[1])


def _merge_rows(top, bot):
    n = top.shape[0] // RG
    y = jnp.concatenate([top.reshape(n, 1, RG, top.shape[1]), bot.reshape(n, 1, RG, top.shape[1])], axis=1)
    return y.reshape(2 * n * RG, top.shape[1])


_LHS = (lambda a: a[0][0] + a[1][1], lambda a: a[1][0] + a[1][1], lambda a: a[0][0], lambda a: a[1][1],
        lambda a: a[0][0] + a[0][1], lambda a: a[1][0] - a[0][0], lambda a: a[0][1] - a[1][1])
_RHS = (lambda b: b[0][0] + b[1][1], lambda b: b[0][0], lambda b: b[0][1] - b[1][1],
        lambda b: b[1][0] - b[0][0], lambda b: b[1][1], lambda b: b[0][0] + b[0][1],
        lambda b: b[1][0] + b[1][1])
_ORDER = (2, 4, 3, 1, 0, 6, 5)


def _combine(m):
    return (((m[3] - m[4]) + m[0] + m[6], m[2] + m[4]),
            (m[1] + m[3], (m[2] - m[1]) + m[0] + m[5]))


def _make_kernel(S, M, Dc, H, D, F):
    NP = H // 2
    FA = F // 128 * 128
    ur = CFG["ur"]
    eps_b = float(np.float32(np.asarray(1e-5, dtype=BF16)))
    qscale = float(np.float32(np.asarray(D ** -0.5, dtype=BF16))) * LOG2E
    neg = -1e9 * LOG2E

    def units(a, kind='a'):
        r0 = a * SB
        us = [[(r0 + ro, ur, c0, SB)] for c0 in range(0, r0, SB) for ro in range(0, SB, ur)]
        us.append([(r0, 256, r0, 128), (r0 + 256, 256, r0, 384)])
        us.append([(r0 + 128, 64, r0 + 128, 128), (r0 + 192, 64, r0 + 128, 128),
                   (r0 + 384, 64, r0 + 384, 128), (r0 + 448, 64, r0 + 384, 128)])
        full, dbig, dsmall = us[:-2], us[-2], us[-1]
        kb, ks = CFG["dpos" + kind]
        keyed = [(i, u) for i, u in enumerate(full)] + [(kb, dbig), (ks, dsmall)]
        us = [u for _, u in sorted(keyed, key=lambda z: z[0])]
        return us

    def kernel(x_hbm, ckv_hbm, wq_hbm, wuk_hbm, wuv_hbm, wo_hbm, wr_hbm, wg_hbm, wu_hbm,
               wd_hbm, c_hbm, wmod_hbm, out_hbm,
               x_s, ckv_s, h_s, wq_b, wk_b, wv_b, wo_s, wg_s, wu_s, wd_s, wma_s, wmb_s,
               q_s, k_s, v_s, ctx_s, out_s, cl_s, hl_s, wor_s, c_s, wr_s, sems):
        def wcopy(which, p):
            src, dst = ((wq_hbm, wq_b), (wuk_hbm, wk_b), (wuv_hbm, wv_b))[which]
            return pltpu.make_async_copy(src.bitcast(U32).at[:, p, :], dst.at[p],
                                         sems.at[2 if which == 0 else 6 if p == 0 else 0 if p < 4 else 1])

        def kv_copies(p0, p1):
            return [wcopy(w, p) for p in range(p0, p1) for w in (1, 2)]

        cp_c = pltpu.make_async_copy(c_hbm, c_s, sems.at[0])
        cp_wr = pltpu.make_async_copy(wr_hbm, wr_s, sems.at[0])
        cp_x = pltpu.make_async_copy(x_hbm.at[0], x_s, sems.at[1])
        cp_ma = pltpu.make_async_copy(wmod_hbm.at[:, 0:2 * M], wma_s, sems.at[0])
        cp_wo = pltpu.make_async_copy(wo_hbm, wo_s, sems.at[2])
        late = [pltpu.make_async_copy(wmod_hbm.at[:, 2 * M:6 * M], wmb_s, sems.at[3]),
                pltpu.make_async_copy(wg_hbm, wg_s, sems.at[3]),
                pltpu.make_async_copy(wu_hbm, wu_s, sems.at[3]),
                pltpu.make_async_copy(wd_hbm, wd_s, sems.at[3])]

        def start(cps):
            for cp in cps:
                cp.start()

        nwait = [0]

        def wait(cps):
            nwait[0] += 1
            with _scope(f"wait{nwait[0]}"):
                for cp in cps:
                    cp.wait()

        def blocks_of(u):
            w = _halves(u)
            hk = u.shape[0] // 2
            return ((w[0][:hk], w[1][:hk]), (w[0][hk:], w[1][hk:]))

        def kv_proj(p, side, r0=0, nr=S):
            bk, bv = blocks_of(wk_b[p]), blocks_of(wv_b[p])
            m = [None] * 7
            for i in _ORDER:
                m[i] = _dot(side.lhs(cl_s[i, r0 // 2:(r0 + nr) // 2, :]),
                            _cat([_RHS[i](bk), _RHS[i](bv)], 1).astype(BF16))
                side.result(m[i])
            cc = _combine(m)
            for e in range(2):
                o = _merge_rows(cc[0][e], cc[1][e])
                k_s[2 * p + e, r0:r0 + nr, :] = o[:, :D].astype(BF16)
                v_s[2 * p + e, r0:r0 + nr, :] = o[:, D:].astype(BF16)

        def modulation(w_s, always, outs):
            cv = c_s[...].astype(F32)
            sc = _rb(cv * _rb(_sigmoid(cv)))
            eye = lax.broadcasted_iota(I32, (128, 128), 0) == lax.broadcasted_iota(I32, (128, 128), 1)
            col = _cat([jnp.sum(jnp.where(eye, sc[:, t:t + 128], 0.0), axis=1, keepdims=True)
                        for t in range(0, M, 128)], 0)
            col = jnp.broadcast_to(col, (M, 128))

            def job(t):
                def run(dep):
                    w = _after(always, w_s[:, t:t + 128], [jnp.tile(dep[:16], (M // 16, 1))])
                    outs.append(_rb(jnp.sum(col * w.astype(F32), axis=0, keepdims=True)))
                    return jnp.broadcast_to(outs[-1], (8, 128))
                return run
            return [job(t) for t in range(0, w_s.shape[1], 128)]

        chunks = CFG["chunks"]
        cstart = [sum(chunks[:i]) for i in range(len(chunks))]
        cp_ckv = [pltpu.make_async_copy(ckv_hbm.at[0, r0:r0 + nr], ckv_s.at[r0:r0 + nr], sems.at[6 + i])
                  for i, (r0, nr) in enumerate(zip(cstart, chunks))]
        start(kv_copies(0, 1) + cp_ckv + kv_copies(1, 4) + [cp_c, cp_wr, cp_ma])
        for i, (r0, nr) in enumerate(zip(cstart, chunks)):
            wait(cp_ckv[i:i + 1] + (kv_copies(0, 1) if i == 0 else []))
            ct, cb = _split_rows(ckv_s[r0:r0 + nr, :].astype(F32))
            ca = ((ct[:, :Dc // 2], ct[:, Dc // 2:]), (cb[:, :Dc // 2], cb[:, Dc // 2:]))
            for j in _ORDER:
                cl_s[j, r0 // 2:(r0 + nr) // 2, :] = _LHS[j](ca).astype(BF16)
            kv_proj(0, _Side(None), r0, nr)
        wait(kv_copies(1, 4) + [cp_c, cp_wr, cp_ma])
        start([cp_x] + kv_copies(4, NP))
        wr = wr_s[...].astype(F32).reshape(1, M)
        always = jnp.broadcast_to(pltpu.bitcast(wr[:, :128], I32) | 1, (8, 128)) != 0
        side, moda = _Side(always), []
        side.spread(modulation(wma_s, always, moda), 5 if CFG["skip_kv"] else 18)
        for p in range(1, 2 if CFG["skip_kv"] else 4):
            kv_proj(p, side)
        sa, ca1 = _cat(moda[:5], 1), _rb(1.0 + _cat(moda[5:], 1))
        wait([cp_x] + kv_copies(4, NP))
        start([wcopy(0, p) for p in range(NP)] + [cp_wo] + late)

        def kv_step(i, carry):
            always = lax.broadcasted_iota(I32, (8, 128), 0) < i + 8
            g = CFG["ln1g"]
            rows = S // 4

            def ln1(r):
                def run(dep):
                    r0 = pl.multiple_of(i * rows + r, g)
                    xv = _cat([_after(always, x_s[pl.ds(r0, g), t:t + 128], [dep[:g]])
                               for t in range(0, M, 128)], 1).astype(F32)
                    mu = jnp.sum(xv, axis=-1, keepdims=True) * (1.0 / M)
                    xc = xv - mu
                    var = jnp.sum(xc * xc, axis=-1, keepdims=True) * (1.0 / M)
                    ht, hb = _split_rows(xc * lax.rsqrt(var + 1e-5) * ca1 + sa)
                    ha = ((ht[:, :256], ht[:, 256:512]), (hb[:, :256], hb[:, 256:512]))
                    rh = pl.ds(pl.multiple_of(i * (rows // 2) + r // 2, g // 2), g // 2)
                    for j in range(7):
                        hl_s[j, rh, :] = _LHS[j](ha).astype(BF16)
                    hl_s[7, rh, :] = _cat([ht[:, 512:], hb[:, 512:]], 1).astype(BF16)
                return run

            side = _Side(always)
            side.spread([ln1(r) for r in range(0, rows, g)], 20)
            for u in range(3):
                kv_proj(4 + 3 * i + u, side)
            return carry

        with _scope('kvloop'):
            lax.fori_loop(0, 4, kv_step, 0)
        wait([wcopy(0, p) for p in range(NP)] + [cp_wo])

        def o_operands(p, always=None, dep=None):
            wa, wb = wo_s[2 * p, :, :512].astype(F32), wo_s[2 * p + 1, :, :512].astype(F32)
            if dep is not None:
                wa, wb = (_cat([_after(always, w[:, t:t + 128], [dep]) for t in range(0, 512, 128)], 1) for w in (wa, wb))
            bo = ((wa[:, :256], wa[:, 256:]), (wb[:, :256], wb[:, 256:]))
            for i in range(7):
                wor_s[i, p] = _RHS[i](bo).astype(BF16)

        if "W" not in CFG["order"].split():
            for p in range(NP):
                o_operands(p)

        def pair(p, carry):
            always = lax.broadcasted_iota(I32, (8, 128), 0) < p + 8
            dist = lax.broadcasted_iota(I32, (G, 128), 1) - lax.broadcasted_iota(I32, (G, 128), 0)
            st, clock, pend = {}, [0], []

            def proj_q(e):
                bq = blocks_of(wq_b[p, :512, :])
                if e == 0:
                    wt = _cat(_halves(wq_b[p, 512:, :]), 1).astype(BF16)
                    st["qt"] = [_dot(hl_s[7, :, :128], wt), _dot(hl_s[7, :, 128:], wt)]
                    st["qm"] = [None] * 7
                    for i in _ORDER[:-1]:
                        st["qm"][i] = _dot(hl_s[i], _RHS[i](bq).astype(BF16))
                    m = st["qm"]
                    top, bot = (m[3] - m[4]) + m[0] + m[6], m[1] + m[3]
                else:
                    m = st["qm"]
                    w = _RHS[5](bq).astype(BF16)
                    m[5] = _cat([_dot(hl_s[5, :S // 4, :], w), _dot(hl_s[5, S // 4:, :], w)], 0)
                    top, bot = m[2] + m[4], (m[2] - m[1]) + m[0] + m[5]
                o = _merge_rows(top + st["qt"][0][:, D * e:D * (e + 1)], bot + st["qt"][1][:, D * e:D * (e + 1)])
                q_s[e] = (o * qscale).astype(BF16)
                clock[0] += 512

            def acc(key, r0, val, op):
                for u in range(val.shape[0] // G):
                    k = (key, r0 // G + u)
                    part = val[G * u:G * (u + 1)]
                    st[k] = op(st[k], part) if k in st else part

            def get(key, r0, nr):
                return _cat([st[(key, u)] for u in range(r0 // G, (r0 + nr) // G)], 0)

            last = [None]

            def take(val, kinds, extra=()):
                ready = [z for z in pend if z[0] <= clock[0] and z[1].shape[0] == val.shape[0] and z[2] in kinds]
                pend[:] = [z for z in pend if not any(z is y for y in ready)]
                deps = [z[1] for z in ready] + list(extra)
                return _after(always, val, deps) if deps else val

            fins = []

            def run_fin(dep, kind):
                if not fins or (dep is not None and kind not in CFG["fin_in"]):
                    return
                e, r0 = fins.pop(0)
                l = get(("l", e), r0, ur)
                if dep is not None and CFG["fin_dep"]:
                    l = _after(always, l, [dep])
                l = jnp.sum(l, axis=-1, keepdims=True)
                r = pl.reciprocal(l, approx=True)
                ctx = get(("o", e), r0, ur) * (r * (2.0 - l * r))
                ctx_s[2 * p + e, r0:r0 + ur, :] = ctx.astype(BF16)
                pend.append((clock[0] + CFG["df"], ctx, "f"))

            def qk(e, a, j):
                us = units(a)
                for (r0, nr, c0, nc) in us[j]:
                    q = take(q_s[e, r0:r0 + nr, :], CFG["qk_takes"])
                    s = _dot_nt(q, k_s[2 * p + e, c0:c0 + nc, :])
                    tiles = []
                    for t in range(nc // 128):
                        x = s[:, 128 * t:128 * (t + 1)]
                        if c0 + 128 * (t + 1) > r0:
                            x = _cat([x[g:g + G] if c0 + 128 * (t + 1) <= r0 + g else
                                      jnp.where(dist <= r0 + g - c0 - 128 * t, x[g:g + G], neg)
                                      for g in range(0, nr, G)], 0)
                        tiles.append(x)
                    mm = tiles[0]
                    for t in tiles[1:]:
                        mm = jnp.maximum(mm, t)
                    acc(("m", e), r0, mm, jnp.maximum)
                    st[("s", e, r0, c0)] = tiles
                clock[0] += us[j][0][1]
                if nr == ur:
                    run_fin(mm, "a")
                    last[0] = mm
                if j == len(us) - 1:
                    for u in range(a * SB // G, (a + 1) * SB // G):
                        k = (("m", e), u)
                        st[k] = jnp.broadcast_to(jnp.max(st[k], axis=-1, keepdims=True), (G, 128))
                    if "M" in CFG["qk_takes"] + CFG["pv_takes"]:
                        for r0 in range(a * SB, (a + 1) * SB, ur):
                            pend.append((clock[0] + CFG["dM"] + (r0 - a * SB), get(("m", e), r0, ur), "M"))

            def pv(e, a, j):
                us = units(a, 'b')
                for (r0, nr, c0, nc) in us[j]:
                    m = take(get(("m", e), r0, nr), CFG["pv_takes"], [last[0][:nr]])
                    ps = [jnp.exp2(x - m) for x in st.pop(("s", e, r0, c0))]
                    ll = ps[0]
                    for t in ps[1:]:
                        ll = ll + t
                    acc(("l", e), r0, ll, jnp.add)
                    if CFG["tl"]:
                        ps[-1] = _after(always, ps[-1], [get(("l", e), r0, nr)])
                    acc(("o", e), r0, _dot(_cat(ps, 1).astype(BF16), v_s[2 * p + e, c0:c0 + nc, :]), jnp.add)
                clock[0] += us[j][0][1]
                if len(us[j]) == 1:
                    run_fin(get(("o", e), r0, nr), "b")
                if nr == ur:
                    last[0] = get(("o", e), r0, nr)
                if j == len(us) - 1:
                    for r0 in range(a * SB, (a + 1) * SB, ur):
                        fins.append((e, r0))

            for tok in CFG["order"].split():
                if tok == "W":
                    o_operands(p, always, st["qm"][2][:D])
                elif tok[0] == "Q":
                    proj_q("AB".index(tok[1]))
                elif tok[0] in "ab":
                    for j in range(len(units(int(tok[1])))):
                        (qk if tok[0] == "a" else pv)("AB".index(tok[2]), int(tok[1]), j)
                elif tok[0] == "x":
                    qa, qe, pa, pe = int(tok[1]), "AB".index(tok[2]), int(tok[3]), "AB".index(tok[4])
                    nq, npv = len(units(qa)), len(units(pa))
                    seq = sorted([((j + 0.5) / nq, 0, j) for j in range(nq)] + [((j + 1.0) / npv, 1, j) for j in range(npv)])
                    for _, kind, j in seq:
                        (pv(pe, pa, j) if kind else qk(qe, qa, j))
            while fins:
                run_fin(None, None)
            return carry

        with _scope('attn'):
            lax.fori_loop(0, NP, pair, 0)

        wait(late)
        lane = lax.broadcasted_iota(I32, (8, 128), 1)
        sub = lax.broadcasted_iota(I32, (8, 128), 0)
        nk = S // 1024
        rk = [jnp.zeros((8, 128), F32) for _ in range(nk)]

        side = _Side(always)

        def o_proj(r0, nr):
            m = [None] * 7
            for p0 in range(0, NP, 2):
                for i in _ORDER:
                    lhs = []
                    for pp in (p0, p0 + 1):
                        a0, a1 = (_split_rows(ctx_s[2 * pp + e, r0:r0 + nr, :].astype(F32)) for e in range(2))
                        lhs.append(_LHS[i](((a0[0], a1[0]), (a0[1], a1[1]))))
                    d = _dot(side.lhs(_cat(lhs, 1)).astype(BF16), _cat([wor_s[i, p0], wor_s[i, p0 + 1]], 0))
                    m[i] = d if m[i] is None else m[i] + d
                    side.result(m[i])
            tail = None
            for h0 in range(0, H, 4):
                d = _dot(side.lhs(_cat([ctx_s[hh, r0:r0 + nr, :] for hh in range(h0, h0 + 4)], 1)),
                         _cat([wo_s[hh, :, 512:] for hh in range(h0, h0 + 4)], 0))
                tail = d if tail is None else tail + d
                side.result(tail)
            cc = _combine(m)
            o = _cat([_merge_rows(cc[0][e], cc[1][e]) for e in range(2)], 1)
            return [o[:, n:n + 128] for n in range(0, 512, 128)] + [tail]

        def ln2(r0, cols):
            nr = cols[0].shape[0]
            a = _rb(_cat(cols, 1))
            x1 = _rb(x_s[r0:r0 + nr, :].astype(F32) + _rb(ga * a))
            x_s[r0:r0 + nr, :] = x1.astype(BF16)
            mu = jnp.sum(x1, axis=-1, keepdims=True) / M
            xc = x1 - mu
            var = _rb(jnp.sum(xc * xc, axis=-1, keepdims=True) / M)
            inv = 1.0 / _rb(jnp.sqrt(_rb(var + eps_b)))
            h2 = _rb(_rb(_rb(_rb(x1 - _rb(mu)) * inv) * cb1) + sb)
            h_s[r0:r0 + nr, :] = h2.astype(BF16)
            out_s[r0:r0 + nr, :] = (x1 + _rb(gb * h2)).astype(BF16)
            r = jnp.sum(h2 * wr, axis=-1, keepdims=True)
            for j in range(nr // 8):
                g = r0 // 8 + j
                rk[g // 128] = jnp.where(lane == g % 128, r[8 * j:8 * j + 8], rk[g // 128])

        eblocks = CFG["eblocks"][:2] if CFG["skip_epi"] else CFG["eblocks"]
        starts = [sum(eblocks[:i]) for i in range(len(eblocks))]
        out_cps = [pltpu.make_async_copy(out_s.at[r0:r0 + nr], out_hbm.at[0, r0:r0 + nr], sems.at[4])
                   for i, (r0, nr) in enumerate(zip(starts, eblocks))]

        def transpose_job(w_s, dst, f0):
            def run(dep):
                wt = _cat([_after(always, w_s[f0:f0 + 128, t:t + 128], [dep[:128]]) for t in range(0, M, 128)], 1)
                dst[f0 // 128, :M, :] = wt.astype(F32).T.astype(BF16)
            return run

        def ln2_job(r0, part):
            return lambda dep: ln2(r0, [_after(always, pt, [dep[:pt.shape[0]]]) for pt in part])

        modb = []
        side.spread(modulation(wmb_s, always, modb), 60)
        side.spread([transpose_job(w_s, dst, f0) for w_s, dst in ((wg_s, k_s), (wu_s, v_s))
                     for f0 in range(0, FA, 128)], 60)
        for i, (r0, nr) in enumerate(zip(starts, eblocks)):
            cols = o_proj(r0, nr)
            if i == 0:
                ga, sb, cb1, gb = (_cat(modb[t:t + 5], 1) for t in range(0, 20, 5))
                cb1 = _rb(1.0 + cb1)
            else:
                out_cps[i - 1].start()
            g = CFG["ln2g"]
            if i + 1 < len(eblocks):
                side.spread([ln2_job(r0 + r, [cl[r:r + g] for cl in cols]) for r in range(0, nr, g)], CFG["ln2span"])
            else:
                ln2(r0, cols)
                out_cps[i].start()

        keys = []
        for t in range(nk):
            rv = _rb(rk[t])
            b = lax.shift_right_logical(pltpu.bitcast(jnp.where(rv == 0.0, 0.0, rv), I32), 16)
            o16 = jnp.where(b >= 0x8000, 0xFFFF - b, b + 0x8000)
            o16 = jnp.where(rv != rv, 0, o16)
            tok = t * 1024 + lane * 8 + sub
            keys.append(pltpu.bitcast((o16 << 11) + (S - 1 - tok) + (1 << 29), F32))
        sel = []
        for _ in range(TOPC):
            mk = keys[0]
            for t in range(1, nk):
                mk = jnp.maximum(mk, keys[t])
            top = jnp.max(jnp.max(mk, axis=1, keepdims=True), axis=0, keepdims=True)
            keys = [jnp.where(kk == top, 0.0, kk) for kk in keys]
            sel.append(top)
        row8 = lax.broadcasted_iota(I32, (8, 1), 0)
        kcol = jnp.zeros((8, 1), F32)
        for ci in range(TOPC):
            kcol = jnp.where(row8 == ci, sel[ci], kcol)
        o16 = (pltpu.bitcast(kcol, I32) - (1 << 29)) >> 11
        rsel = pltpu.bitcast(jnp.where(o16 >= 0x8000, o16 - 0x8000, 0xFFFF - o16) << 16, F32)
        toks = [S - 1 - (pltpu.bitcast(sel[ci], I32)[0, 0] & (S - 1)) for ci in range(TOPC)]
        grps = [pl.multiple_of(tk & (S - 16), 16) for tk in toks]

        row16 = lax.broadcasted_iota(I32, (16, M), 0)
        rowc = lax.broadcasted_iota(I32, (8, M), 0)
        xs = jnp.zeros((8, M), F32)
        x1s = jnp.zeros((8, M), F32)
        for ci in range(TOPC):
            msk = row16 == (toks[ci] & 15)
            hv = jnp.sum(jnp.where(msk, h_s[pl.ds(grps[ci], 16), :].astype(F32), 0.0), axis=0, keepdims=True)
            xv = jnp.sum(jnp.where(msk, x_s[pl.ds(grps[ci], 16), :].astype(F32), 0.0), axis=0, keepdims=True)
            xs = jnp.where(rowc == ci, hv, xs)
            x1s = jnp.where(rowc == ci, xv, x1s)

        xsb = xs.astype(BF16)
        gp = _rb(_cat([_dot(xsb, _cat([k_s[j, :M, :] for j in range(FA // 128)], 1)), _dot_nt(xsb, wg_s[FA:, :])], 1))
        g = _rb(gp * _rb(_sigmoid(gp)))
        u = _rb(_cat([_dot(xsb, _cat([v_s[j, :M, :] for j in range(FA // 128)], 1)), _dot_nt(xsb, wu_s[FA:, :])], 1))
        y = _rb(_dot((g * u).astype(BF16), wd_s[...]))
        y = _rb(y * _rb(_sigmoid(rsel)))
        onew = x1s + _rb(gb * _rb(xs + y))

        wait(out_cps)
        for ci in range(TOPC):
            msk = row16 == (toks[ci] & 15)
            old = out_s[pl.ds(grps[ci], 16), :].astype(F32)
            out_s[pl.ds(grps[ci], 16), :] = jnp.where(msk, onew[ci:ci + 1], old).astype(BF16)
        fresh = []
        for ci in range(TOPC):
            f = grps[ci] >= 0
            for cj in range(ci):
                f = jnp.logical_and(f, grps[cj] != grps[ci])
            fresh.append(f)
        patch = [pltpu.make_async_copy(out_s.at[pl.ds(grps[ci], 16)], out_hbm.at[0, pl.ds(grps[ci], 16)],
                                       sems.at[5]) for ci in range(TOPC)]
        for ci in range(TOPC):
            pl.when(fresh[ci])(patch[ci].start)
        for ci in range(TOPC):
            pl.when(fresh[ci])(patch[ci].wait)

    return kernel


@jax.jit
def pallas_adaLN_cond__compressed_kv_cla__moe_arch_mod__prompt_kernel(
    A_x, A_c_kv, A_w_q, A_w_uk, A_w_uv, A_w_o, B_x, B_w_r, B_w_gate, B_w_up, B_w_down, c, w_mod,
):
    del B_x
    _, S, M = A_x.shape
    Dc = A_c_kv.shape[2]
    H, D = A_w_q.shape[1:]
    F = B_w_gate.shape[1]
    any_spec = pl.BlockSpec(memory_space=pl.ANY)
    vmem_spec = pl.BlockSpec(memory_space=pltpu.VMEM)
    return pl.pallas_call(
        _make_kernel(S, M, Dc, H, D, F),
        out_shape=jax.ShapeDtypeStruct(A_x.shape, A_x.dtype),
        in_specs=[any_spec] * 12,
        out_specs=any_spec,
        scratch_shapes=[
            pltpu.VMEM((S, M), BF16),
            pltpu.VMEM((S, Dc), BF16),
            pltpu.VMEM((S, M), BF16),
            pltpu.VMEM((H // 2, M, D), U32),
            pltpu.VMEM((H // 2, Dc, D), U32),
            pltpu.VMEM((H // 2, Dc, D), U32),
            pltpu.VMEM((H, D, M), BF16),
            pltpu.VMEM((F, M), BF16),
            pltpu.VMEM((F, M), BF16),
            pltpu.VMEM((F, M), BF16),
            pltpu.VMEM((M, 2 * M), BF16),
            pltpu.VMEM((M, 4 * M), BF16),
            pltpu.VMEM((2, S, D), BF16),
            pltpu.VMEM((H, S, D), BF16),
            pltpu.VMEM((H, S, D), BF16),
            pltpu.VMEM((H, S, D), BF16),
            pltpu.VMEM((S, M), BF16),
            pltpu.VMEM((7, S // 2, Dc // 2), BF16),
            pltpu.VMEM((8, S // 2, 256), BF16),
            pltpu.VMEM((7, H // 2, D, 256), BF16),
            pltpu.VMEM((1, M), BF16),
            pltpu.VMEM((M,), BF16),
            pltpu.SemaphoreType.DMA((6 + len(CFG['chunks']),)),
        ],
        compiler_params=pltpu.CompilerParams(vmem_limit_bytes=124 * 1024 * 1024, flags=CFG["flags"]),
        name="adaln_mla_mod",
    )(A_x, A_c_kv, A_w_q, A_w_uk, A_w_uv, A_w_o, B_w_r, B_w_gate.T, B_w_up.T, B_w_down, c, w_mod)
```

```python
import contextlib

import numpy as np
import jax
import jax.numpy as jnp
from jax import lax
import jax.experimental.pallas as pl
import jax.experimental.pallas.tpu as pltpu

CFG = dict(flags=None, skip_epi=False, chunks=(512, 512, 1024), lag=2, lag1=2, g0at=1, c1=2, lnat=2,
           dposa=(-2, 0.5), dposb=(0.5, 1.5), df=256, dM=256,
           eblocks=(512, 512, 384, 256, 192, 128, 64), ln2g=8, ln2span=60, ln1g=32,
           order='QA W a0A QB a1A b0A a2A b1A a3A b2A a0B b3A a1B b0B a2B b1B a3B b2B b3B')

F32 = jnp.float32
BF16 = jnp.bfloat16
U32 = jnp.uint32
I32 = jnp.int32
TOPC = 8
LOG2E = 1.4426950408889634
EPS = 1e-5
RG = 16
G = 64
UR = 256
SB = 512
HG = 8


def _scope(name):
    return jax.named_scope(name) if CFG.get('scopes') else contextlib.nullcontext()


def _rb(a):
    return a.astype(BF16).astype(F32)


def _dot(a, b):
    return jnp.dot(a, b, preferred_element_type=F32)


def _dot_nt(a, b):
    return lax.dot_general(a, b, (((1,), (1,)), ((), ())), preferred_element_type=F32)


def _sigmoid(a):
    return 1.0 / (1.0 + jnp.exp(-a))


def _cat(xs, axis):
    return jnp.concatenate(xs, axis=axis) if len(xs) > 1 else xs[0]


def _fold(op, xs):
    acc = xs[0]
    for x in xs[1:]:
        acc = op(acc, x)
    return acc


def _words(w):
    return pltpu.bitcast(w.reshape(w.shape[0] * w.shape[1], w.shape[2]), U32)


def _halves(u):
    return pltpu.bitcast(u << 16, F32), pltpu.bitcast(u & np.uint32(0xFFFF0000), F32)


def _after(always, val, deps):
    t = _fold(jnp.maximum, deps)
    if val.dtype == BF16:
        t = pltpu.bitcast(t.astype(BF16), I32)
        out = jnp.where(jnp.tile(always, (t.shape[0] // 8, 1)), pltpu.bitcast(val, I32), t)
        return pltpu.bitcast(out, BF16)
    if val.dtype != F32:
        t = pltpu.bitcast(t, val.dtype)
    return jnp.where(jnp.tile(always, (t.shape[0] // 8, 1)), val, t)


class _Side:
    def __init__(self, always=None, lag=1, stagger=0):
        self.stagger = stagger
        self.always, self.lag, self.jobs, self.done, self.n = always, lag, {}, {}, 0

    def spread(self, jobs, span):
        for t, job in enumerate(jobs):
            self.jobs.setdefault(self.n + t * span // len(jobs), []).append(job)

    def lhs(self, x):
        toks = self.done.pop(self.n, None)
        if not toks:
            return x
        rows = 8 if x.dtype == F32 else 16
        head = _after(self.always, x[:rows, :128], [jnp.tile(t, (rows // 8, 1)) for t in toks])
        return _cat([_cat([head, x[rows:, :128]], 0), x[:, 128:]], 1)

    def result(self, d):
        jobs = self.jobs.pop(self.n, ())
        for t, job in enumerate(jobs):
            tok = job(d[self.stagger * t // len(jobs) // 8 * 8:, :128])
            if tok is not None:
                self.done.setdefault(self.n + self.lag, []).append(tok)
        self.n += 1


def _split_rows(x):
    n = x.shape[0] // (2 * RG)
    y = x.reshape(n, 2, RG, x.shape[1])
    return y[:, 0].reshape(n * RG, x.shape[1]), y[:, 1].reshape(n * RG, x.shape[1])


def _merge_rows(top, bot):
    n = top.shape[0] // RG
    y = jnp.concatenate([top.reshape(n, 1, RG, top.shape[1]), bot.reshape(n, 1, RG, top.shape[1])], axis=1)
    return y.reshape(2 * n * RG, top.shape[1])


_LHS = (lambda a: a[0][0] + a[1][1], lambda a: a[1][0] + a[1][1], lambda a: a[0][0], lambda a: a[1][1],
        lambda a: a[0][0] + a[0][1], lambda a: a[1][0] - a[0][0], lambda a: a[0][1] - a[1][1])
_RHS = (lambda b: b[0][0] + b[1][1], lambda b: b[0][0], lambda b: b[0][1] - b[1][1],
        lambda b: b[1][0] - b[0][0], lambda b: b[1][1], lambda b: b[0][0] + b[0][1],
        lambda b: b[1][0] + b[1][1])
_ORDER = (2, 4, 3, 1, 0, 6, 5)


def _column(m, e):
    if e == 0:
        return (m[3] - m[4]) + m[0] + m[6], m[1] + m[3]
    return m[2] + m[4], (m[2] - m[1]) + m[0] + m[5]


def _row_blocks(x):
    top, bot = _split_rows(x)
    hk = x.shape[1] // 2
    return (top[:, :hk], top[:, hk:]), (bot[:, :hk], bot[:, hk:])


def _pair_blocks(u):
    w = _halves(u)
    hk = u.shape[0] // 2
    return (w[0][:hk], w[1][:hk]), (w[0][hk:], w[1][hk:])


def _units(a, kind):
    r0 = a * SB
    full = [[(r0 + ro, UR, c0, SB)] for c0 in range(0, r0, SB) for ro in range(0, SB, UR)]
    big = [(r0, 256, r0, 128), (r0 + 256, 256, r0, 384)]
    small = [(r0 + 128, 64, r0 + 128, 128), (r0 + 192, 64, r0 + 128, 128),
             (r0 + 384, 64, r0 + 384, 128), (r0 + 448, 64, r0 + 384, 128)]
    kb, ks = CFG["dpos" + kind]
    return [u for _, u in sorted(list(enumerate(full)) + [(kb, big), (ks, small)], key=lambda z: z[0])]


def _start(cps):
    for cp in cps:
        cp.start()


def _make_kernel(S, M, Dc, H, D, F):
    NP, NG, PG = H // 2, H // HG, HG // 2
    FA = F // 128 * 128
    eps_b = float(np.asarray(EPS, dtype=BF16).astype(np.float32))
    qscale = float(np.asarray(D ** -0.5, dtype=BF16).astype(np.float32)) * LOG2E
    masked = -1e9 * LOG2E
    nwait = [0]

    def _wait(cps):
        nwait[0] += 1
        with _scope(f"wait{nwait[0]}"):
            for cp in cps:
                cp.wait()

    def kernel(x_hbm, ckv_hbm, wq_hbm, wuk_hbm, wuv_hbm, wo_hbm, wr_hbm, wg_hbm, wu_hbm,
               wd_hbm, c_hbm, wmod_hbm, out_hbm,
               x_s, wq_u, wo_s, wg_s, wu_s, wd_s, wmb_s, k_s, v_s, hl_s, c_s, wr_s, sems, qsems, csems):
        cp_wo = [pltpu.make_async_copy(wo_hbm, wo_s, sems.at[0])]
        cp_late = [pltpu.make_async_copy(wmod_hbm.at[:, 2 * M:6 * M], wmb_s, sems.at[1]),
                   pltpu.make_async_copy(wg_hbm, wg_s, sems.at[1]),
                   pltpu.make_async_copy(wu_hbm, wu_s, sems.at[1]),
                   pltpu.make_async_copy(wd_hbm, wd_s, sems.at[1])]

        def pair_words(ref, g, j):
            return ref[g, pl.ds(j, ref.shape[1] // PG, stride=PG), :]

        def all_true(x):
            return (pltpu.bitcast(x, I32) | 1) != 0

        def modulation(w_s, always, outs):
            cv = c_s[...].astype(F32)
            sc = _rb(cv * _rb(_sigmoid(cv)))
            eye = lax.broadcasted_iota(I32, (128, 128), 0) == lax.broadcasted_iota(I32, (128, 128), 1)
            col = _cat([jnp.sum(jnp.where(eye, sc[:, t:t + 128], 0.0), axis=1, keepdims=True)
                        for t in range(0, M, 128)], 0)
            col = jnp.broadcast_to(col, (M, 128))

            def job(t):
                def run(dep):
                    w = _after(always, w_s[:, t:t + 128], [jnp.tile(dep[:16], (M // 16, 1))])
                    outs.append(_rb(jnp.sum(col * w.astype(F32), axis=0, keepdims=True)))
                    return jnp.broadcast_to(outs[-1], (8, 128))
                return run
            return [job(t) for t in range(0, w_s.shape[1], 128)]

        def phase1(ckv_s, cl_s, w0_s, w0_u, wk_g, wv_g, wq_g, wk_u, wv_u, wma_s):
            chunks = CFG["chunks"]
            cstart = [sum(chunks[:i]) for i in range(len(chunks))]
            cp_w0 = [pltpu.make_async_copy(w.at[:, 0:2, :], w0_s.at[i], sems.at[2])
                     for i, w in enumerate((wuk_hbm, wuv_hbm))]
            cp_ckv = [pltpu.make_async_copy(ckv_hbm.at[0, r0:r0 + nr], ckv_s.at[r0:r0 + nr], csems.at[i])
                      for i, (r0, nr) in enumerate(zip(cstart, chunks))]
            cp_kv = [[pltpu.make_async_copy(w.at[:, HG * g:HG * (g + 1), :], dst.at[g], sems.at[3 if g == 0 else 4])
                      for w, dst in ((wuk_hbm, wk_g), (wuv_hbm, wv_g))] for g in range(NG)]
            cp_kv_rest = [cp for cps in cp_kv[1:] for cp in cps]
            cp_ln = [pltpu.make_async_copy(c_hbm, c_s, sems.at[5]),
                     pltpu.make_async_copy(wr_hbm, wr_s, sems.at[5]),
                     pltpu.make_async_copy(wmod_hbm.at[:, 0:2 * M], wma_s, sems.at[5])]

            def cp_step(g):
                rows = pl.ds(pl.multiple_of(S // NG * g, S // NG), S // NG)
                return [pltpu.make_async_copy(wq_hbm.at[:, pl.ds(pl.multiple_of(HG * g, HG), HG), :],
                                              wq_g.at[g], qsems.at[g]),
                        pltpu.make_async_copy(x_hbm.at[0, rows], x_s.at[rows], qsems.at[g])]

            def repack(always, src, dst, g, step=64):
                def job(r):
                    def run(dep):
                        u = _after(always, _words(src[g, r:r + step]), [jnp.tile(dep[:8], (PG * step // 8, 1))])
                        dst[g, PG * r:PG * (r + step), :] = u
                        return pltpu.bitcast(_fold(jnp.bitwise_and, [u[t:t + 8] for t in range(0, PG * step, 8)]), F32)
                    return run
                return [job(r) for r in range(0, src.shape[1], step)]

            def kv_proj(p, uk, uv, side, r0=0, nr=S):
                bk, bv = _pair_blocks(uk), _pair_blocks(uv)
                m = [None] * 7
                for i in _ORDER:
                    m[i] = _dot(side.lhs(cl_s[i, r0 // 2:(r0 + nr) // 2, :]),
                                _cat([_RHS[i](bk), _RHS[i](bv)], 1).astype(BF16))
                    side.result(m[i])
                for e in range(2):
                    o = _merge_rows(*_column(m, e))
                    k_s[2 * p + e, r0:r0 + nr, :] = o[:, :D].astype(BF16)
                    v_s[2 * p + e, r0:r0 + nr, :] = o[:, D:].astype(BF16)

            def kv_pair(p, side):
                kv_proj(p, pair_words(wk_u, p // PG, p % PG), pair_words(wv_u, p // PG, p % PG), side)

            _start(cp_w0 + cp_ckv[:1])
            _wait(cp_w0)
            _start(cp_ckv[1:])
            for i in range(2):
                for r in range(Dc):
                    w0_u[i, r:r + 1, :] = pltpu.bitcast(w0_s[i, r], U32)
            for i, (r0, nr) in enumerate(zip(cstart, chunks)):
                _wait(cp_ckv[i:i + 1])
                if i == 0:
                    _start(cp_kv[0])
                blocks = _row_blocks(ckv_s[r0:r0 + nr, :].astype(F32))
                for j in _ORDER:
                    cl_s[j, r0 // 2:(r0 + nr) // 2, :] = _LHS[j](blocks).astype(BF16)
                kv_proj(0, w0_u[0], w0_u[1], _Side(), r0, nr)
            _wait(cp_kv[0])
            _start(cp_kv_rest + cp_ln + cp_step(0))
            wk_u[0] = _words(wk_g[0])
            wv_u[0] = _words(wv_g[0])
            for p in range(1, PG - 1):
                kv_pair(p, _Side())
            _wait(cp_kv_rest)
            side = _Side(all_true(w0_u[0, :8, :]), CFG["lag1"], S // 2 - 64)
            side.spread([job for g in range(1, NG) for src, dst in ((wk_g, wk_u), (wv_g, wv_u))
                         for job in repack(side.always, src, dst, g)], 6)
            kv_pair(PG - 1, side)
            _wait(cp_ln)
            _start([cp for g in range(1, NG) for cp in cp_step(g)] + cp_wo)

            def step(i, carry):
                for cp in cp_step(i):
                    cp.wait()
                always = lax.broadcasted_iota(I32, (8, 128), 0) < i + 8
                g, rows, mod = CFG["ln1g"], S // NG, []

                def ln1(r):
                    def run(dep):
                        r0 = pl.multiple_of(i * rows + r, g)
                        xv = _cat([_after(always, x_s[pl.ds(r0, g), t:t + 128], [dep[:g]])
                                   for t in range(0, M, 128)], 1).astype(F32)
                        mu = jnp.sum(xv, axis=-1, keepdims=True) * (1.0 / M)
                        xc = xv - mu
                        var = jnp.sum(xc * xc, axis=-1, keepdims=True) * (1.0 / M)
                        sa, ca = _cat(mod[:M // 128], 1), _cat(mod[M // 128:], 1)
                        h = xc * lax.rsqrt(var + EPS) * _rb(1.0 + ca) + sa
                        blocks = _row_blocks(h[:, :512])
                        rh = pl.ds(pl.multiple_of(i * (rows // 2) + r // 2, g // 2), g // 2)
                        for j in range(7):
                            hl_s[j, rh, :] = _LHS[j](blocks).astype(BF16)
                        hl_s[7, rh, :] = _cat(_split_rows(h[:, 512:]), 1).astype(BF16)
                    return run

                side = _Side(always, CFG["lag1"], S // 2 - 64)
                side.spread(modulation(wma_s, always, mod) + [ln1(r) for r in range(0, rows, g)], 20)
                side.spread(repack(always, wq_g, wq_u, i), 20)
                for u in range(PG - 1):
                    kv_pair(PG + (PG - 1) * i + u, side)
                return carry

            with _scope('kvloop'):
                lax.fori_loop(0, NG, step, 0)

        pl.run_scoped(
            phase1,
            pltpu.VMEM((S, Dc), BF16), pltpu.VMEM((7, S // 2, Dc // 2), BF16),
            pltpu.VMEM((2, Dc, 2, D), BF16), pltpu.VMEM((2, Dc, D), U32),
            pltpu.VMEM((NG, Dc, HG, D), BF16), pltpu.VMEM((NG, Dc, HG, D), BF16), pltpu.VMEM((NG, M, HG, D), BF16),
            pltpu.VMEM((NG, PG * Dc, D), U32), pltpu.VMEM((NG, PG * Dc, D), U32), pltpu.VMEM((M, 2 * M), BF16))

        def attend_pair(p, q_s, ctx_s, wor_s):
            always = lax.broadcasted_iota(I32, (8, 128), 0) < p + 8
            dist = lax.broadcasted_iota(I32, (G, 128), 1) - lax.broadcasted_iota(I32, (G, 128), 0)
            st, clock, pend, fins, last = {}, [0], [], [], [None]

            def proj_q(e):
                u = pair_words(wq_u, p // PG, p % PG)
                bq = _pair_blocks(u[:512])
                if e == 0:
                    wt = _cat(_halves(u[512:]), 1).astype(BF16)
                    st["qt"] = [_dot(hl_s[7, :, :128], wt), _dot(hl_s[7, :, 128:], wt)]
                    st["qm"] = [None] * 7
                    for i in _ORDER[:-1]:
                        st["qm"][i] = _dot(hl_s[i], _RHS[i](bq).astype(BF16))
                else:
                    w = _RHS[5](bq).astype(BF16)
                    st["qm"][5] = _cat([_dot(hl_s[5, :S // 4, :], w), _dot(hl_s[5, S // 4:, :], w)], 0)
                top, bot = _column(st["qm"], e)
                o = _merge_rows(top + st["qt"][0][:, D * e:D * (e + 1)], bot + st["qt"][1][:, D * e:D * (e + 1)])
                q_s[e] = (o * qscale).astype(BF16)
                clock[0] += 512

            def o_operands():
                dep = st["qm"][2][:D]
                wa, wb = (_cat([_after(always, wo_s[2 * p + e, :, t:t + 128], [dep]) for t in range(0, 512, 128)],
                               1).astype(F32) for e in range(2))
                for i in range(7):
                    wor_s[i, p] = _RHS[i](((wa[:, :256], wa[:, 256:]), (wb[:, :256], wb[:, 256:]))).astype(BF16)

            def acc(key, r0, val, op):
                for u in range(val.shape[0] // G):
                    k = (key, r0 // G + u)
                    part = val[G * u:G * (u + 1)]
                    st[k] = op(st[k], part) if k in st else part

            def get(key, r0, nr):
                return _cat([st[(key, u)] for u in range(r0 // G, (r0 + nr) // G)], 0)

            def take(val, kinds, extra=()):
                ready = [z for z in pend if z[0] <= clock[0] and z[1].shape[0] == val.shape[0] and z[2] in kinds]
                pend[:] = [z for z in pend if not any(z is y for y in ready)]
                deps = [z[1] for z in ready] + list(extra)
                return _after(always, val, deps) if deps else val

            def normalize(dep):
                if not fins:
                    return
                e, r0 = fins.pop(0)
                l = get(("l", e), r0, UR)
                if dep is not None:
                    l = _after(always, l, [dep])
                l = jnp.sum(l, axis=-1, keepdims=True)
                r = pl.reciprocal(l, approx=True)
                ctx = get(("o", e), r0, UR) * (r * (2.0 - l * r))
                ctx_s[2 * p + e, r0:r0 + UR, :] = ctx.astype(BF16)
                pend.append((clock[0] + CFG["df"], ctx, "f"))

            def scores(e, a):
                for unit in _units(a, "a"):
                    for (r0, nr, c0, nc) in unit:
                        s = _dot_nt(take(q_s[e, r0:r0 + nr, :], "fM"), k_s[2 * p + e, c0:c0 + nc, :])
                        tiles = []
                        for t in range(c0, c0 + nc, 128):
                            x = s[:, t - c0:t - c0 + 128]
                            if t + 128 > r0:
                                x = _cat([x[g:g + G] if t + 128 <= r0 + g else
                                          jnp.where(dist <= r0 + g - t, x[g:g + G], masked)
                                          for g in range(0, nr, G)], 0)
                            tiles.append(x)
                        mm = _fold(jnp.maximum, tiles)
                        acc(("m", e), r0, mm, jnp.maximum)
                        st[("s", e, r0, c0)] = tiles
                    clock[0] += nr
                    if nr == UR:
                        normalize(mm)
                        last[0] = mm
                for u in range(a * SB // G, (a + 1) * SB // G):
                    k = (("m", e), u)
                    st[k] = jnp.broadcast_to(jnp.max(st[k], axis=-1, keepdims=True), (G, 128))
                for r0 in range(a * SB, (a + 1) * SB, UR):
                    pend.append((clock[0] + CFG["dM"] + r0 - a * SB, get(("m", e), r0, UR), "M"))

            def context(e, a):
                for unit in _units(a, "b"):
                    for (r0, nr, c0, nc) in unit:
                        m = take(get(("m", e), r0, nr), "f", [last[0][:nr]])
                        ps = [jnp.exp2(x - m) for x in st.pop(("s", e, r0, c0))]
                        acc(("l", e), r0, _fold(jnp.add, ps), jnp.add)
                        ps[-1] = _after(always, ps[-1], [get(("l", e), r0, nr)])
                        acc(("o", e), r0, _dot(_cat(ps, 1).astype(BF16), v_s[2 * p + e, c0:c0 + nc, :]), jnp.add)
                    clock[0] += nr
                    if len(unit) == 1:
                        normalize(get(("o", e), r0, nr))
                    if nr == UR:
                        last[0] = get(("o", e), r0, nr)
                fins.extend((e, r0) for r0 in range(a * SB, (a + 1) * SB, UR))

            for tok in CFG["order"].split():
                if tok == "W":
                    o_operands()
                elif tok[0] == "Q":
                    proj_q("AB".index(tok[1]))
                else:
                    (scores if tok[0] == "a" else context)("AB".index(tok[2]), int(tok[1]))
            while fins:
                normalize(None)

        def finish(ctx_s, wor_s, h_s, out_s):
            _wait(cp_late)
            wr = wr_s[...].astype(F32).reshape(1, M)
            always = all_true(jnp.broadcast_to(wr[:, :128], (8, 128)))
            lane = lax.broadcasted_iota(I32, (8, 128), 1)
            sub = lax.broadcasted_iota(I32, (8, 128), 0)
            score = [jnp.zeros((8, 128), F32) for _ in range(S // 1024)]
            side, mod = _Side(always, CFG["lag"]), []

            def o_proj(r0, nr):
                m = [None] * 7
                for p0 in range(0, NP, 2):
                    blocks = []
                    for pp in (p0, p0 + 1):
                        a0, a1 = (_split_rows(ctx_s[2 * pp + e, r0:r0 + nr, :].astype(F32)) for e in range(2))
                        blocks.append(((a0[0], a1[0]), (a0[1], a1[1])))
                    for i in _ORDER:
                        d = _dot(side.lhs(_cat([_LHS[i](b) for b in blocks], 1)).astype(BF16),
                                 _cat([wor_s[i, p0], wor_s[i, p0 + 1]], 0))
                        m[i] = d if m[i] is None else m[i] + d
                        side.result(m[i])
                tail = None
                for h0 in range(0, H, 4):
                    d = _dot(side.lhs(_cat([ctx_s[hh, r0:r0 + nr, :] for hh in range(h0, h0 + 4)], 1)),
                             _cat([wo_s[hh, :, 512:] for hh in range(h0, h0 + 4)], 0))
                    tail = d if tail is None else tail + d
                    side.result(tail)
                return _cat([_merge_rows(*_column(m, e)) for e in range(2)] + [tail], 1)

            def gates():
                ga, sb, cb, gb = (_cat(mod[t:t + M // 128], 1) for t in range(0, len(mod), M // 128))
                return ga, sb, _rb(1.0 + cb), gb

            def ln2(r0, attn):
                nr = attn.shape[0]
                ga, sb, cb1, gb = gates()
                x1 = _rb(x_s[r0:r0 + nr, :].astype(F32) + _rb(ga * _rb(attn)))
                x_s[r0:r0 + nr, :] = x1.astype(BF16)
                mu = jnp.sum(x1, axis=-1, keepdims=True) / M
                xc = x1 - mu
                var = _rb(jnp.sum(xc * xc, axis=-1, keepdims=True) / M)
                inv = 1.0 / _rb(jnp.sqrt(_rb(var + eps_b)))
                h2 = _rb(_rb(_rb(_rb(x1 - _rb(mu)) * inv) * cb1) + sb)
                h_s[r0:r0 + nr, :] = h2.astype(BF16)
                out_s[r0:r0 + nr, :] = (x1 + _rb(gb * h2)).astype(BF16)
                r = jnp.sum(h2 * wr, axis=-1, keepdims=True)
                for j in range(nr // 8):
                    g = r0 // 8 + j
                    score[g // 128] = jnp.where(lane == g % 128, r[8 * j:8 * j + 8], score[g // 128])

            def ln2_job(r0, attn):
                return lambda dep: ln2(r0, _cat([_after(always, attn[:, t:t + 128], [dep[:attn.shape[0]]])
                                                 for t in range(0, M, 128)], 1))

            def transpose_job(w_s, dst, f0):
                def run(dep):
                    wt = _cat([_after(always, w_s[f0:f0 + 128, t:t + 128], [dep[:128]])
                               for t in range(0, M, 128)], 1)
                    dst[f0 // 128, :M, :] = wt.astype(F32).T.astype(BF16)
                return run

            eblocks = CFG["eblocks"][:2] if CFG["skip_epi"] else CFG["eblocks"]
            starts = [sum(eblocks[:i]) for i in range(len(eblocks))]
            cp_out = [pltpu.make_async_copy(out_s.at[r0:r0 + nr], out_hbm.at[0, r0:r0 + nr], sems.at[6])
                      for r0, nr in zip(starts, eblocks)]
            side.spread(modulation(wmb_s, always, mod), 60)
            side.spread([transpose_job(w_s, dst, f0) for w_s, dst in ((wg_s, k_s), (wu_s, v_s))
                         for f0 in range(0, FA, 128)], 60)
            for i, (r0, nr) in enumerate(zip(starts, eblocks)):
                attn = o_proj(r0, nr)
                if i > 0:
                    cp_out[i - 1].start()
                if i + 1 < len(eblocks):
                    g = CFG["ln2g"]
                    side.spread([ln2_job(r0 + r, attn[r:r + g]) for r in range(0, nr, g)], CFG["ln2span"])
                else:
                    ln2(r0, attn)
                    cp_out[i].start()

            keys = []
            for t, r in enumerate(score):
                r = _rb(r)
                b = lax.shift_right_logical(pltpu.bitcast(jnp.where(r == 0.0, 0.0, r), I32), 16)
                rank = jnp.where(r != r, 0, jnp.where(b >= 0x8000, 0xFFFF - b, b + 0x8000))
                keys.append(pltpu.bitcast((rank << 11) + (S - 1 - (t * 1024 + lane * 8 + sub)) + (1 << 29), F32))
            tops = []
            for _ in range(TOPC):
                top = jnp.max(jnp.max(_fold(jnp.maximum, keys), axis=1, keepdims=True), axis=0, keepdims=True)
                keys = [jnp.where(k == top, 0.0, k) for k in keys]
                tops.append(top)
            slot = lax.broadcasted_iota(I32, (TOPC, 1), 0)
            kcol = jnp.zeros((TOPC, 1), F32)
            for c in range(TOPC):
                kcol = jnp.where(slot == c, tops[c], kcol)
            rank = (pltpu.bitcast(kcol, I32) - (1 << 29)) >> 11
            r_sel = pltpu.bitcast(jnp.where(rank >= 0x8000, rank - 0x8000, 0xFFFF - rank) << 16, F32)
            toks = [S - 1 - (pltpu.bitcast(top, I32)[0, 0] & (S - 1)) for top in tops]
            grps = [pl.multiple_of(tok & (S - 16), 16) for tok in toks]
            row16 = lax.broadcasted_iota(I32, (16, M), 0)
            hits = [row16 == (tok & 15) for tok in toks]

            def gather(ref):
                out = jnp.zeros((TOPC, M), F32)
                for c in range(TOPC):
                    row = jnp.sum(jnp.where(hits[c], ref[pl.ds(grps[c], 16), :].astype(F32), 0.0),
                                  axis=0, keepdims=True)
                    out = jnp.where(slot == c, row, out)
                return out

            def up(xb, wt_s, w_s):
                return _rb(_cat([_dot(xb, _cat([wt_s[j, :M, :] for j in range(FA // 128)], 1)),
                                 _dot_nt(xb, w_s[FA:, :])], 1))

            xs = gather(h_s)
            gate = up(xs.astype(BF16), k_s, wg_s)
            act = _rb(gate * _rb(_sigmoid(gate))) * up(xs.astype(BF16), v_s, wu_s)
            y = _rb(_rb(_dot(act.astype(BF16), wd_s[...])) * _rb(_sigmoid(r_sel)))
            new = gather(x_s) + _rb(gates()[3] * _rb(xs + y))

            _wait(cp_out)
            for c in range(TOPC):
                old = out_s[pl.ds(grps[c], 16), :].astype(F32)
                out_s[pl.ds(grps[c], 16), :] = jnp.where(hits[c], new[c:c + 1], old).astype(BF16)
            patch = [pltpu.make_async_copy(out_s.at[pl.ds(g0, 16)], out_hbm.at[0, pl.ds(g0, 16)], sems.at[7])
                     for g0 in grps]
            fresh = [_fold(jnp.logical_and, [grps[j] != grps[c] for j in range(c)]) for c in range(1, TOPC)]
            patch[0].start()
            for f, cp in zip(fresh, patch[1:]):
                pl.when(f)(cp.start)
            patch[0].wait()
            for f, cp in zip(fresh, patch[1:]):
                pl.when(f)(cp.wait)

        def phase23(q_s, ctx_s, wor_s, h_s, out_s):
            _wait(cp_wo)
            _start(cp_late)
            with _scope('attn'):
                pl.loop(0, NP)(lambda p: attend_pair(p, q_s, ctx_s, wor_s))
            finish(ctx_s, wor_s, h_s, out_s)

        pl.run_scoped(
            phase23,
            pltpu.VMEM((2, S, D), BF16), pltpu.VMEM((H, S, D), BF16), pltpu.VMEM((7, NP, D, 256), BF16),
            pltpu.VMEM((S, M), BF16), pltpu.VMEM((S, M), BF16))

    return kernel


@jax.jit
def pallas_adaLN_cond__compressed_kv_cla__moe_arch_mod__prompt_kernel(
    A_x, A_c_kv, A_w_q, A_w_uk, A_w_uv, A_w_o, B_x, B_w_r, B_w_gate, B_w_up, B_w_down, c, w_mod,
):
    del B_x
    _, S, M = A_x.shape
    Dc = A_c_kv.shape[2]
    H, D = A_w_q.shape[1:]
    F = B_w_gate.shape[1]
    assert (A_x.shape, A_c_kv.shape, H, D) == ((1, 2048, 640), (1, 2048, 512), 32, 128)
    return pl.pallas_call(
        _make_kernel(S, M, Dc, H, D, F),
        out_shape=jax.ShapeDtypeStruct(A_x.shape, A_x.dtype),
        in_specs=[pl.BlockSpec(memory_space=pl.ANY)] * 12,
        out_specs=pl.BlockSpec(memory_space=pl.ANY),
        scratch_shapes=[
            pltpu.VMEM((S, M), BF16),
            pltpu.VMEM((H // HG, HG // 2 * M, D), U32),
            pltpu.VMEM((H, D, M), BF16),
            pltpu.VMEM((F, M), BF16),
            pltpu.VMEM((F, M), BF16),
            pltpu.VMEM((F, M), BF16),
            pltpu.VMEM((M, 4 * M), BF16),
            pltpu.VMEM((H, S, D), BF16),
            pltpu.VMEM((H, S, D), BF16),
            pltpu.VMEM((8, S // 2, 256), BF16),
            pltpu.VMEM((1, M), BF16),
            pltpu.VMEM((M,), BF16),
            pltpu.SemaphoreType.DMA((8,)),
            pltpu.SemaphoreType.DMA((H // HG,)),
            pltpu.SemaphoreType.DMA((len(CFG['chunks']),)),
        ],
        compiler_params=pltpu.CompilerParams(vmem_limit_bytes=120 * 1024 * 1024, flags=CFG["flags"]),
        name="adaln_mla_mod",
    )(A_x, A_c_kv, A_w_q, A_w_uk, A_w_uv, A_w_o, B_w_r, B_w_gate.T, B_w_up.T, B_w_down, c, w_mod)
```

```python
import contextlib

import numpy as np
import jax
import jax.numpy as jnp
from jax import lax
import jax.experimental.pallas as pl
import jax.experimental.pallas.tpu as pltpu

CFG = dict(flags=None, skip_epi=False, chunks=(512, 512, 1024), lag=2, lag1=2, mstep=64, rstep=16, mspan=4, lspan=14, rspan=16, l1tok=1,
           dposa=(-2, 0.5), dposb=(1.5, 2.5), df=256, dM=256,
           eblocks=(512, 512, 384, 256, 192, 128, 64), ln2g=8, ln2span=60, ln1g=32,
           order='QA W a0A a1A b0A a2A b1A a3A b2A QB a0B a1B b3A b0B a2B b1B a3B b2B b3B')

F32 = jnp.float32
BF16 = jnp.bfloat16
U32 = jnp.uint32
I32 = jnp.int32
TOPC = 8
LOG2E = 1.4426950408889634
EPS = 1e-5
RG = 16
G = 64
UR = 256
SB = 512
HG = 8


def _scope(name):
    return jax.named_scope(name) if CFG.get('scopes') else contextlib.nullcontext()


def _rb(a):
    return a.astype(BF16).astype(F32)


def _dot(a, b):
    return jnp.dot(a, b, preferred_element_type=F32)


def _dot_nt(a, b):
    return lax.dot_general(a, b, (((1,), (1,)), ((), ())), preferred_element_type=F32)


def _sigmoid(a):
    return 1.0 / (1.0 + jnp.exp(-a))


def _cat(xs, axis):
    return jnp.concatenate(xs, axis=axis) if len(xs) > 1 else xs[0]


def _fold(op, xs):
    acc = xs[0]
    for x in xs[1:]:
        acc = op(acc, x)
    return acc


def _words(w):
    return pltpu.bitcast(w.reshape(w.shape[0] * w.shape[1], w.shape[2]), U32)


def _halves(u):
    return pltpu.bitcast(u << 16, F32), pltpu.bitcast(u & np.uint32(0xFFFF0000), F32)


def _after(always, val, deps):
    t = _fold(jnp.maximum, deps)
    if val.dtype == BF16:
        t = pltpu.bitcast(t.astype(BF16), I32)
        out = jnp.where(jnp.tile(always, (t.shape[0] // 8, 1)), pltpu.bitcast(val, I32), t)
        return pltpu.bitcast(out, BF16)
    if val.dtype != F32:
        t = pltpu.bitcast(t, val.dtype)
    return jnp.where(jnp.tile(always, (t.shape[0] // 8, 1)), val, t)


class _Side:
    def __init__(self, always=None, lag=1, stagger=0):
        self.stagger = stagger
        self.always, self.lag, self.jobs, self.done, self.n = always, lag, {}, {}, 0

    def spread(self, jobs, span, delay=0):
        for t, job in enumerate(jobs):
            self.jobs.setdefault(self.n + delay + t * span // len(jobs), []).append(job)

    def lhs(self, x):
        toks = self.done.pop(self.n, None)
        if not toks:
            return x
        rows = 8 if x.dtype == F32 else 16
        head = _after(self.always, x[:rows, :128], [jnp.tile(t, (rows // 8, 1)) for t in toks])
        return _cat([_cat([head, x[rows:, :128]], 0), x[:, 128:]], 1)

    def result(self, d):
        jobs = self.jobs.pop(self.n, ())
        for t, job in enumerate(jobs):
            tok = job(d[self.stagger * t // len(jobs) // 8 * 8:, :128])
            if tok is not None:
                self.done.setdefault(self.n + self.lag, []).append(tok)
        self.n += 1


def _split_rows(x):
    n = x.shape[0] // (2 * RG)
    y = x.reshape(n, 2, RG, x.shape[1])
    return y[:, 0].reshape(n * RG, x.shape[1]), y[:, 1].reshape(n * RG, x.shape[1])


def _merge_rows(top, bot):
    n = top.shape[0] // RG
    y = jnp.concatenate([top.reshape(n, 1, RG, top.shape[1]), bot.reshape(n, 1, RG, top.shape[1])], axis=1)
    return y.reshape(2 * n * RG, top.shape[1])


_LHS = (lambda a: a[0][0] + a[1][1], lambda a: a[1][0] + a[1][1], lambda a: a[0][0], lambda a: a[1][1],
        lambda a: a[0][0] + a[0][1], lambda a: a[1][0] - a[0][0], lambda a: a[0][1] - a[1][1])
_RHS = (lambda b: b[0][0] + b[1][1], lambda b: b[0][0], lambda b: b[0][1] - b[1][1],
        lambda b: b[1][0] - b[0][0], lambda b: b[1][1], lambda b: b[0][0] + b[0][1],
        lambda b: b[1][0] + b[1][1])
_ORDER = (2, 4, 3, 1, 0, 6, 5)


def _column(m, e):
    if e == 0:
        return (m[3] - m[4]) + m[0] + m[6], m[1] + m[3]
    return m[2] + m[4], (m[2] - m[1]) + m[0] + m[5]


def _row_blocks(x):
    top, bot = _split_rows(x)
    hk = x.shape[1] // 2
    return (top[:, :hk], top[:, hk:]), (bot[:, :hk], bot[:, hk:])


def _pair_blocks(u):
    w = _halves(u)
    hk = u.shape[0] // 2
    return (w[0][:hk], w[1][:hk]), (w[0][hk:], w[1][hk:])


def _units(a, kind):
    r0 = a * SB
    full = [[(r0 + ro, UR, c0, SB)] for c0 in range(0, r0, SB) for ro in range(0, SB, UR)]
    big = [(r0, 256, r0, 128), (r0 + 256, 256, r0, 384)]
    small = [(r0 + 128, 64, r0 + 128, 128), (r0 + 192, 64, r0 + 128, 128),
             (r0 + 384, 64, r0 + 384, 128), (r0 + 448, 64, r0 + 384, 128)]
    kb, ks = CFG["dpos" + kind]
    return [u for _, u in sorted(list(enumerate(full)) + [(kb, big), (ks, small)], key=lambda z: z[0])]


def _start(cps):
    for cp in cps:
        cp.start()


def _make_kernel(S, M, Dc, H, D, F):
    NP, NG, PG = H // 2, H // HG, HG // 2
    FA = F // 128 * 128
    eps_b = float(np.asarray(EPS, dtype=BF16).astype(np.float32))
    qscale = float(np.asarray(D ** -0.5, dtype=BF16).astype(np.float32)) * LOG2E
    masked = -1e9 * LOG2E
    nwait = [0]

    def _wait(cps):
        nwait[0] += 1
        with _scope(f"wait{nwait[0]}"):
            for cp in cps:
                cp.wait()

    def kernel(x_hbm, ckv_hbm, wq_hbm, wuk_hbm, wuv_hbm, wo_hbm, wr_hbm, wg_hbm, wu_hbm,
               wd_hbm, c_hbm, wmod_hbm, out_hbm,
               x_s, wq_u, wo_s, wg_s, wu_s, wd_s, wmb_s, k_s, v_s, hl_s, c_s, wr_s, sems, qsems, csems):
        cp_wo = [pltpu.make_async_copy(wo_hbm, wo_s, sems.at[0])]
        cp_late = [pltpu.make_async_copy(wmod_hbm.at[:, 2 * M:6 * M], wmb_s, sems.at[1]),
                   pltpu.make_async_copy(wg_hbm, wg_s, sems.at[1]),
                   pltpu.make_async_copy(wu_hbm, wu_s, sems.at[1]),
                   pltpu.make_async_copy(wd_hbm, wd_s, sems.at[1])]

        def pair_words(ref, g, j):
            return ref[g, pl.ds(j, ref.shape[1] // PG, stride=PG), :]

        def all_true(x):
            return (pltpu.bitcast(x, I32) | 1) != 0

        def modulation(w_s, always, outs):
            cv = c_s[...].astype(F32)
            sc = _rb(cv * _rb(_sigmoid(cv)))
            eye = lax.broadcasted_iota(I32, (128, 128), 0) == lax.broadcasted_iota(I32, (128, 128), 1)
            col = _cat([jnp.sum(jnp.where(eye, sc[:, t:t + 128], 0.0), axis=1, keepdims=True)
                        for t in range(0, M, 128)], 0)
            col = jnp.broadcast_to(col, (M, 128))

            step, part = CFG["mstep"], {}

            def job(t, r):
                def run(dep):
                    w = _after(always, w_s[r:r + step, t:t + 128], [jnp.tile(dep[:16], (step // 16, 1))])
                    prod = col[r:r + step] * w.astype(F32)
                    part[t] = _fold(jnp.add, ([part[t]] if r else []) + [prod[j:j + 8] for j in range(0, step, 8)])
                    if r + step == M:
                        outs.append(_rb(jnp.sum(part[t], axis=0, keepdims=True)))
                    return part[t]
                return run
            return [job(t, r) for t in range(0, w_s.shape[1], 128) for r in range(0, M, step)]

        def phase1(ckv_s, cl_s, w0_s, w0_u, wk_g, wv_g, wq_g, wk_u, wv_u, wma_s):
            chunks = CFG["chunks"]
            cstart = [sum(chunks[:i]) for i in range(len(chunks))]
            cp_w0 = [pltpu.make_async_copy(w.at[:, 0:2, :], w0_s.at[i], sems.at[2])
                     for i, w in enumerate((wuk_hbm, wuv_hbm))]
            cp_ckv = [pltpu.make_async_copy(ckv_hbm.at[0, r0:r0 + nr], ckv_s.at[r0:r0 + nr], csems.at[i])
                      for i, (r0, nr) in enumerate(zip(cstart, chunks))]
            cp_kv = [[pltpu.make_async_copy(w.at[:, HG * g:HG * (g + 1), :], dst.at[g], sems.at[3 if g == 0 else 4])
                      for w, dst in ((wuk_hbm, wk_g), (wuv_hbm, wv_g))] for g in range(NG)]
            cp_kv_rest = [cp for cps in cp_kv[1:] for cp in cps]
            cp_ln = [pltpu.make_async_copy(c_hbm, c_s, sems.at[5]),
                     pltpu.make_async_copy(wr_hbm, wr_s, sems.at[5]),
                     pltpu.make_async_copy(wmod_hbm.at[:, 0:2 * M], wma_s, sems.at[5])]

            def cp_step(g):
                rows = pl.ds(pl.multiple_of(S // NG * g, S // NG), S // NG)
                return [pltpu.make_async_copy(wq_hbm.at[:, pl.ds(pl.multiple_of(HG * g, HG), HG), :],
                                              wq_g.at[g], qsems.at[g]),
                        pltpu.make_async_copy(x_hbm.at[0, rows], x_s.at[rows], qsems.at[g])]

            def repack(always, src, dst, g, step=CFG['rstep']):
                def job(r):
                    def run(dep):
                        u = _after(always, _words(src[g, r:r + step]), [jnp.tile(dep[:8], (PG * step // 8, 1))])
                        dst[g, PG * r:PG * (r + step), :] = u
                        return pltpu.bitcast(_fold(jnp.bitwise_and, [u[t:t + 8] for t in range(0, PG * step, 8)]), F32)
                    return run
                return [job(r) for r in range(0, src.shape[1], step)]

            def kv_proj(p, uk, uv, side, r0=0, nr=S):
                bk, bv = _pair_blocks(uk), _pair_blocks(uv)
                m = [None] * 7
                for i in _ORDER:
                    m[i] = _dot(side.lhs(cl_s[i, r0 // 2:(r0 + nr) // 2, :]),
                                _cat([_RHS[i](bk), _RHS[i](bv)], 1).astype(BF16))
                    side.result(m[i])
                for e in range(2):
                    o = _merge_rows(*_column(m, e))
                    k_s[2 * p + e, r0:r0 + nr, :] = o[:, :D].astype(BF16)
                    v_s[2 * p + e, r0:r0 + nr, :] = o[:, D:].astype(BF16)

            def kv_pair(p, side):
                kv_proj(p, pair_words(wk_u, p // PG, p % PG), pair_words(wv_u, p // PG, p % PG), side)

            _start(cp_w0 + cp_ckv[:1])
            _wait(cp_w0)
            _start(cp_ckv[1:])
            for i in range(2):
                for r in range(Dc):
                    w0_u[i, r:r + 1, :] = pltpu.bitcast(w0_s[i, r], U32)
            for i, (r0, nr) in enumerate(zip(cstart, chunks)):
                _wait(cp_ckv[i:i + 1])
                if i == 0:
                    _start(cp_kv[0])
                blocks = _row_blocks(ckv_s[r0:r0 + nr, :].astype(F32))
                for j in _ORDER:
                    cl_s[j, r0 // 2:(r0 + nr) // 2, :] = _LHS[j](blocks).astype(BF16)
                kv_proj(0, w0_u[0], w0_u[1], _Side(), r0, nr)
            _wait(cp_kv[0])
            _start(cp_kv_rest + cp_ln + cp_step(0))
            wk_u[0] = _words(wk_g[0])
            wv_u[0] = _words(wv_g[0])
            for p in range(1, PG - 1):
                kv_pair(p, _Side())
            _wait(cp_kv_rest)
            side = _Side(all_true(w0_u[0, :8, :]), CFG["lag1"], S // 2 - 64)
            side.spread([job for g in range(1, NG) for src, dst in ((wk_g, wk_u), (wv_g, wv_u))
                         for job in repack(side.always, src, dst, g)], 6)
            kv_pair(PG - 1, side)
            _wait(cp_ln)
            _start([cp for g in range(1, NG) for cp in cp_step(g)] + cp_wo)

            def step(i, carry):
                for cp in cp_step(i):
                    cp.wait()
                always = lax.broadcasted_iota(I32, (8, 128), 0) < i + 8
                g, rows, mod = CFG["ln1g"], S // NG, []

                def ln1(r):
                    def run(dep):
                        r0 = pl.multiple_of(i * rows + r, g)
                        xv = _cat([_after(always, x_s[pl.ds(r0, g), t:t + 128], [dep[:g]])
                                   for t in range(0, M, 128)], 1).astype(F32)
                        mu = jnp.sum(xv, axis=-1, keepdims=True) * (1.0 / M)
                        xc = xv - mu
                        var = jnp.sum(xc * xc, axis=-1, keepdims=True) * (1.0 / M)
                        sa, ca = _cat(mod[:M // 128], 1), _cat(mod[M // 128:], 1)
                        h = xc * lax.rsqrt(var + EPS) * _rb(1.0 + ca) + sa
                        blocks = _row_blocks(h[:, :512])
                        rh = pl.ds(pl.multiple_of(i * (rows // 2) + r // 2, g // 2), g // 2)
                        for j in range(7):
                            hl_s[j, rh, :] = _LHS[j](blocks).astype(BF16)
                        hl_s[7, rh, :] = _cat(_split_rows(h[:, 512:]), 1).astype(BF16)
                        if CFG["l1tok"]:
                            return _fold(jnp.maximum, [h[j:j + 8, t:t + 128] for j in range(0, g, 8)
                                                       for t in range(0, M, 128)])
                    return run

                side = _Side(always, CFG["lag1"], S // 2 - 64)
                side.spread(modulation(wma_s, always, mod), CFG["mspan"])
                side.spread([ln1(r) for r in range(0, rows, g)], CFG["lspan"], CFG["mspan"])
                side.spread(repack(always, wq_g, wq_u, i), CFG['rspan'])
                for u in range(PG - 1):
                    kv_pair(PG + (PG - 1) * i + u, side)
                return carry

            with _scope('kvloop'):
                lax.fori_loop(0, NG, step, 0)

        pl.run_scoped(
            phase1,
            pltpu.VMEM((S, Dc), BF16), pltpu.VMEM((7, S // 2, Dc // 2), BF16),
            pltpu.VMEM((2, Dc, 2, D), BF16), pltpu.VMEM((2, Dc, D), U32),
            pltpu.VMEM((NG, Dc, HG, D), BF16), pltpu.VMEM((NG, Dc, HG, D), BF16), pltpu.VMEM((NG, M, HG, D), BF16),
            pltpu.VMEM((NG, PG * Dc, D), U32), pltpu.VMEM((NG, PG * Dc, D), U32), pltpu.VMEM((M, 2 * M), BF16))

        def attend_pair(p, q_s, ctx_s, wor_s):
            always = lax.broadcasted_iota(I32, (8, 128), 0) < p + 8
            dist = lax.broadcasted_iota(I32, (G, 128), 1) - lax.broadcasted_iota(I32, (G, 128), 0)
            st, clock, pend, fins, last = {}, [0], [], [], [None]

            def proj_q(e):
                u = pair_words(wq_u, p // PG, p % PG)
                bq = _pair_blocks(u[:512])
                if e == 0:
                    wt = _cat(_halves(u[512:]), 1).astype(BF16)
                    st["qt"] = [_dot(hl_s[7, :, :128], wt), _dot(hl_s[7, :, 128:], wt)]
                    st["qm"] = [None] * 7
                    for i in _ORDER[:-1]:
                        st["qm"][i] = _dot(hl_s[i], _RHS[i](bq).astype(BF16))
                else:
                    w = _RHS[5](bq).astype(BF16)
                    st["qm"][5] = _cat([_dot(hl_s[5, :S // 4, :], w), _dot(hl_s[5, S // 4:, :], w)], 0)
                top, bot = _column(st["qm"], e)
                o = _merge_rows(top + st["qt"][0][:, D * e:D * (e + 1)], bot + st["qt"][1][:, D * e:D * (e + 1)])
                q_s[e] = (o * qscale).astype(BF16)
                clock[0] += 512

            def o_operands():
                dep = _cat([st["qm"][2][t:t + 16] for t in range(0, S // 2, S // 16)], 0)
                wa, wb = (_cat([_after(always, wo_s[2 * p + e, :, t:t + 128], [dep]) for t in range(0, 512, 128)],
                               1).astype(F32) for e in range(2))
                for i in range(7):
                    wor_s[i, p] = _RHS[i](((wa[:, :256], wa[:, 256:]), (wb[:, :256], wb[:, 256:]))).astype(BF16)

            def acc(key, r0, val, op):
                for u in range(val.shape[0] // G):
                    k = (key, r0 // G + u)
                    part = val[G * u:G * (u + 1)]
                    st[k] = op(st[k], part) if k in st else part

            def get(key, r0, nr):
                return _cat([st[(key, u)] for u in range(r0 // G, (r0 + nr) // G)], 0)

            def take(val, kinds, extra=()):
                ready = [z for z in pend if z[0] <= clock[0] and z[1].shape[0] == val.shape[0] and z[2] in kinds]
                pend[:] = [z for z in pend if not any(z is y for y in ready)]
                deps = [z[1] for z in ready] + list(extra)
                return _after(always, val, deps) if deps else val

            def normalize(dep):
                if not fins:
                    return
                e, r0 = fins.pop(0)
                l = get(("l", e), r0, UR)
                if dep is not None:
                    l = _after(always, l, [dep])
                l = jnp.sum(l, axis=-1, keepdims=True)
                r = pl.reciprocal(l, approx=True)
                ctx = get(("o", e), r0, UR) * (r * (2.0 - l * r))
                ctx_s[2 * p + e, r0:r0 + UR, :] = ctx.astype(BF16)
                pend.append((clock[0] + CFG["df"], ctx, "f"))

            def scores(e, a):
                for unit in _units(a, "a"):
                    for (r0, nr, c0, nc) in unit:
                        s = _dot_nt(take(q_s[e, r0:r0 + nr, :], "fM"), k_s[2 * p + e, c0:c0 + nc, :])
                        tiles = []
                        for t in range(c0, c0 + nc, 128):
                            x = s[:, t - c0:t - c0 + 128]
                            if t + 128 > r0:
                                x = _cat([x[g:g + G] if t + 128 <= r0 + g else
                                          jnp.where(dist <= r0 + g - t, x[g:g + G], masked)
                                          for g in range(0, nr, G)], 0)
                            tiles.append(x)
                        mm = _fold(jnp.maximum, tiles)
                        acc(("m", e), r0, mm, jnp.maximum)
                        st[("s", e, r0, c0)] = tiles
                    clock[0] += nr
                    if nr == UR:
                        normalize(mm)
                        last[0] = mm
                for u in range(a * SB // G, (a + 1) * SB // G):
                    k = (("m", e), u)
                    st[k] = jnp.broadcast_to(jnp.max(st[k], axis=-1, keepdims=True), (G, 128))
                for r0 in range(a * SB, (a + 1) * SB, UR):
                    pend.append((clock[0] + CFG["dM"] + r0 - a * SB, get(("m", e), r0, UR), "M"))

            def context(e, a):
                for unit in _units(a, "b"):
                    for (r0, nr, c0, nc) in unit:
                        m = take(get(("m", e), r0, nr), "f", [last[0][:nr]])
                        ps = [jnp.exp2(x - m) for x in st.pop(("s", e, r0, c0))]
                        acc(("l", e), r0, _fold(jnp.add, ps), jnp.add)
                        ps[-1] = _after(always, ps[-1], [get(("l", e), r0, nr)])
                        acc(("o", e), r0, _dot(_cat(ps, 1).astype(BF16), v_s[2 * p + e, c0:c0 + nc, :]), jnp.add)
                    clock[0] += nr
                    if len(unit) == 1:
                        normalize(get(("o", e), r0, nr))
                    if nr == UR:
                        last[0] = get(("o", e), r0, nr)
                fins.extend((e, r0) for r0 in range(a * SB, (a + 1) * SB, UR))

            for tok in CFG["order"].split():
                if tok == "W":
                    o_operands()
                elif tok[0] == "Q":
                    proj_q("AB".index(tok[1]))
                else:
                    (scores if tok[0] == "a" else context)("AB".index(tok[2]), int(tok[1]))
            while fins:
                normalize(None)

        def finish(ctx_s, wor_s, h_s, out_s):
            _wait(cp_late)
            wr = wr_s[...].astype(F32).reshape(1, M)
            always = all_true(jnp.broadcast_to(wr[:, :128], (8, 128)))
            lane = lax.broadcasted_iota(I32, (8, 128), 1)
            sub = lax.broadcasted_iota(I32, (8, 128), 0)
            score = [jnp.zeros((8, 128), F32) for _ in range(S // 1024)]
            side, mod = _Side(always, CFG["lag"]), []

            def o_proj(r0, nr):
                m = [None] * 7
                for p0 in range(0, NP, 2):
                    blocks = []
                    for pp in (p0, p0 + 1):
                        a0, a1 = (_split_rows(ctx_s[2 * pp + e, r0:r0 + nr, :].astype(F32)) for e in range(2))
                        blocks.append(((a0[0], a1[0]), (a0[1], a1[1])))
                    for i in _ORDER:
                        d = _dot(side.lhs(_cat([_LHS[i](b) for b in blocks], 1)).astype(BF16),
                                 _cat([wor_s[i, p0], wor_s[i, p0 + 1]], 0))
                        m[i] = d if m[i] is None else m[i] + d
                        side.result(m[i])
                tail = None
                for h0 in range(0, H, 4):
                    d = _dot(side.lhs(_cat([ctx_s[hh, r0:r0 + nr, :] for hh in range(h0, h0 + 4)], 1)),
                             _cat([wo_s[hh, :, 512:] for hh in range(h0, h0 + 4)], 0))
                    tail = d if tail is None else tail + d
                    side.result(tail)
                return _cat([_merge_rows(*_column(m, e)) for e in range(2)] + [tail], 1)

            def gates():
                ga, sb, cb, gb = (_cat(mod[t:t + M // 128], 1) for t in range(0, len(mod), M // 128))
                return ga, sb, _rb(1.0 + cb), gb

            def ln2(r0, attn):
                nr = attn.shape[0]
                ga, sb, cb1, gb = gates()
                x1 = _rb(x_s[r0:r0 + nr, :].astype(F32) + _rb(ga * _rb(attn)))
                x_s[r0:r0 + nr, :] = x1.astype(BF16)
                mu = jnp.sum(x1, axis=-1, keepdims=True) / M
                xc = x1 - mu
                var = _rb(jnp.sum(xc * xc, axis=-1, keepdims=True) / M)
                inv = 1.0 / _rb(jnp.sqrt(_rb(var + eps_b)))
                h2 = _rb(_rb(_rb(_rb(x1 - _rb(mu)) * inv) * cb1) + sb)
                h_s[r0:r0 + nr, :] = h2.astype(BF16)
                out_s[r0:r0 + nr, :] = (x1 + _rb(gb * h2)).astype(BF16)
                r = jnp.sum(h2 * wr, axis=-1, keepdims=True)
                for j in range(nr // 8):
                    g = r0 // 8 + j
                    score[g // 128] = jnp.where(lane == g % 128, r[8 * j:8 * j + 8], score[g // 128])

            def ln2_job(r0, attn):
                return lambda dep: ln2(r0, _cat([_after(always, attn[:, t:t + 128], [dep[:attn.shape[0]]])
                                                 for t in range(0, M, 128)], 1))

            def transpose_job(w_s, dst, f0):
                def run(dep):
                    wt = _cat([_after(always, w_s[f0:f0 + 128, t:t + 128], [dep[:128]])
                               for t in range(0, M, 128)], 1)
                    dst[f0 // 128, :M, :] = wt.astype(F32).T.astype(BF16)
                return run

            eblocks = CFG["eblocks"][:2] if CFG["skip_epi"] else CFG["eblocks"]
            starts = [sum(eblocks[:i]) for i in range(len(eblocks))]
            cp_out = [pltpu.make_async_copy(out_s.at[r0:r0 + nr], out_hbm.at[0, r0:r0 + nr], sems.at[6])
                      for r0, nr in zip(starts, eblocks)]
            side.spread(modulation(wmb_s, always, mod), 60)
            side.spread([transpose_job(w_s, dst, f0) for w_s, dst in ((wg_s, k_s), (wu_s, v_s))
                         for f0 in range(0, FA, 128)], 60)
            for i, (r0, nr) in enumerate(zip(starts, eblocks)):
                attn = o_proj(r0, nr)
                if i > 0:
                    cp_out[i - 1].start()
                if i + 1 < len(eblocks):
                    g = CFG["ln2g"]
                    side.spread([ln2_job(r0 + r, attn[r:r + g]) for r in range(0, nr, g)], CFG["ln2span"])
                else:
                    ln2(r0, attn)
                    cp_out[i].start()

            keys = []
            for t, r in enumerate(score):
                r = _rb(r)
                b = lax.shift_right_logical(pltpu.bitcast(jnp.where(r == 0.0, 0.0, r), I32), 16)
                rank = jnp.where(r != r, 0, jnp.where(b >= 0x8000, 0xFFFF - b, b + 0x8000))
                keys.append(pltpu.bitcast((rank << 11) + (S - 1 - (t * 1024 + lane * 8 + sub)) + (1 << 29), F32))
            tops = []
            for _ in range(TOPC):
                top = jnp.max(jnp.max(_fold(jnp.maximum, keys), axis=1, keepdims=True), axis=0, keepdims=True)
                keys = [jnp.where(k == top, 0.0, k) for k in keys]
                tops.append(top)
            slot = lax.broadcasted_iota(I32, (TOPC, 1), 0)
            kcol = jnp.zeros((TOPC, 1), F32)
            for c in range(TOPC):
                kcol = jnp.where(slot == c, tops[c], kcol)
            rank = (pltpu.bitcast(kcol, I32) - (1 << 29)) >> 11
            r_sel = pltpu.bitcast(jnp.where(rank >= 0x8000, rank - 0x8000, 0xFFFF - rank) << 16, F32)
            toks = [S - 1 - (pltpu.bitcast(top, I32)[0, 0] & (S - 1)) for top in tops]
            grps = [pl.multiple_of(tok & (S - 16), 16) for tok in toks]
            row16 = lax.broadcasted_iota(I32, (16, M), 0)
            hits = [row16 == (tok & 15) for tok in toks]

            def gather(ref):
                out = jnp.zeros((TOPC, M), F32)
                for c in range(TOPC):
                    row = jnp.sum(jnp.where(hits[c], ref[pl.ds(grps[c], 16), :].astype(F32), 0.0),
                                  axis=0, keepdims=True)
                    out = jnp.where(slot == c, row, out)
                return out

            def up(xb, wt_s, w_s):
                return _rb(_cat([_dot(xb, _cat([wt_s[j, :M, :] for j in range(FA // 128)], 1)),
                                 _dot_nt(xb, w_s[FA:, :])], 1))

            xs = gather(h_s)
            gate = up(xs.astype(BF16), k_s, wg_s)
            act = _rb(gate * _rb(_sigmoid(gate))) * up(xs.astype(BF16), v_s, wu_s)
            y = _rb(_rb(_dot(act.astype(BF16), wd_s[...])) * _rb(_sigmoid(r_sel)))
            new = gather(x_s) + _rb(gates()[3] * _rb(xs + y))

            _wait(cp_out)
            for c in range(TOPC):
                old = out_s[pl.ds(grps[c], 16), :].astype(F32)
                out_s[pl.ds(grps[c], 16), :] = jnp.where(hits[c], new[c:c + 1], old).astype(BF16)
            patch = [pltpu.make_async_copy(out_s.at[pl.ds(g0, 16)], out_hbm.at[0, pl.ds(g0, 16)], sems.at[7])
                     for g0 in grps]
            fresh = [_fold(jnp.logical_and, [grps[j] != grps[c] for j in range(c)]) for c in range(1, TOPC)]
            patch[0].start()
            for f, cp in zip(fresh, patch[1:]):
                pl.when(f)(cp.start)
            patch[0].wait()
            for f, cp in zip(fresh, patch[1:]):
                pl.when(f)(cp.wait)

        def phase23(q_s, ctx_s, wor_s, h_s, out_s):
            _wait(cp_wo)
            _start(cp_late)
            with _scope('attn'):
                pl.loop(0, NP)(lambda p: attend_pair(p, q_s, ctx_s, wor_s))
            finish(ctx_s, wor_s, h_s, out_s)

        pl.run_scoped(
            phase23,
            pltpu.VMEM((2, S, D), BF16), pltpu.VMEM((H, S, D), BF16), pltpu.VMEM((7, NP, D, 256), BF16),
            pltpu.VMEM((S, M), BF16), pltpu.VMEM((S, M), BF16))

    return kernel


@jax.jit
def pallas_adaLN_cond__compressed_kv_cla__moe_arch_mod__prompt_kernel(
    A_x, A_c_kv, A_w_q, A_w_uk, A_w_uv, A_w_o, B_x, B_w_r, B_w_gate, B_w_up, B_w_down, c, w_mod,
):
    del B_x
    _, S, M = A_x.shape
    Dc = A_c_kv.shape[2]
    H, D = A_w_q.shape[1:]
    F = B_w_gate.shape[1]
    assert (A_x.shape, A_c_kv.shape, H, D) == ((1, 2048, 640), (1, 2048, 512), 32, 128)
    return pl.pallas_call(
        _make_kernel(S, M, Dc, H, D, F),
        out_shape=jax.ShapeDtypeStruct(A_x.shape, A_x.dtype),
        in_specs=[pl.BlockSpec(memory_space=pl.ANY)] * 12,
        out_specs=pl.BlockSpec(memory_space=pl.ANY),
        scratch_shapes=[
            pltpu.VMEM((S, M), BF16),
            pltpu.VMEM((H // HG, HG // 2 * M, D), U32),
            pltpu.VMEM((H, D, M), BF16),
            pltpu.VMEM((F, M), BF16),
            pltpu.VMEM((F, M), BF16),
            pltpu.VMEM((F, M), BF16),
            pltpu.VMEM((M, 4 * M), BF16),
            pltpu.VMEM((H, S, D), BF16),
            pltpu.VMEM((H, S, D), BF16),
            pltpu.VMEM((8, S // 2, 256), BF16),
            pltpu.VMEM((1, M), BF16),
            pltpu.VMEM((M,), BF16),
            pltpu.SemaphoreType.DMA((8,)),
            pltpu.SemaphoreType.DMA((H // HG,)),
            pltpu.SemaphoreType.DMA((len(CFG['chunks']),)),
        ],
        compiler_params=pltpu.CompilerParams(vmem_limit_bytes=120 * 1024 * 1024, flags=CFG["flags"]),
        name="adaln_mla_mod",
    )(A_x, A_c_kv, A_w_q, A_w_uk, A_w_uv, A_w_o, B_w_r, B_w_gate.T, B_w_up.T, B_w_down, c, w_mod)
```

```python
import numpy as np
import jax
import jax.numpy as jnp
from jax import lax
import jax.experimental.pallas as pl
import jax.experimental.pallas.tpu as pltpu

F32 = jnp.float32
BF16 = jnp.bfloat16
U32 = jnp.uint32
I32 = jnp.int32
TOPC = 8
LOG2E = 1.4426950408889634
EPS = 1e-5
RG = 16
G = 64
UR = 256
SB = 512
HG = 8
KV_CHUNKS = (512, 512, 1024)
OUT_BLOCKS = (512, 512, 384, 256, 192, 128, 64)
PAIR_ORDER = "QA W a0A a1A b0A a2A b1A a3A b2A QB a0B a1B b3A b0B a2B b1B a3B b2B b3B".split()


def _rb(a):
    return a.astype(BF16).astype(F32)


def _dot(a, b):
    return jnp.dot(a, b, preferred_element_type=F32)


def _dot_nt(a, b):
    return lax.dot_general(a, b, (((1,), (1,)), ((), ())), preferred_element_type=F32)


def _sigmoid(a):
    return 1.0 / (1.0 + jnp.exp(-a))


def _cat(xs, axis):
    return jnp.concatenate(xs, axis=axis) if len(xs) > 1 else xs[0]


def _fold(op, xs):
    acc = xs[0]
    for x in xs[1:]:
        acc = op(acc, x)
    return acc


def _words(w):
    return pltpu.bitcast(w.reshape(w.shape[0] * w.shape[1], w.shape[2]), U32)


def _halves(u):
    return pltpu.bitcast(u << 16, F32), pltpu.bitcast(u & np.uint32(0xFFFF0000), F32)


def _after(always, val, deps):
    t = _fold(jnp.maximum, deps)
    if val.dtype == BF16:
        t = pltpu.bitcast(t.astype(BF16), I32)
        out = jnp.where(jnp.tile(always, (t.shape[0] // 8, 1)), pltpu.bitcast(val, I32), t)
        return pltpu.bitcast(out, BF16)
    if val.dtype != F32:
        t = pltpu.bitcast(t, val.dtype)
    return jnp.where(jnp.tile(always, (t.shape[0] // 8, 1)), val, t)


class _Side:
    def __init__(self, always=None, stagger=0):
        self.always, self.stagger, self.jobs, self.done, self.n = always, stagger, {}, {}, 0

    def spread(self, jobs, span, delay=0):
        for t, job in enumerate(jobs):
            self.jobs.setdefault(self.n + delay + t * span // len(jobs), []).append(job)

    def lhs(self, x):
        toks = self.done.pop(self.n, None)
        if not toks:
            return x
        rows = 8 if x.dtype == F32 else 16
        head = _after(self.always, x[:rows, :128], [jnp.tile(t, (rows // 8, 1)) for t in toks])
        return _cat([_cat([head, x[rows:, :128]], 0), x[:, 128:]], 1)

    def result(self, d):
        jobs = self.jobs.pop(self.n, ())
        for t, job in enumerate(jobs):
            tok = job(d[self.stagger * t // len(jobs) // 8 * 8:, :128])
            if tok is not None:
                self.done.setdefault(self.n + 2, []).append(tok)
        self.n += 1


def _split_rows(x):
    n = x.shape[0] // (2 * RG)
    y = x.reshape(n, 2, RG, x.shape[1])
    return y[:, 0].reshape(n * RG, x.shape[1]), y[:, 1].reshape(n * RG, x.shape[1])


def _merge_rows(top, bot):
    n = top.shape[0] // RG
    y = jnp.concatenate([top.reshape(n, 1, RG, top.shape[1]), bot.reshape(n, 1, RG, top.shape[1])], axis=1)
    return y.reshape(2 * n * RG, top.shape[1])


_LHS = (lambda a: a[0][0] + a[1][1], lambda a: a[1][0] + a[1][1], lambda a: a[0][0], lambda a: a[1][1],
        lambda a: a[0][0] + a[0][1], lambda a: a[1][0] - a[0][0], lambda a: a[0][1] - a[1][1])
_RHS = (lambda b: b[0][0] + b[1][1], lambda b: b[0][0], lambda b: b[0][1] - b[1][1],
        lambda b: b[1][0] - b[0][0], lambda b: b[1][1], lambda b: b[0][0] + b[0][1],
        lambda b: b[1][0] + b[1][1])
_ORDER = (2, 4, 3, 1, 0, 6, 5)


def _column(m, e):
    if e == 0:
        return (m[3] - m[4]) + m[0] + m[6], m[1] + m[3]
    return m[2] + m[4], (m[2] - m[1]) + m[0] + m[5]


def _row_blocks(x):
    top, bot = _split_rows(x)
    hk = x.shape[1] // 2
    return (top[:, :hk], top[:, hk:]), (bot[:, :hk], bot[:, hk:])


def _pair_blocks(u):
    w = _halves(u)
    hk = u.shape[0] // 2
    return (w[0][:hk], w[1][:hk]), (w[0][hk:], w[1][hk:])


def _units(a, diag_pos):
    r0 = a * SB
    full = [[(r0 + ro, UR, c0, SB)] for c0 in range(0, r0, SB) for ro in range(0, SB, UR)]
    big = [(r0, 256, r0, 128), (r0 + 256, 256, r0, 384)]
    small = [(r0 + 128, 64, r0 + 128, 128), (r0 + 192, 64, r0 + 128, 128),
             (r0 + 384, 64, r0 + 384, 128), (r0 + 448, 64, r0 + 384, 128)]
    return [u for _, u in sorted(list(enumerate(full)) + list(zip(diag_pos, (big, small))), key=lambda z: z[0])]


def _start(cps):
    for cp in cps:
        cp.start()


def _wait(cps):
    for cp in cps:
        cp.wait()


def _make_kernel(S, M, Dc, H, D, F):
    NP, NG, PG = H // 2, H // HG, HG // 2
    FA = F // 128 * 128
    eps_b = float(np.asarray(EPS, dtype=BF16).astype(np.float32))
    qscale = float(np.asarray(D ** -0.5, dtype=BF16).astype(np.float32)) * LOG2E
    masked = -1e9 * LOG2E

    def kernel(x_hbm, ckv_hbm, wq_hbm, wuk_hbm, wuv_hbm, wo_hbm, wr_hbm, wg_hbm, wu_hbm,
               wd_hbm, c_hbm, wmod_hbm, out_hbm,
               x_s, wq_u, wo_s, wg_s, wu_s, wd_s, wmb_s, k_s, v_s, hl_s, c_s, wr_s, sems, qsems, csems):
        cp_wo = [pltpu.make_async_copy(wo_hbm, wo_s, sems.at[0])]
        cp_late = [pltpu.make_async_copy(wmod_hbm.at[:, 2 * M:6 * M], wmb_s, sems.at[1]),
                   pltpu.make_async_copy(wg_hbm, wg_s, sems.at[1]),
                   pltpu.make_async_copy(wu_hbm, wu_s, sems.at[1]),
                   pltpu.make_async_copy(wd_hbm, wd_s, sems.at[1])]

        def pair_words(ref, g, j):
            return ref[g, pl.ds(j, ref.shape[1] // PG, stride=PG), :]

        def all_true(x):
            return (pltpu.bitcast(x, I32) | 1) != 0

        def modulation(w_s, always, outs):
            cv = c_s[...].astype(F32)
            sc = _rb(cv * _rb(_sigmoid(cv)))
            eye = lax.broadcasted_iota(I32, (128, 128), 0) == lax.broadcasted_iota(I32, (128, 128), 1)
            col = _cat([jnp.sum(jnp.where(eye, sc[:, t:t + 128], 0.0), axis=1, keepdims=True)
                        for t in range(0, M, 128)], 0)
            col = jnp.broadcast_to(col, (M, 128))

            step, part = 64, {}

            def job(t, r):
                def run(dep):
                    w = _after(always, w_s[r:r + step, t:t + 128], [jnp.tile(dep[:16], (step // 16, 1))])
                    prod = col[r:r + step] * w.astype(F32)
                    part[t] = _fold(jnp.add, ([part[t]] if r else []) + [prod[j:j + 8] for j in range(0, step, 8)])
                    if r + step == M:
                        outs.append(_rb(jnp.sum(part[t], axis=0, keepdims=True)))
                    return part[t]
                return run
            return [job(t, r) for t in range(0, w_s.shape[1], 128) for r in range(0, M, step)]

        def phase1(ckv_s, cl_s, w0_s, w0_u, wk_g, wv_g, wq_g, wk_u, wv_u, wma_s):
            chunks = KV_CHUNKS
            cstart = [sum(chunks[:i]) for i in range(len(chunks))]
            cp_w0 = [pltpu.make_async_copy(w.at[:, 0:2, :], w0_s.at[i], sems.at[2])
                     for i, w in enumerate((wuk_hbm, wuv_hbm))]
            cp_ckv = [pltpu.make_async_copy(ckv_hbm.at[0, r0:r0 + nr], ckv_s.at[r0:r0 + nr], csems.at[i])
                      for i, (r0, nr) in enumerate(zip(cstart, chunks))]
            cp_kv = [[pltpu.make_async_copy(w.at[:, HG * g:HG * (g + 1), :], dst.at[g], sems.at[3 if g == 0 else 4])
                      for w, dst in ((wuk_hbm, wk_g), (wuv_hbm, wv_g))] for g in range(NG)]
            cp_kv_rest = [cp for cps in cp_kv[1:] for cp in cps]
            cp_ln = [pltpu.make_async_copy(c_hbm, c_s, sems.at[5]),
                     pltpu.make_async_copy(wr_hbm, wr_s, sems.at[5]),
                     pltpu.make_async_copy(wmod_hbm.at[:, 0:2 * M], wma_s, sems.at[5])]

            def cp_step(g):
                rows = pl.ds(pl.multiple_of(S // NG * g, S // NG), S // NG)
                return [pltpu.make_async_copy(wq_hbm.at[:, pl.ds(pl.multiple_of(HG * g, HG), HG), :],
                                              wq_g.at[g], qsems.at[g]),
                        pltpu.make_async_copy(x_hbm.at[0, rows], x_s.at[rows], qsems.at[g])]

            def repack(always, src, dst, g, step=16):
                def job(r):
                    def run(dep):
                        u = _after(always, _words(src[g, r:r + step]), [jnp.tile(dep[:8], (PG * step // 8, 1))])
                        dst[g, PG * r:PG * (r + step), :] = u
                        return pltpu.bitcast(_fold(jnp.bitwise_and, [u[t:t + 8] for t in range(0, PG * step, 8)]), F32)
                    return run
                return [job(r) for r in range(0, src.shape[1], step)]

            def kv_proj(p, uk, uv, side, r0=0, nr=S):
                bk, bv = _pair_blocks(uk), _pair_blocks(uv)
                m = [None] * 7
                for i in _ORDER:
                    m[i] = _dot(side.lhs(cl_s[i, r0 // 2:(r0 + nr) // 2, :]),
                                _cat([_RHS[i](bk), _RHS[i](bv)], 1).astype(BF16))
                    side.result(m[i])
                for e in range(2):
                    o = _merge_rows(*_column(m, e))
                    k_s[2 * p + e, r0:r0 + nr, :] = o[:, :D].astype(BF16)
                    v_s[2 * p + e, r0:r0 + nr, :] = o[:, D:].astype(BF16)

            def kv_pair(p, side):
                kv_proj(p, pair_words(wk_u, p // PG, p % PG), pair_words(wv_u, p // PG, p % PG), side)

            _start(cp_w0 + cp_ckv[:1])
            _wait(cp_w0)
            _start(cp_ckv[1:])
            for i in range(2):
                for r in range(Dc):
                    w0_u[i, r:r + 1, :] = pltpu.bitcast(w0_s[i, r], U32)
            for i, (r0, nr) in enumerate(zip(cstart, chunks)):
                _wait(cp_ckv[i:i + 1])
                if i == 0:
                    _start(cp_kv[0])
                blocks = _row_blocks(ckv_s[r0:r0 + nr, :].astype(F32))
                for j in _ORDER:
                    cl_s[j, r0 // 2:(r0 + nr) // 2, :] = _LHS[j](blocks).astype(BF16)
                kv_proj(0, w0_u[0], w0_u[1], _Side(), r0, nr)
            _wait(cp_kv[0])
            _start(cp_kv_rest + cp_ln + cp_step(0))
            wk_u[0] = _words(wk_g[0])
            wv_u[0] = _words(wv_g[0])
            for p in range(1, PG - 1):
                kv_pair(p, _Side())
            _wait(cp_kv_rest)
            side = _Side(all_true(w0_u[0, :8, :]), S // 2 - 64)
            side.spread([job for g in range(1, NG) for src, dst in ((wk_g, wk_u), (wv_g, wv_u))
                         for job in repack(side.always, src, dst, g)], 6)
            kv_pair(PG - 1, side)
            _wait(cp_ln)
            _start([cp for g in range(1, NG) for cp in cp_step(g)] + cp_wo)

            def step(i, carry):
                _wait(cp_step(i))
                always = lax.broadcasted_iota(I32, (8, 128), 0) < i + 8
                g, rows, mod = 2 * RG, S // NG, []

                def ln1(r):
                    def run(dep):
                        r0 = pl.multiple_of(i * rows + r, g)
                        xv = _cat([_after(always, x_s[pl.ds(r0, g), t:t + 128], [dep[:g]])
                                   for t in range(0, M, 128)], 1).astype(F32)
                        mu = jnp.sum(xv, axis=-1, keepdims=True) * (1.0 / M)
                        xc = xv - mu
                        var = jnp.sum(xc * xc, axis=-1, keepdims=True) * (1.0 / M)
                        sa, ca = _cat(mod[:M // 128], 1), _cat(mod[M // 128:], 1)
                        h = xc * lax.rsqrt(var + EPS) * _rb(1.0 + ca) + sa
                        blocks = _row_blocks(h[:, :512])
                        rh = pl.ds(pl.multiple_of(i * (rows // 2) + r // 2, g // 2), g // 2)
                        for j in range(7):
                            hl_s[j, rh, :] = _LHS[j](blocks).astype(BF16)
                        hl_s[7, rh, :] = _cat(_split_rows(h[:, 512:]), 1).astype(BF16)
                        return _fold(jnp.maximum, [h[j:j + 8, t:t + 128] for j in range(0, g, 8)
                                                   for t in range(0, M, 128)])
                    return run

                side = _Side(always, S // 2 - 64)
                side.spread(modulation(wma_s, always, mod), 4)
                side.spread([ln1(r) for r in range(0, rows, g)], 14, 4)
                side.spread(repack(always, wq_g, wq_u, i), 16)
                for u in range(PG - 1):
                    kv_pair(PG + (PG - 1) * i + u, side)
                return carry

            lax.fori_loop(0, NG, step, 0)

        pl.run_scoped(
            phase1,
            pltpu.VMEM((S, Dc), BF16), pltpu.VMEM((7, S // 2, Dc // 2), BF16),
            pltpu.VMEM((2, Dc, 2, D), BF16), pltpu.VMEM((2, Dc, D), U32),
            pltpu.VMEM((NG, Dc, HG, D), BF16), pltpu.VMEM((NG, Dc, HG, D), BF16), pltpu.VMEM((NG, M, HG, D), BF16),
            pltpu.VMEM((NG, PG * Dc, D), U32), pltpu.VMEM((NG, PG * Dc, D), U32), pltpu.VMEM((M, 2 * M), BF16))

        def attend_pair(p, q_s, ctx_s, wor_s):
            always = lax.broadcasted_iota(I32, (8, 128), 0) < p + 8
            dist = lax.broadcasted_iota(I32, (G, 128), 1) - lax.broadcasted_iota(I32, (G, 128), 0)
            st, clock, pend, fins, last = {}, [0], [], [], [None]

            def proj_q(e):
                u = pair_words(wq_u, p // PG, p % PG)
                bq = _pair_blocks(u[:512])
                if e == 0:
                    wt = _cat(_halves(u[512:]), 1).astype(BF16)
                    st["qt"] = [_dot(hl_s[7, :, :128], wt), _dot(hl_s[7, :, 128:], wt)]
                    st["qm"] = [None] * 7
                    for i in _ORDER[:-1]:
                        st["qm"][i] = _dot(hl_s[i], _RHS[i](bq).astype(BF16))
                else:
                    w = _RHS[5](bq).astype(BF16)
                    st["qm"][5] = _cat([_dot(hl_s[5, :S // 4, :], w), _dot(hl_s[5, S // 4:, :], w)], 0)
                top, bot = _column(st["qm"], e)
                o = _merge_rows(top + st["qt"][0][:, D * e:D * (e + 1)], bot + st["qt"][1][:, D * e:D * (e + 1)])
                q_s[e] = (o * qscale).astype(BF16)
                clock[0] += 512

            def o_operands():
                dep = _cat([st["qm"][2][t:t + 16] for t in range(0, S // 2, S // 16)], 0)
                wa, wb = (_cat([_after(always, wo_s[2 * p + e, :, t:t + 128], [dep]) for t in range(0, 512, 128)],
                               1).astype(F32) for e in range(2))
                for i in range(7):
                    wor_s[i, p] = _RHS[i](((wa[:, :256], wa[:, 256:]), (wb[:, :256], wb[:, 256:]))).astype(BF16)

            def acc(key, r0, val, op):
                for u in range(val.shape[0] // G):
                    k = (key, r0 // G + u)
                    part = val[G * u:G * (u + 1)]
                    st[k] = op(st[k], part) if k in st else part

            def get(key, r0, nr):
                return _cat([st[(key, u)] for u in range(r0 // G, (r0 + nr) // G)], 0)

            def take(val, kinds, extra=()):
                ready = [z for z in pend if z[0] <= clock[0] and z[1].shape[0] == val.shape[0] and z[2] in kinds]
                pend[:] = [z for z in pend if not any(z is y for y in ready)]
                deps = [z[1] for z in ready] + list(extra)
                return _after(always, val, deps) if deps else val

            def normalize(dep):
                if not fins:
                    return
                e, r0 = fins.pop(0)
                l = get(("l", e), r0, UR)
                if dep is not None:
                    l = _after(always, l, [dep])
                l = jnp.sum(l, axis=-1, keepdims=True)
                r = pl.reciprocal(l, approx=True)
                ctx = get(("o", e), r0, UR) * (r * (2.0 - l * r))
                ctx_s[2 * p + e, r0:r0 + UR, :] = ctx.astype(BF16)
                pend.append((clock[0] + UR, ctx, "f"))

            def scores(e, a):
                for unit in _units(a, (-1, 0.5)):
                    for (r0, nr, c0, nc) in unit:
                        s = _dot_nt(take(q_s[e, r0:r0 + nr, :], "fM"), k_s[2 * p + e, c0:c0 + nc, :])
                        tiles = []
                        for t in range(c0, c0 + nc, 128):
                            x = s[:, t - c0:t - c0 + 128]
                            if t + 128 > r0:
                                x = _cat([x[g:g + G] if t + 128 <= r0 + g else
                                          jnp.where(dist <= r0 + g - t, x[g:g + G], masked)
                                          for g in range(0, nr, G)], 0)
                            tiles.append(x)
                        mm = _fold(jnp.maximum, tiles)
                        acc(("m", e), r0, mm, jnp.maximum)
                        st[("s", e, r0, c0)] = tiles
                    clock[0] += nr
                    if nr == UR:
                        normalize(mm)
                        last[0] = mm
                for u in range(a * SB // G, (a + 1) * SB // G):
                    k = (("m", e), u)
                    st[k] = jnp.broadcast_to(jnp.max(st[k], axis=-1, keepdims=True), (G, 128))
                for r0 in range(a * SB, (a + 1) * SB, UR):
                    pend.append((clock[0] + UR + r0 - a * SB, get(("m", e), r0, UR), "M"))

            def context(e, a):
                for unit in _units(a, (1.5, 2.5)):
                    for (r0, nr, c0, nc) in unit:
                        m = take(get(("m", e), r0, nr), "f", [last[0][:nr]])
                        ps = [jnp.exp2(x - m) for x in st.pop(("s", e, r0, c0))]
                        acc(("l", e), r0, _fold(jnp.add, ps), jnp.add)
                        ps[-1] = _after(always, ps[-1], [get(("l", e), r0, nr)])
                        acc(("o", e), r0, _dot(_cat(ps, 1).astype(BF16), v_s[2 * p + e, c0:c0 + nc, :]), jnp.add)
                    clock[0] += nr
                    if len(unit) == 1:
                        normalize(get(("o", e), r0, nr))
                    if nr == UR:
                        last[0] = get(("o", e), r0, nr)
                fins.extend((e, r0) for r0 in range(a * SB, (a + 1) * SB, UR))

            for tok in PAIR_ORDER:
                if tok == "W":
                    o_operands()
                elif tok[0] == "Q":
                    proj_q("AB".index(tok[1]))
                else:
                    (scores if tok[0] == "a" else context)("AB".index(tok[2]), int(tok[1]))
            while fins:
                normalize(None)

        def finish(ctx_s, wor_s, h_s, out_s):
            _wait(cp_late)
            wr = wr_s[...].astype(F32).reshape(1, M)
            always = all_true(jnp.broadcast_to(wr[:, :128], (8, 128)))
            lane = lax.broadcasted_iota(I32, (8, 128), 1)
            sub = lax.broadcasted_iota(I32, (8, 128), 0)
            score = [jnp.zeros((8, 128), F32) for _ in range(S // 1024)]
            side, mod = _Side(always), []

            def o_proj(r0, nr):
                m = [None] * 7
                for p0 in range(0, NP, 2):
                    blocks = []
                    for pp in (p0, p0 + 1):
                        a0, a1 = (_split_rows(ctx_s[2 * pp + e, r0:r0 + nr, :].astype(F32)) for e in range(2))
                        blocks.append(((a0[0], a1[0]), (a0[1], a1[1])))
                    for i in _ORDER:
                        d = _dot(side.lhs(_cat([_LHS[i](b) for b in blocks], 1)).astype(BF16),
                                 _cat([wor_s[i, p0], wor_s[i, p0 + 1]], 0))
                        m[i] = d if m[i] is None else m[i] + d
                        side.result(m[i])
                tail = None
                for h0 in range(0, H, 4):
                    d = _dot(side.lhs(_cat([ctx_s[hh, r0:r0 + nr, :] for hh in range(h0, h0 + 4)], 1)),
                             _cat([wo_s[hh, :, 512:] for hh in range(h0, h0 + 4)], 0))
                    tail = d if tail is None else tail + d
                    side.result(tail)
                return _cat([_merge_rows(*_column(m, e)) for e in range(2)] + [tail], 1)

            def gates():
                ga, sb, cb, gb = (_cat(mod[t:t + M // 128], 1) for t in range(0, len(mod), M // 128))
                return ga, sb, _rb(1.0 + cb), gb

            def ln2(r0, attn):
                nr = attn.shape[0]
                ga, sb, cb1, gb = gates()
                x1 = _rb(x_s[r0:r0 + nr, :].astype(F32) + _rb(ga * _rb(attn)))
                x_s[r0:r0 + nr, :] = x1.astype(BF16)
                mu = jnp.sum(x1, axis=-1, keepdims=True) / M
                xc = x1 - mu
                var = _rb(jnp.sum(xc * xc, axis=-1, keepdims=True) / M)
                inv = 1.0 / _rb(jnp.sqrt(_rb(var + eps_b)))
                h2 = _rb(_rb(_rb(_rb(x1 - _rb(mu)) * inv) * cb1) + sb)
                h_s[r0:r0 + nr, :] = h2.astype(BF16)
                out_s[r0:r0 + nr, :] = (x1 + _rb(gb * h2)).astype(BF16)
                r = jnp.sum(h2 * wr, axis=-1, keepdims=True)
                for j in range(nr // 8):
                    g = r0 // 8 + j
                    score[g // 128] = jnp.where(lane == g % 128, r[8 * j:8 * j + 8], score[g // 128])

            def ln2_job(r0, attn):
                return lambda dep: ln2(r0, _cat([_after(always, attn[:, t:t + 128], [dep[:attn.shape[0]]])
                                                 for t in range(0, M, 128)], 1))

            def transpose_job(w_s, dst, f0):
                def run(dep):
                    wt = _cat([_after(always, w_s[f0:f0 + 128, t:t + 128], [dep[:128]])
                               for t in range(0, M, 128)], 1)
                    dst[f0 // 128, :M, :] = wt.astype(F32).T.astype(BF16)
                return run

            eblocks = OUT_BLOCKS
            starts = [sum(eblocks[:i]) for i in range(len(eblocks))]
            cp_out = [pltpu.make_async_copy(out_s.at[r0:r0 + nr], out_hbm.at[0, r0:r0 + nr], sems.at[6])
                      for r0, nr in zip(starts, eblocks)]
            side.spread(modulation(wmb_s, always, mod), 60)
            side.spread([transpose_job(w_s, dst, f0) for w_s, dst in ((wg_s, k_s), (wu_s, v_s))
                         for f0 in range(0, FA, 128)], 60)
            for i, (r0, nr) in enumerate(zip(starts, eblocks)):
                attn = o_proj(r0, nr)
                if i > 0:
                    cp_out[i - 1].start()
                if i + 1 < len(eblocks):
                    side.spread([ln2_job(r0 + r, attn[r:r + 8]) for r in range(0, nr, 8)], 60)
                else:
                    ln2(r0, attn)
                    cp_out[i].start()

            keys = []
            for t, r in enumerate(score):
                r = _rb(r)
                b = lax.shift_right_logical(pltpu.bitcast(jnp.where(r == 0.0, 0.0, r), I32), 16)
                rank = jnp.where(r != r, 0, jnp.where(b >= 0x8000, 0xFFFF - b, b + 0x8000))
                keys.append(pltpu.bitcast((rank << 11) + (S - 1 - (t * 1024 + lane * 8 + sub)) + (1 << 29), F32))
            tops = []
            for _ in range(TOPC):
                top = jnp.max(jnp.max(_fold(jnp.maximum, keys), axis=1, keepdims=True), axis=0, keepdims=True)
                keys = [jnp.where(k == top, 0.0, k) for k in keys]
                tops.append(top)
            slot = lax.broadcasted_iota(I32, (TOPC, 1), 0)
            kcol = jnp.zeros((TOPC, 1), F32)
            for c in range(TOPC):
                kcol = jnp.where(slot == c, tops[c], kcol)
            rank = (pltpu.bitcast(kcol, I32) - (1 << 29)) >> 11
            r_sel = pltpu.bitcast(jnp.where(rank >= 0x8000, rank - 0x8000, 0xFFFF - rank) << 16, F32)
            toks = [S - 1 - (pltpu.bitcast(top, I32)[0, 0] & (S - 1)) for top in tops]
            grps = [pl.multiple_of(tok & (S - 16), 16) for tok in toks]
            row16 = lax.broadcasted_iota(I32, (16, M), 0)
            hits = [row16 == (tok & 15) for tok in toks]

            def gather(ref):
                out = jnp.zeros((TOPC, M), F32)
                for c in range(TOPC):
                    row = jnp.sum(jnp.where(hits[c], ref[pl.ds(grps[c], 16), :].astype(F32), 0.0),
                                  axis=0, keepdims=True)
                    out = jnp.where(slot == c, row, out)
                return out

            def up(xb, wt_s, w_s):
                return _rb(_cat([_dot(xb, _cat([wt_s[j, :M, :] for j in range(FA // 128)], 1)),
                                 _dot_nt(xb, w_s[FA:, :])], 1))

            xs = gather(h_s)
            gate = up(xs.astype(BF16), k_s, wg_s)
            act = _rb(gate * _rb(_sigmoid(gate))) * up(xs.astype(BF16), v_s, wu_s)
            y = _rb(_rb(_dot(act.astype(BF16), wd_s[...])) * _rb(_sigmoid(r_sel)))
            new = gather(x_s) + _rb(gates()[3] * _rb(xs + y))

            _wait(cp_out)
            for c in range(TOPC):
                old = out_s[pl.ds(grps[c], 16), :].astype(F32)
                out_s[pl.ds(grps[c], 16), :] = jnp.where(hits[c], new[c:c + 1], old).astype(BF16)
            patch = [pltpu.make_async_copy(out_s.at[pl.ds(g0, 16)], out_hbm.at[0, pl.ds(g0, 16)], sems.at[7])
                     for g0 in grps]
            fresh = [_fold(jnp.logical_and, [grps[j] != grps[c] for j in range(c)]) for c in range(1, TOPC)]
            patch[0].start()
            for f, cp in zip(fresh, patch[1:]):
                pl.when(f)(cp.start)
            patch[0].wait()
            for f, cp in zip(fresh, patch[1:]):
                pl.when(f)(cp.wait)

        def phase23(q_s, ctx_s, wor_s, h_s, out_s):
            _wait(cp_wo)
            _start(cp_late)
            pl.loop(0, NP)(lambda p: attend_pair(p, q_s, ctx_s, wor_s))
            finish(ctx_s, wor_s, h_s, out_s)

        pl.run_scoped(
            phase23,
            pltpu.VMEM((2, S, D), BF16), pltpu.VMEM((H, S, D), BF16), pltpu.VMEM((7, NP, D, 256), BF16),
            pltpu.VMEM((S, M), BF16), pltpu.VMEM((S, M), BF16))

    return kernel


@jax.jit
def pallas_adaLN_cond__compressed_kv_cla__moe_arch_mod__prompt_kernel(
    A_x, A_c_kv, A_w_q, A_w_uk, A_w_uv, A_w_o, B_x, B_w_r, B_w_gate, B_w_up, B_w_down, c, w_mod,
):
    del B_x
    _, S, M = A_x.shape
    Dc = A_c_kv.shape[2]
    H, D = A_w_q.shape[1:]
    F = B_w_gate.shape[1]
    assert (A_x.shape, A_c_kv.shape, H, D) == ((1, 2048, 640), (1, 2048, 512), 32, 128)
    return pl.pallas_call(
        _make_kernel(S, M, Dc, H, D, F),
        out_shape=jax.ShapeDtypeStruct(A_x.shape, A_x.dtype),
        in_specs=[pl.BlockSpec(memory_space=pl.ANY)] * 12,
        out_specs=pl.BlockSpec(memory_space=pl.ANY),
        scratch_shapes=[
            pltpu.VMEM((S, M), BF16),
            pltpu.VMEM((H // HG, HG // 2 * M, D), U32),
            pltpu.VMEM((H, D, M), BF16),
            pltpu.VMEM((F, M), BF16),
            pltpu.VMEM((F, M), BF16),
            pltpu.VMEM((F, M), BF16),
            pltpu.VMEM((M, 4 * M), BF16),
            pltpu.VMEM((H, S, D), BF16),
            pltpu.VMEM((H, S, D), BF16),
            pltpu.VMEM((8, S // 2, 256), BF16),
            pltpu.VMEM((1, M), BF16),
            pltpu.VMEM((M,), BF16),
            pltpu.SemaphoreType.DMA((8,)),
            pltpu.SemaphoreType.DMA((H // HG,)),
            pltpu.SemaphoreType.DMA((len(KV_CHUNKS),)),
        ],
        compiler_params=pltpu.CompilerParams(vmem_limit_bytes=120 * 1024 * 1024),
        name="adaln_mla_mod",
    )(A_x, A_c_kv, A_w_q, A_w_uk, A_w_uv, A_w_o, B_w_r, B_w_gate.T, B_w_up.T, B_w_down, c, w_mod)
```

```python
import numpy as np
import jax
import jax.numpy as jnp
from jax import lax
import jax.experimental.pallas as pl
import jax.experimental.pallas.tpu as pltpu

F32 = jnp.float32
BF16 = jnp.bfloat16
U32 = jnp.uint32
I32 = jnp.int32
TOPC = 8
LOG2E = 1.4426950408889634
EPS = 1e-5
RG = 16
G = 64
UR = 256
SB = 512
HG = 8
KV_CHUNKS = (512, 512, 1024)
OUT_BLOCKS = (512, 512, 384, 256, 192, 128, 64)
PAIR_ORDER = "QA W a0A a1A b0A a2A b1A a3A b2A QB a0B a1B b3A b0B a2B b1B a3B b2B b3B".split()


def _rb(a):
    return a.astype(BF16).astype(F32)


def _dot(a, b):
    return jnp.dot(a, b, preferred_element_type=F32)


def _dot_nt(a, b):
    return lax.dot_general(a, b, (((1,), (1,)), ((), ())), preferred_element_type=F32)


def _sigmoid(a):
    return 1.0 / (1.0 + jnp.exp(-a))


def _cat(xs, axis):
    return jnp.concatenate(xs, axis=axis) if len(xs) > 1 else xs[0]


def _fold(op, xs):
    acc = xs[0]
    for x in xs[1:]:
        acc = op(acc, x)
    return acc


def _words(w):
    return pltpu.bitcast(w.reshape(w.shape[0] * w.shape[1], w.shape[2]), U32)


def _halves(u):
    return pltpu.bitcast(u << 16, F32), pltpu.bitcast(u & np.uint32(0xFFFF0000), F32)


def _after(always, val, deps):
    t = _fold(jnp.maximum, deps)
    if val.dtype == BF16:
        t = pltpu.bitcast(t.astype(BF16), I32)
        out = jnp.where(jnp.tile(always, (t.shape[0] // 8, 1)), pltpu.bitcast(val, I32), t)
        return pltpu.bitcast(out, BF16)
    if val.dtype != F32:
        t = pltpu.bitcast(t, val.dtype)
    return jnp.where(jnp.tile(always, (t.shape[0] // 8, 1)), val, t)


class _Side:
    def __init__(self, always=None, stagger=0):
        self.always, self.stagger, self.jobs, self.done, self.n = always, stagger, {}, {}, 0

    def spread(self, jobs, span, delay=0):
        for t, job in enumerate(jobs):
            self.jobs.setdefault(self.n + delay + t * span // len(jobs), []).append(job)

    def lhs(self, x):
        toks = self.done.pop(self.n, None)
        if not toks:
            return x
        rows = 8 if x.dtype == F32 else 16
        head = _after(self.always, x[:rows, :128], [jnp.tile(t, (rows // 8, 1)) for t in toks])
        return _cat([_cat([head, x[rows:, :128]], 0), x[:, 128:]], 1)

    def result(self, d):
        jobs = self.jobs.pop(self.n, ())
        for t, job in enumerate(jobs):
            tok = job(d[self.stagger * t // len(jobs) // 8 * 8:, :128])
            if tok is not None:
                self.done.setdefault(self.n + 2, []).append(tok)
        self.n += 1


def _split_rows(x):
    n = x.shape[0] // (2 * RG)
    y = x.reshape(n, 2, RG, x.shape[1])
    return y[:, 0].reshape(n * RG, x.shape[1]), y[:, 1].reshape(n * RG, x.shape[1])


def _merge_rows(top, bot):
    n = top.shape[0] // RG
    y = jnp.concatenate([top.reshape(n, 1, RG, top.shape[1]), bot.reshape(n, 1, RG, top.shape[1])], axis=1)
    return y.reshape(2 * n * RG, top.shape[1])


_LHS = (lambda a: a[0][0] + a[1][1], lambda a: a[1][0] + a[1][1], lambda a: a[0][0], lambda a: a[1][1],
        lambda a: a[0][0] + a[0][1], lambda a: a[1][0] - a[0][0], lambda a: a[0][1] - a[1][1])
_RHS = (lambda b: b[0][0] + b[1][1], lambda b: b[0][0], lambda b: b[0][1] - b[1][1],
        lambda b: b[1][0] - b[0][0], lambda b: b[1][1], lambda b: b[0][0] + b[0][1],
        lambda b: b[1][0] + b[1][1])
_ORDER = (2, 4, 3, 1, 0, 6, 5)


def _column(m, e):
    if e == 0:
        return (m[3] - m[4]) + m[0] + m[6], m[1] + m[3]
    return m[2] + m[4], (m[2] - m[1]) + m[0] + m[5]


def _row_blocks(x):
    top, bot = _split_rows(x)
    hk = x.shape[1] // 2
    return (top[:, :hk], top[:, hk:]), (bot[:, :hk], bot[:, hk:])


def _pair_blocks(u):
    w = _halves(u)
    hk = u.shape[0] // 2
    return (w[0][:hk], w[1][:hk]), (w[0][hk:], w[1][hk:])


def _units(a, diag_pos):
    r0 = a * SB
    full = [[(r0 + ro, UR, c0, SB)] for c0 in range(0, r0, SB) for ro in range(0, SB, UR)]
    big = [(r0, 256, r0, 128), (r0 + 256, 256, r0, 384)]
    small = [(r0 + 128, 64, r0 + 128, 128), (r0 + 192, 64, r0 + 128, 128),
             (r0 + 384, 64, r0 + 384, 128), (r0 + 448, 64, r0 + 384, 128)]
    return [u for _, u in sorted(list(enumerate(full)) + list(zip(diag_pos, (big, small))), key=lambda z: z[0])]


def _start(cps):
    for cp in cps:
        cp.start()


def _wait(cps):
    for cp in cps:
        cp.wait()


def _make_kernel(S, M, Dc, H, D, F):
    NP, NG, PG = H // 2, H // HG, HG // 2
    FA = F // 128 * 128
    eps_b = float(np.asarray(EPS, dtype=BF16).astype(np.float32))
    qscale = float(np.asarray(D ** -0.5, dtype=BF16).astype(np.float32)) * LOG2E
    masked = -1e9 * LOG2E

    def kernel(x_hbm, ckv_hbm, wq_hbm, wuk_hbm, wuv_hbm, wo_hbm, wr_hbm, wg_hbm, wu_hbm,
               wd_hbm, c_hbm, wmod_hbm, out_hbm,
               x_s, wq_u, wo_s, wg_s, wu_s, wd_s, wmb_s, k_s, v_s, hl_s, c_s, wr_s, sems, qsems, csems):
        cp_wo = [pltpu.make_async_copy(wo_hbm, wo_s, sems.at[0])]
        cp_late = [pltpu.make_async_copy(wmod_hbm.at[:, 2 * M:6 * M], wmb_s, sems.at[1]),
                   pltpu.make_async_copy(wg_hbm, wg_s, sems.at[1]),
                   pltpu.make_async_copy(wu_hbm, wu_s, sems.at[1]),
                   pltpu.make_async_copy(wd_hbm, wd_s, sems.at[1])]

        def pair_words(ref, g, j):
            return ref[g, pl.ds(j, (ref.shape[1] - 8) // PG, stride=PG), :]

        def all_true(x):
            return (pltpu.bitcast(x, I32) | 1) != 0

        def modulation(w_s, always, outs):
            cv = c_s[...].astype(F32)
            sc = _rb(cv * _rb(_sigmoid(cv)))
            eye = lax.broadcasted_iota(I32, (128, 128), 0) == lax.broadcasted_iota(I32, (128, 128), 1)
            col = _cat([jnp.sum(jnp.where(eye, sc[:, t:t + 128], 0.0), axis=1, keepdims=True)
                        for t in range(0, M, 128)], 0)
            col = jnp.broadcast_to(col, (M, 128))

            step, part = 64, {}

            def job(t, r):
                def run(dep):
                    w = _after(always, w_s[r:r + step, t:t + 128], [jnp.tile(dep[:16], (step // 16, 1))])
                    prod = col[r:r + step] * w.astype(F32)
                    part[t] = _fold(jnp.add, ([part[t]] if r else []) + [prod[j:j + 8] for j in range(0, step, 8)])
                    if r + step == M:
                        outs.append(_rb(jnp.sum(part[t], axis=0, keepdims=True)))
                    return part[t]
                return run
            return [job(t, r) for t in range(0, w_s.shape[1], 128) for r in range(0, M, step)]

        def phase1(ckv_s, cl_s, w0_s, w0_u, wk_g, wv_g, wq_g, wk_u, wv_u, wma_s):
            chunks = KV_CHUNKS
            cstart = [sum(chunks[:i]) for i in range(len(chunks))]
            cp_w0 = [pltpu.make_async_copy(w.at[:, 0:2, :], w0_s.at[i], sems.at[2])
                     for i, w in enumerate((wuk_hbm, wuv_hbm))]
            cp_ckv = [pltpu.make_async_copy(ckv_hbm.at[0, r0:r0 + nr], ckv_s.at[r0:r0 + nr], csems.at[i])
                      for i, (r0, nr) in enumerate(zip(cstart, chunks))]
            cp_kv = [[pltpu.make_async_copy(w.at[:, HG * g:HG * (g + 1), :], dst.at[g], sems.at[3 if g == 0 else 4])
                      for w, dst in ((wuk_hbm, wk_g), (wuv_hbm, wv_g))] for g in range(NG)]
            cp_kv_rest = [cp for cps in cp_kv[1:] for cp in cps]
            cp_ln = [pltpu.make_async_copy(c_hbm, c_s, sems.at[5]),
                     pltpu.make_async_copy(wr_hbm, wr_s, sems.at[5]),
                     pltpu.make_async_copy(wmod_hbm.at[:, 0:2 * M], wma_s, sems.at[5])]

            def cp_step(g):
                rows = pl.ds(pl.multiple_of(S // NG * g, S // NG), S // NG)
                return [pltpu.make_async_copy(wq_hbm.at[:, pl.ds(pl.multiple_of(HG * g, HG), HG), :],
                                              wq_g.at[g], qsems.at[g]),
                        pltpu.make_async_copy(x_hbm.at[0, rows], x_s.at[rows], qsems.at[g])]

            def repack(always, src, dst, g, step=16):
                def job(r):
                    def run(dep):
                        u = _after(always, _words(src[g, r:r + step]), [jnp.tile(dep[:8], (PG * step // 8, 1))])
                        dst[g, PG * r:PG * (r + step), :] = u
                        return pltpu.bitcast(_fold(jnp.bitwise_and, [u[t:t + 8] for t in range(0, PG * step, 8)]), F32)
                    return run
                return [job(r) for r in range(0, src.shape[1], step)]

            def kv_proj(p, uk, uv, side, r0=0, nr=S):
                bk, bv = _pair_blocks(uk), _pair_blocks(uv)
                m = [None] * 7
                for i in _ORDER:
                    m[i] = _dot(side.lhs(cl_s[i, r0 // 2:(r0 + nr) // 2, :]),
                                _cat([_RHS[i](bk), _RHS[i](bv)], 1).astype(BF16))
                    side.result(m[i])
                for e in range(2):
                    o = _merge_rows(*_column(m, e))
                    k_s[2 * p + e, r0:r0 + nr, :] = o[:, :D].astype(BF16)
                    v_s[2 * p + e, r0:r0 + nr, :] = o[:, D:].astype(BF16)

            def kv_pair(p, side):
                kv_proj(p, pair_words(wk_u, p // PG, p % PG), pair_words(wv_u, p // PG, p % PG), side)

            _start(cp_w0 + cp_ckv[:1])
            for ref in (wq_u, wk_u, wv_u):
                ref[:, ref.shape[1] - 8:, :] = jnp.zeros((NG, 8, D), U32)
            _wait(cp_w0)
            _start(cp_ckv[1:])
            for i in range(2):
                for r in range(Dc):
                    w0_u[i, r:r + 1, :] = pltpu.bitcast(w0_s[i, r], U32)
            for i, (r0, nr) in enumerate(zip(cstart, chunks)):
                _wait(cp_ckv[i:i + 1])
                if i == 0:
                    _start(cp_kv[0])
                blocks = _row_blocks(ckv_s[r0:r0 + nr, :].astype(F32))
                for j in _ORDER:
                    cl_s[j, r0 // 2:(r0 + nr) // 2, :] = _LHS[j](blocks).astype(BF16)
                kv_proj(0, w0_u[0], w0_u[1], _Side(), r0, nr)
            _wait(cp_kv[0])
            _start(cp_kv_rest + cp_ln + cp_step(0))
            wk_u[0, :PG * Dc, :] = _words(wk_g[0])
            wv_u[0, :PG * Dc, :] = _words(wv_g[0])
            for p in range(1, PG - 1):
                kv_pair(p, _Side())
            _wait(cp_kv_rest)
            side = _Side(all_true(w0_u[0, :8, :]), S // 2 - 64)
            side.spread([job for g in range(1, NG) for src, dst in ((wk_g, wk_u), (wv_g, wv_u))
                         for job in repack(side.always, src, dst, g)], 6)
            kv_pair(PG - 1, side)
            _wait(cp_ln)
            _start([cp for g in range(1, NG) for cp in cp_step(g)] + cp_wo)

            def step(i, carry):
                _wait(cp_step(i))
                always = lax.broadcasted_iota(I32, (8, 128), 0) < i + 8
                g, rows, mod = 2 * RG, S // NG, []

                def ln1(r):
                    def run(dep):
                        r0 = pl.multiple_of(i * rows + r, g)
                        xv = _cat([_after(always, x_s[pl.ds(r0, g), t:t + 128], [dep[:g]])
                                   for t in range(0, M, 128)], 1).astype(F32)
                        mu = jnp.sum(xv, axis=-1, keepdims=True) * (1.0 / M)
                        xc = xv - mu
                        var = jnp.sum(xc * xc, axis=-1, keepdims=True) * (1.0 / M)
                        sa, ca = _cat(mod[:M // 128], 1), _cat(mod[M // 128:], 1)
                        h = xc * lax.rsqrt(var + EPS) * _rb(1.0 + ca) + sa
                        blocks = _row_blocks(h[:, :512])
                        rh = pl.ds(pl.multiple_of(i * (rows // 2) + r // 2, g // 2), g // 2)
                        for j in range(7):
                            hl_s[j, rh, :] = _LHS[j](blocks).astype(BF16)
                        hl_s[7, rh, :] = _cat(_split_rows(h[:, 512:]), 1).astype(BF16)
                        return _fold(jnp.maximum, [h[j:j + 8, t:t + 128] for j in range(0, g, 8)
                                                   for t in range(0, M, 128)])
                    return run

                side = _Side(always, S // 2 - 64)
                side.spread(modulation(wma_s, always, mod), 4)
                side.spread([ln1(r) for r in range(0, rows, g)], 14, 4)
                side.spread(repack(always, wq_g, wq_u, i), 16)
                for u in range(PG - 1):
                    kv_pair(PG + (PG - 1) * i + u, side)
                return carry

            lax.fori_loop(0, NG, step, 0)

        pl.run_scoped(
            phase1,
            pltpu.VMEM((S, Dc), BF16), pltpu.VMEM((7, S // 2, Dc // 2), BF16),
            pltpu.VMEM((2, Dc, 2, D), BF16), pltpu.VMEM((2, Dc, D), U32),
            pltpu.VMEM((NG, Dc, HG, D), BF16), pltpu.VMEM((NG, Dc, HG, D), BF16), pltpu.VMEM((NG, M, HG, D), BF16),
            pltpu.VMEM((NG, PG * Dc + 8, D), U32), pltpu.VMEM((NG, PG * Dc + 8, D), U32),
            pltpu.VMEM((M, 2 * M), BF16))

        def attend_pair(p, q_s, ctx_s, wor_s):
            always = lax.broadcasted_iota(I32, (8, 128), 0) < p + 8
            dist = lax.broadcasted_iota(I32, (G, 128), 1) - lax.broadcasted_iota(I32, (G, 128), 0)
            st, clock, pend, fins, last = {}, [0], [], [], [None]

            def proj_q(e):
                u = pair_words(wq_u, p // PG, p % PG)
                bq = _pair_blocks(u[:512])
                if e == 0:
                    wt = _cat(_halves(u[512:]), 1).astype(BF16)
                    st["qt"] = [_dot(hl_s[7, :, :128], wt), _dot(hl_s[7, :, 128:], wt)]
                    st["qm"] = [None] * 7
                    for i in _ORDER[:-1]:
                        st["qm"][i] = _dot(hl_s[i], _RHS[i](bq).astype(BF16))
                else:
                    w = _RHS[5](bq).astype(BF16)
                    st["qm"][5] = _cat([_dot(hl_s[5, :S // 4, :], w), _dot(hl_s[5, S // 4:, :], w)], 0)
                top, bot = _column(st["qm"], e)
                o = _merge_rows(top + st["qt"][0][:, D * e:D * (e + 1)], bot + st["qt"][1][:, D * e:D * (e + 1)])
                q_s[e] = (o * qscale).astype(BF16)
                clock[0] += 512

            def o_operands():
                dep = _cat([st["qm"][2][t:t + 16] for t in range(0, S // 2, S // 16)], 0)
                wa, wb = (_cat([_after(always, wo_s[2 * p + e, :, t:t + 128], [dep]) for t in range(0, 512, 128)],
                               1).astype(F32) for e in range(2))
                for i in range(7):
                    wor_s[i, p] = _RHS[i](((wa[:, :256], wa[:, 256:]), (wb[:, :256], wb[:, 256:]))).astype(BF16)

            def acc(key, r0, val, op):
                for u in range(val.shape[0] // G):
                    k = (key, r0 // G + u)
                    part = val[G * u:G * (u + 1)]
                    st[k] = op(st[k], part) if k in st else part

            def get(key, r0, nr):
                return _cat([st[(key, u)] for u in range(r0 // G, (r0 + nr) // G)], 0)

            def take(val, kinds, extra=()):
                ready = [z for z in pend if z[0] <= clock[0] and z[1].shape[0] == val.shape[0] and z[2] in kinds]
                pend[:] = [z for z in pend if not any(z is y for y in ready)]
                deps = [z[1] for z in ready] + list(extra)
                return _after(always, val, deps) if deps else val

            def normalize(dep):
                if not fins:
                    return
                e, r0 = fins.pop(0)
                l = get(("l", e), r0, UR)
                if dep is not None:
                    l = _after(always, l, [dep])
                l = jnp.sum(l, axis=-1, keepdims=True)
                r = pl.reciprocal(l, approx=True)
                ctx = get(("o", e), r0, UR) * (r * (2.0 - l * r))
                ctx_s[2 * p + e, r0:r0 + UR, :] = ctx.astype(BF16)
                pend.append((clock[0] + UR, ctx, "f"))

            def scores(e, a):
                for unit in _units(a, (-1, 0.5)):
                    for (r0, nr, c0, nc) in unit:
                        s = _dot_nt(take(q_s[e, r0:r0 + nr, :], "fM"), k_s[2 * p + e, c0:c0 + nc, :])
                        tiles = []
                        for t in range(c0, c0 + nc, 128):
                            x = s[:, t - c0:t - c0 + 128]
                            if t + 128 > r0:
                                x = _cat([x[g:g + G] if t + 128 <= r0 + g else
                                          jnp.where(dist <= r0 + g - t, x[g:g + G], masked)
                                          for g in range(0, nr, G)], 0)
                            tiles.append(x)
                        mm = _fold(jnp.maximum, tiles)
                        acc(("m", e), r0, mm, jnp.maximum)
                        st[("s", e, r0, c0)] = tiles
                    clock[0] += nr
                    if nr == UR:
                        normalize(mm)
                        last[0] = mm
                for u in range(a * SB // G, (a + 1) * SB // G):
                    k = (("m", e), u)
                    st[k] = jnp.broadcast_to(jnp.max(st[k], axis=-1, keepdims=True), (G, 128))
                for r0 in range(a * SB, (a + 1) * SB, UR):
                    pend.append((clock[0] + UR + r0 - a * SB, get(("m", e), r0, UR), "M"))

            def context(e, a):
                for unit in _units(a, (1.5, 2.5)):
                    for (r0, nr, c0, nc) in unit:
                        m = take(get(("m", e), r0, nr), "f", [last[0][:nr]])
                        ps = [jnp.exp2(x - m) for x in st.pop(("s", e, r0, c0))]
                        acc(("l", e), r0, _fold(jnp.add, ps), jnp.add)
                        ps[-1] = _after(always, ps[-1], [get(("l", e), r0, nr)])
                        acc(("o", e), r0, _dot(_cat(ps, 1).astype(BF16), v_s[2 * p + e, c0:c0 + nc, :]), jnp.add)
                    clock[0] += nr
                    if len(unit) == 1:
                        normalize(get(("o", e), r0, nr))
                    if nr == UR:
                        last[0] = get(("o", e), r0, nr)
                fins.extend((e, r0) for r0 in range(a * SB, (a + 1) * SB, UR))

            for tok in PAIR_ORDER:
                if tok == "W":
                    o_operands()
                elif tok[0] == "Q":
                    proj_q("AB".index(tok[1]))
                else:
                    (scores if tok[0] == "a" else context)("AB".index(tok[2]), int(tok[1]))
            while fins:
                normalize(None)

        def finish(ctx_s, wor_s, h_s, out_s):
            _wait(cp_late)
            wr = wr_s[...].astype(F32).reshape(1, M)
            always = all_true(jnp.broadcast_to(wr[:, :128], (8, 128)))
            lane = lax.broadcasted_iota(I32, (8, 128), 1)
            sub = lax.broadcasted_iota(I32, (8, 128), 0)
            score = [jnp.zeros((8, 128), F32) for _ in range(S // 1024)]
            side, mod = _Side(always), []

            def o_proj(r0, nr):
                m = [None] * 7
                for p0 in range(0, NP, 2):
                    blocks = []
                    for pp in (p0, p0 + 1):
                        a0, a1 = (_split_rows(ctx_s[2 * pp + e, r0:r0 + nr, :].astype(F32)) for e in range(2))
                        blocks.append(((a0[0], a1[0]), (a0[1], a1[1])))
                    for i in _ORDER:
                        d = _dot(side.lhs(_cat([_LHS[i](b) for b in blocks], 1)).astype(BF16),
                                 _cat([wor_s[i, p0], wor_s[i, p0 + 1]], 0))
                        m[i] = d if m[i] is None else m[i] + d
                        side.result(m[i])
                tail = None
                for h0 in range(0, H, 4):
                    d = _dot(side.lhs(_cat([ctx_s[hh, r0:r0 + nr, :] for hh in range(h0, h0 + 4)], 1)),
                             _cat([wo_s[hh, :, 512:] for hh in range(h0, h0 + 4)], 0))
                    tail = d if tail is None else tail + d
                    side.result(tail)
                return _cat([_merge_rows(*_column(m, e)) for e in range(2)] + [tail], 1)

            def gates():
                ga, sb, cb, gb = (_cat(mod[t:t + M // 128], 1) for t in range(0, len(mod), M // 128))
                return ga, sb, _rb(1.0 + cb), gb

            def ln2(r0, attn):
                nr = attn.shape[0]
                ga, sb, cb1, gb = gates()
                x1 = _rb(x_s[r0:r0 + nr, :].astype(F32) + _rb(ga * _rb(attn)))
                x_s[r0:r0 + nr, :] = x1.astype(BF16)
                mu = jnp.sum(x1, axis=-1, keepdims=True) / M
                xc = x1 - mu
                var = _rb(jnp.sum(xc * xc, axis=-1, keepdims=True) / M)
                inv = 1.0 / _rb(jnp.sqrt(_rb(var + eps_b)))
                h2 = _rb(_rb(_rb(_rb(x1 - _rb(mu)) * inv) * cb1) + sb)
                h_s[r0:r0 + nr, :] = h2.astype(BF16)
                out_s[r0:r0 + nr, :] = (x1 + _rb(gb * h2)).astype(BF16)
                r = jnp.sum(h2 * wr, axis=-1, keepdims=True)
                for j in range(nr // 8):
                    g = r0 // 8 + j
                    score[g // 128] = jnp.where(lane == g % 128, r[8 * j:8 * j + 8], score[g // 128])

            def ln2_job(r0, attn):
                return lambda dep: ln2(r0, _cat([_after(always, attn[:, t:t + 128], [dep[:attn.shape[0]]])
                                                 for t in range(0, M, 128)], 1))

            def transpose_job(w_s, dst, f0):
                def run(dep):
                    wt = _cat([_after(always, w_s[f0:f0 + 128, t:t + 128], [dep[:128]])
                               for t in range(0, M, 128)], 1)
                    dst[f0 // 128, :M, :] = wt.astype(F32).T.astype(BF16)
                return run

            eblocks = OUT_BLOCKS
            starts = [sum(eblocks[:i]) for i in range(len(eblocks))]
            cp_out = [pltpu.make_async_copy(out_s.at[r0:r0 + nr], out_hbm.at[0, r0:r0 + nr], sems.at[6])
                      for r0, nr in zip(starts, eblocks)]
            side.spread(modulation(wmb_s, always, mod), 60)
            side.spread([transpose_job(w_s, dst, f0) for w_s, dst in ((wg_s, k_s), (wu_s, v_s))
                         for f0 in range(0, FA, 128)], 60)
            for i, (r0, nr) in enumerate(zip(starts, eblocks)):
                attn = o_proj(r0, nr)
                if i > 0:
                    cp_out[i - 1].start()
                if i + 1 < len(eblocks):
                    side.spread([ln2_job(r0 + r, attn[r:r + 8]) for r in range(0, nr, 8)], 60)
                else:
                    ln2(r0, attn)
                    cp_out[i].start()

            keys = []
            for t, r in enumerate(score):
                r = _rb(r)
                b = lax.shift_right_logical(pltpu.bitcast(jnp.where(r == 0.0, 0.0, r), I32), 16)
                rank = jnp.where(r != r, 0, jnp.where(b >= 0x8000, 0xFFFF - b, b + 0x8000))
                keys.append(pltpu.bitcast((rank << 11) + (S - 1 - (t * 1024 + lane * 8 + sub)) + (1 << 29), F32))
            tops = []
            for _ in range(TOPC):
                top = jnp.max(jnp.max(_fold(jnp.maximum, keys), axis=1, keepdims=True), axis=0, keepdims=True)
                keys = [jnp.where(k == top, 0.0, k) for k in keys]
                tops.append(top)
            slot = lax.broadcasted_iota(I32, (TOPC, 1), 0)
            kcol = jnp.zeros((TOPC, 1), F32)
            for c in range(TOPC):
                kcol = jnp.where(slot == c, tops[c], kcol)
            rank = (pltpu.bitcast(kcol, I32) - (1 << 29)) >> 11
            r_sel = pltpu.bitcast(jnp.where(rank >= 0x8000, rank - 0x8000, 0xFFFF - rank) << 16, F32)
            toks = [S - 1 - (pltpu.bitcast(top, I32)[0, 0] & (S - 1)) for top in tops]
            grps = [pl.multiple_of(tok & (S - 16), 16) for tok in toks]
            row16 = lax.broadcasted_iota(I32, (16, M), 0)
            hits = [row16 == (tok & 15) for tok in toks]

            def gather(ref):
                out = jnp.zeros((TOPC, M), F32)
                for c in range(TOPC):
                    row = jnp.sum(jnp.where(hits[c], ref[pl.ds(grps[c], 16), :].astype(F32), 0.0),
                                  axis=0, keepdims=True)
                    out = jnp.where(slot == c, row, out)
                return out

            def up(xb, wt_s, w_s):
                return _rb(_cat([_dot(xb, _cat([wt_s[j, :M, :] for j in range(FA // 128)], 1)),
                                 _dot_nt(xb, w_s[FA:, :])], 1))

            xs = gather(h_s)
            gate = up(xs.astype(BF16), k_s, wg_s)
            act = _rb(gate * _rb(_sigmoid(gate))) * up(xs.astype(BF16), v_s, wu_s)
            y = _rb(_rb(_dot(act.astype(BF16), wd_s[...])) * _rb(_sigmoid(r_sel)))
            new = gather(x_s) + _rb(gates()[3] * _rb(xs + y))

            _wait(cp_out)
            for c in range(TOPC):
                old = out_s[pl.ds(grps[c], 16), :].astype(F32)
                out_s[pl.ds(grps[c], 16), :] = jnp.where(hits[c], new[c:c + 1], old).astype(BF16)
            patch = [pltpu.make_async_copy(out_s.at[pl.ds(g0, 16)], out_hbm.at[0, pl.ds(g0, 16)], sems.at[7])
                     for g0 in grps]
            fresh = [_fold(jnp.logical_and, [grps[j] != grps[c] for j in range(c)]) for c in range(1, TOPC)]
            patch[0].start()
            for f, cp in zip(fresh, patch[1:]):
                pl.when(f)(cp.start)
            patch[0].wait()
            for f, cp in zip(fresh, patch[1:]):
                pl.when(f)(cp.wait)

        def phase23(q_s, ctx_s, wor_s, h_s, out_s):
            _wait(cp_wo)
            _start(cp_late)
            pl.loop(0, NP)(lambda p: attend_pair(p, q_s, ctx_s, wor_s))
            finish(ctx_s, wor_s, h_s, out_s)

        pl.run_scoped(
            phase23,
            pltpu.VMEM((2, S, D), BF16), pltpu.VMEM((H, S, D), BF16), pltpu.VMEM((7, NP, D, 256), BF16),
            pltpu.VMEM((S, M), BF16), pltpu.VMEM((S, M), BF16))

    return kernel


@jax.jit
def pallas_adaLN_cond__compressed_kv_cla__moe_arch_mod__prompt_kernel(
    A_x, A_c_kv, A_w_q, A_w_uk, A_w_uv, A_w_o, B_x, B_w_r, B_w_gate, B_w_up, B_w_down, c, w_mod,
):
    del B_x
    _, S, M = A_x.shape
    Dc = A_c_kv.shape[2]
    H, D = A_w_q.shape[1:]
    F = B_w_gate.shape[1]
    assert (A_x.shape, A_c_kv.shape, H, D) == ((1, 2048, 640), (1, 2048, 512), 32, 128)
    return pl.pallas_call(
        _make_kernel(S, M, Dc, H, D, F),
        out_shape=jax.ShapeDtypeStruct(A_x.shape, A_x.dtype),
        in_specs=[pl.BlockSpec(memory_space=pl.ANY)] * 12,
        out_specs=pl.BlockSpec(memory_space=pl.ANY),
        scratch_shapes=[
            pltpu.VMEM((S, M), BF16),
            pltpu.VMEM((H // HG, HG // 2 * M + 8, D), U32),
            pltpu.VMEM((H, D, M), BF16),
            pltpu.VMEM((F, M), BF16),
            pltpu.VMEM((F, M), BF16),
            pltpu.VMEM((F, M), BF16),
            pltpu.VMEM((M, 4 * M), BF16),
            pltpu.VMEM((H, S, D), BF16),
            pltpu.VMEM((H, S, D), BF16),
            pltpu.VMEM((8, S // 2, 256), BF16),
            pltpu.VMEM((1, M), BF16),
            pltpu.VMEM((M,), BF16),
            pltpu.SemaphoreType.DMA((8,)),
            pltpu.SemaphoreType.DMA((H // HG,)),
            pltpu.SemaphoreType.DMA((len(KV_CHUNKS),)),
        ],
        compiler_params=pltpu.CompilerParams(vmem_limit_bytes=120 * 1024 * 1024),
        name="adaln_mla_mod",
    )(A_x, A_c_kv, A_w_q, A_w_uk, A_w_uv, A_w_o, B_w_r, B_w_gate.T, B_w_up.T, B_w_down, c, w_mod)
```
